```python
import jax
import jax.numpy as jnp

def _softmax(x, axis=-1):
    return jax.nn.softmax(x, axis=axis)
def _gelu(x):
    return jax.nn.gelu(x, approximate=True)
def _silu(x):
    return jax.nn.silu(x)
def _sigmoid(x):
    return jax.nn.sigmoid(x)
def _layernorm(x, axis=-1, eps=1e-5):
    m = jnp.mean(x, axis=axis, keepdims=True)
    v = jnp.var(x, axis=axis, keepdims=True)
    return (x - m) / jnp.sqrt(v + eps)
def _scatter_add(tgt, idx, src, axis=0):
    return tgt.at[idx].add(src)
def _segment_sum(src, seg, n):
    return jax.ops.segment_sum(src, seg, n)
class _Rng:
    def __init__(self, key):
        self._k = key
    def _next(self):
        self._k, sub = jax.random.split(self._k)
        return sub
    def normal(self, shape):
        return jax.random.normal(self._next(), shape, dtype=jnp.bfloat16)
    def randint(self, lo, hi, shape):
        return jax.random.randint(self._next(), shape, lo, hi, dtype=jnp.int32)
    def uniform(self, shape, lo=0.0, hi=1.0):
        return jax.random.uniform(self._next(), shape, jnp.bfloat16, lo, hi)
    def permutation(self, n):
        return jax.random.permutation(self._next(), n)


kernel_name = 'parallel_sum__ssm_conv_h3__dense_activation_gelu__prompt'

def setup_inputs():
    _rng = _Rng(jax.random.key(int.from_bytes(__import__("os").urandom(4), "little")))
    _w = (lambda a: (lambda t: t.astype(jnp.bfloat16) if jnp.issubdtype(t.dtype, jnp.floating) else t)(jnp.asarray(a)))
    def _A_setup():
        B, S, D = 1, 2048, 640
        ks = 4
        return {
            "q": _w((lambda *s: _rng.normal(s) * 0.05)(B, S, D)),
            "k": _w((lambda *s: _rng.normal(s) * 0.05)(B, S, D)),
            "v": _w((lambda *s: _rng.normal(s) * 0.05)(B, S, D)),
            "shift_k": _w((lambda *s: _rng.normal(s) * 0.05)(D, ks) * 0.5),
            "ssm_k": _w((lambda *s: _rng.normal(s) * 0.05)(D, S) * (1.0 / S ** 0.5)),
            "ssm_D": _w((lambda *s: _rng.normal(s) * 0.05)(D)),
        }
    _A_in = _A_setup()

    def _B_setup():
        B, S, D, F = 1, 2048, 640, 1728
        return {
            "x": _w((lambda *s: _rng.normal(s) * 0.05)(B, S, D)),
            "w1": _w((lambda *s: _rng.normal(s) * 0.05)(D, F) * (D ** -0.5)),
            "b1": _w((lambda *s: _rng.normal(s) * 0.05)(F) * 0.01),
            "w2": _w((lambda *s: _rng.normal(s) * 0.05)(F, D) * (F ** -0.5)),
            "b2": _w((lambda *s: _rng.normal(s) * 0.05)(D) * 0.01),
        }
    _B_in = _B_setup()

    return {
        "A_q": _A_in["q"],
        "A_k": _A_in["k"],
        "A_v": _A_in["v"],
        "A_shift_k": _A_in["shift_k"],
        "A_ssm_k": _A_in["ssm_k"],
        "A_ssm_D": _A_in["ssm_D"],
        "B_x": _B_in["x"],
        "B_w1": _B_in["w1"],
        "B_b1": _B_in["b1"],
        "B_w2": _B_in["w2"],
        "B_b2": _B_in["b2"],
    }

def reference(A_q, A_k, A_v, A_shift_k, A_ssm_k, A_ssm_D, B_x, B_w1, B_b1, B_w2, B_b2):
    def _A_ref(q, k, v, shift_k, ssm_k, ssm_D):
        B, S, D = q.shape
        ks = shift_k.shape[-1]
        k_pad = jnp.pad(k, ((0, 0), (ks - 1, 0), (0, 0)))
        k_shift = jnp.zeros_like(k)
        for t in range(ks):
            k_shift = k_shift + k_pad[:, t:t + S, :] * shift_k[:, ks - 1 - t][None, None, :]
        kv = k_shift * v
        L = 2 * S
        kv_pad = jnp.pad(kv, ((0, 0), (0, S), (0, 0)))
        kf_pad = jnp.pad(ssm_k, ((0, 0), (0, S)))
        kv_f = (lambda x, axes=(-2,-1): jnp.fft.rfft2(x.astype(jnp.float32), axes=axes))(kv_pad[:, None, :, :], axes=(1, 2))
        kf_f = (lambda x, axes=(-2,-1): jnp.fft.rfft2(x.astype(jnp.float32), axes=axes))(kf_pad[:, None, :], axes=(1, 2))
        kf_f = (lambda x, *d: x.transpose(*d))(kf_f, 1, 2, 0)
        y_f = kv_f * kf_f[None, :, :, :]
        y = (lambda x, s, axes=(-2,-1): jnp.fft.irfft2(x, s=s, axes=axes).astype(jnp.bfloat16))(y_f, (1, L), axes=(1, 2))[:, 0, :S, :]
        y = y + kv * ssm_D[None, None, :]
        return q * y

    def _B_ref(x, w1, b1, w2, b2):
        h = jnp.einsum("bsd,df->bsf", x, w1) + b1
        h = _gelu(h)
        return jnp.einsum("bsf,fd->bsd", h, w2) + b2

    x = A_q
    xn = _layernorm(x, axis=-1)
    return x + _A_ref(xn, A_k, A_v, A_shift_k, A_ssm_k, A_ssm_D) + _B_ref(xn, B_w1, B_b1, B_w2, B_b2)
```

```python
import functools
import jax, jax.numpy as jnp, numpy as np
from jax import lax
from jax.experimental import pallas as pl
from jax.experimental.pallas import tpu as pltpu

S, D, F = 2048, 640, 1728
B = 128
NB = S // B
TM = 256
NSTEP = S // TM
NT = D // 128
R8 = B // 8
Z = NB
DUM = NB + 1
H0 = NB + 2
f32 = jnp.float32
bf16 = jnp.bfloat16
u32 = jnp.uint32
NT_DIMS = (((1,), (1,)), ((), ()))

def dft_mats():
    k = np.concatenate([np.arange(0, B, 2), np.arange(1, B, 2)]).astype(np.float64) + 0.5
    n = np.arange(B, dtype=np.float64)
    th = 2 * np.pi * np.outer(k, n) / (2 * B)
    Fm = np.concatenate([np.cos(th), -np.sin(th)], 0)
    Gm = np.concatenate([np.cos(th).T, -np.sin(th).T], 1) / B
    return Fm.astype(np.float32), Gm.astype(np.float32)

def make(depth=2, cl=1, tie=True, kvanchor=(1536,), hchunks=2, kvrows=64, loop_end=8, hdyn=True):
    def kern(z_ref, x_hbm, k_hbm, v_hbm, h_hbm, w1_hbm, w2_hbm, sk_ref, sD_ref, b1_ref, b2_ref, Fm_ref, Gm_ref,
             o_hbm,
             UH, x_v, o_v, k_v, v_v, h_v, w1_v, w2_v, w1p, w2p, kvb_ref, Q_ref, xn_ref,
             sem_x, sem_k, sem_v, sem_h, sem_w, sem_o):
        def rows(i):
            return pl.ds(pl.multiple_of(i * TM, TM), TM)
        cx = lambda i: pltpu.make_async_copy(x_hbm.at[rows(i)], x_v.at[rows(i)], sem_x.at[i])
        ck = lambda i: pltpu.make_async_copy(k_hbm.at[rows(i)], k_v.at[pl.ds(pl.multiple_of(16 + i * TM, 16), TM)], sem_k.at[i])
        cv = lambda i: pltpu.make_async_copy(v_hbm.at[rows(i)], v_v.at[rows(i)], sem_v.at[i])
        ch = lambda c: pltpu.make_async_copy(h_hbm.at[pl.ds(c * 128, 128)], h_v.at[pl.ds(c * 128, 128)], sem_h.at[c])
        co = lambda i: pltpu.make_async_copy(o_v.at[rows(i)], o_hbm.at[rows(i)], sem_o.at[i])
        cw1 = pltpu.make_async_copy(w1_hbm, w1_v, sem_w.at[0])
        cw2 = pltpu.make_async_copy(w2_hbm, w2_v, sem_w.at[1])

        ck(0).start(); cv(0).start()
        for c in range(NT):
            ch(c).start()
        cx(0).start()

        zero = z_ref[0]
        never = jnp.full((8, 128), zero, jnp.int32) != 0
        k_v[0:16, :] = jnp.zeros((16, D), bf16)

        def kv_block(base, anchors=None):
            sk = sk_ref[...].astype(f32)
            nrc = TM // kvrows
            for c in range(NT):
                cs = slice(c * 128, (c + 1) * 128)
                if anchors is not None and c < len(anchors):
                    fr = pl.ds(pl.multiple_of(S + 16 + zero * 16, 16), 16)
                    k_v[fr, 0:128] = anchors[c]
                    fr = pl.ds(pl.multiple_of(S + zero * 16, 16), 16)
                    v_v[fr, 0:128] = anchors[c]
                for rc in range(nrc):
                    r0 = pl.multiple_of(base + rc * kvrows, 16)
                    kext = k_v[pl.ds(r0, kvrows + 16), cs].astype(f32)[8:]
                    ks = kext[8:] * sk[0:1, cs]
                    for j in range(1, 4):
                        ks = ks + pltpu.roll(kext, j, 0)[8:, :] * sk[j:j + 1, cs]
                    kv = ks * v_v[pl.ds(r0, kvrows), cs].astype(f32)
                    kvb_ref[rc * kvrows // 2:(rc + 1) * kvrows // 2, cs] = pltpu.bitcast(kv.astype(bf16), u32)

        UH[Z] = jnp.zeros(UH.shape[1:], f32)
        Fm = Fm_ref[...]
        hb = B // 2
        waits = {0: [0, 1], 2: [2, 3, 4]} if hchunks == 2 else {c: [c] for c in range(NT)}
        for c in range(NT):
            with jax.named_scope("waith"):
                if c == 0:
                    ck(0).wait(); cv(0).wait()
                for cc in waits.get(c, []):
                    ch(cc).wait()
            if c == 0:
                cw1.start()
            if c == 2:
                cw2.start(); ck(1).start(); cv(1).start()
            cs = slice(c * 128, (c + 1) * 128)
            hp_re = hp_im = None
            for a in range(NB):
                hh = lax.dot_general(Fm, h_v[cs, a * B:(a + 1) * B], NT_DIMS, preferred_element_type=f32)
                hre = hh[:B]; him = hh[B:]
                if a == 0:
                    hre = hre + sD_ref[...].astype(f32)[None, cs]
                    c_, d_ = hre, him
                else:
                    c_ = jnp.concatenate([hre[:hb] - hp_im[:hb], hre[hb:] + hp_im[hb:]], axis=0)
                    d_ = jnp.concatenate([him[:hb] + hp_re[:hb], him[hb:] - hp_re[hb:]], axis=0)
                UH[H0 + a, :, 0, :, cs] = c_.reshape(R8, 8, 128)
                UH[H0 + a, :, 1, :, cs] = (d_ - c_).reshape(R8, 8, 128)
                UH[H0 + a, :, 2, :, cs] = (c_ + d_).reshape(R8, 8, 128)
                hp_re, hp_im = hre, him
            if c == 1:
                kv_block(0)

        def step(t, first):
            nlag = 2 if first else NB
            tn = jnp.minimum(t + 1, NSTEP - 1) if not first else 1
            Fm = Fm_ref[...]
            for j in range(2):
                kvb = pltpu.bitcast(kvb_ref[j * (B // 2):(j + 1) * (B // 2), :], bf16)
                u = jnp.dot(Fm, kvb, preferred_element_type=f32)
                a = u[:B]; b = u[B:]
                UH[2 * t + j, :, 0] = (a + b).reshape(R8, 8, D)
                UH[2 * t + j, :, 1] = a.reshape(R8, 8, D)
                UH[2 * t + j, :, 2] = b.reshape(R8, 8, D)

            x = x_v[rows(t), :].astype(f32)
            m = jnp.mean(x, axis=-1, keepdims=True)
            xc = x - m
            var = jnp.mean(xc * xc, axis=-1, keepdims=True)
            xn = xc * lax.rsqrt(var + 1e-5)
            xn_ref[...] = pltpu.bitcast(xn.astype(bf16), u32)
            xnb = pltpu.bitcast(xn_ref[...], bf16)

            if first:
                w1 = w1_v[...]; w2 = w2_v[...]
                w1p[...] = pltpu.bitcast(w1, u32); w2p[...] = pltpu.bitcast(w2, u32)
            else:
                w1 = pltpu.bitcast(w1p[...], bf16); w2 = pltpu.bitcast(w2p[...], bf16)
            h = lax.dot_general(xnb, w1, NT_DIMS, preferred_element_type=f32) + b1_ref[...].astype(f32)[None, :]
            c1 = np.float32(np.sqrt(2 / np.pi)); c2 = np.float32(np.sqrt(2 / np.pi) * 0.044715)
            th = jnp.tanh(h * (c1 + c2 * (h * h)))
            g = (h + h * th).astype(bf16)
            o = jnp.dot(g, w2, preferred_element_type=f32)

            anchors = None
            if kvanchor:
                anchors = [g[0:16, a_:a_ + 128] if a_ >= 0 else o[0:16, (-a_ - 1) * 128:(-a_) * 128].astype(bf16) for a_ in kvanchor]
            kv_block(tn * TM + (zero * 16 if first else 0), anchors)

            if first:
                uslot = [1, 0]
            else:
                uslot = [2 * t + 1 - l if l < 4 else jnp.where(2 * t + 1 - l >= 0, 2 * t + 1 - l, Z) for l in range(nlag)]
            pend = []
            def fence(v):
                pend.append(v)
                if len(pend) >= depth:
                    UH[DUM + zero, 0, 0, :, 0:128] = pend.pop(0)
            for ci in range(NT):
                cs = slice(ci * 128, (ci + 1) * 128)
                for r2 in range(0, R8, 2):
                    ld = lambda s: [UH[s, r2:r2 + 2, c_, :, cs].reshape(16, 128) for c_ in range(3)]
                    acc1 = None; acc0 = None
                    ucur = ld(uslot[0])
                    for l in range(nlag):
                        hv = ld(H0 + l + (zero if (hdyn and not first) else 0))
                        p1 = [hv[c_] * ucur[c_] for c_ in range(3)]
                        if l + 1 < nlag:
                            ucur = ld(uslot[l + 1])
                            p0 = [hv[c_] * ucur[c_] for c_ in range(3)]
                            acc0 = p0 if acc0 is None else [x_ + y_ for x_, y_ in zip(acc0, p0)]
                        acc1 = p1 if acc1 is None else [x_ + y_ for x_, y_ in zip(acc1, p1)]
                        if depth > 0 and not first and (l + 1) % cl == 0 and l + 1 < nlag:
                            fence(acc1[2][8:16])
                    w = []
                    for j, acc in ((0, acc0), (1, acc1)):
                        w.append(pltpu.bitcast((acc[0] - acc[2]).astype(bf16), u32))
                        w.append(pltpu.bitcast((acc[0] + acc[1]).astype(bf16), u32))
                    if tie and not first:
                        s_ = (w[0] | w[1]) | (w[2] | w[3])
                        w = [jnp.where(never, s_, w_) for w_ in w]
                        if depth > 0:
                            fence(pltpu.bitcast(s_, f32))
                    for j in range(2):
                        col = slice(ci * 256 + j * 128, ci * 256 + (j + 1) * 128)
                        Q_ref[r2 * 4:r2 * 4 + 8, col] = w[2 * j]
                        Q_ref[B // 2 + r2 * 4:B // 2 + r2 * 4 + 8, col] = w[2 * j + 1]

            yy = jnp.dot(Gm_ref[...], pltpu.bitcast(Q_ref[...], bf16), preferred_element_type=f32)
            y = jnp.concatenate([jnp.concatenate([yy[:, c * 256 + j * 128: c * 256 + (j + 1) * 128] for c in range(NT)], axis=1) for j in range(2)], axis=0)

            xn = pltpu.bitcast(xn_ref[...], bf16).astype(f32)
            x = x_v[rows(t), :].astype(f32)
            out = x + xn * y + (0.5 * o + b2_ref[...].astype(f32)[None, :])
            o_v[rows(t), :] = out.astype(bf16)

        with jax.named_scope("waitw"):
            cx(0).wait(); ck(1).wait(); cv(1).wait(); cw1.wait(); cw2.wait()
        for i in range(1, NSTEP):
            cx(i).start()
            if i + 1 < NSTEP:
                ck(i + 1).start(); cv(i + 1).start()
        with jax.named_scope("step0"):
            step(0, True)
        co(0).start()

        def body(t, carry, do=True):
            cx(t).wait()
            @pl.when(t + 1 < NSTEP)
            def _():
                ck(t + 1).wait(); cv(t + 1).wait()
            if do:
                with jax.named_scope("step"):
                    step(t, False)
            co(t).start()
            return carry
        lax.fori_loop(1, loop_end, body, 0)
        if loop_end < NSTEP:
            lax.fori_loop(loop_end, NSTEP, functools.partial(body, do=False), 0)
        with jax.named_scope("waito"):
            for i in range(NSTEP):
                co(i).wait()

    Fm, Gm = dft_mats()
    @jax.jit
    def f(A_q, A_k, A_v, A_shift_k, A_ssm_k, A_ssm_D, B_x, B_w1, B_b1, B_w2, B_b2):
        anyspec = pl.BlockSpec(memory_space=pl.ANY)
        vm = pl.BlockSpec(memory_space=pltpu.VMEM)
        out = pl.pallas_call(
            kern,
            in_specs=[pl.BlockSpec(memory_space=pltpu.SMEM)] + [anyspec] * 6 + [vm] * 6,
            out_specs=anyspec,
            out_shape=jax.ShapeDtypeStruct((S, D), bf16),
            scratch_shapes=[pltpu.VMEM((2 * NB + 2, R8, 3, 8, D), f32),
                            pltpu.VMEM((S, D), bf16), pltpu.VMEM((S, D), bf16),
                            pltpu.VMEM((S + 64, D), bf16), pltpu.VMEM((S + 64, D), bf16),
                            pltpu.VMEM((D, S), bf16), pltpu.VMEM((F, D), bf16), pltpu.VMEM((F, D), bf16),
                            pltpu.VMEM((F // 2, D), u32), pltpu.VMEM((F // 2, D), u32),
                            pltpu.VMEM((TM // 2, D), u32), pltpu.VMEM((B, 2 * D), u32), pltpu.VMEM((TM // 2, D), u32),
                            pltpu.SemaphoreType.DMA((NSTEP,)), pltpu.SemaphoreType.DMA((NSTEP,)), pltpu.SemaphoreType.DMA((NSTEP,)),
                            pltpu.SemaphoreType.DMA((NT,)), pltpu.SemaphoreType.DMA((2,)), pltpu.SemaphoreType.DMA((NSTEP,))],
            compiler_params=pltpu.CompilerParams(vmem_limit_bytes=110 * 1024 * 1024),
        )(jnp.zeros((1,), jnp.int32), A_q.reshape(S, D), A_k.reshape(S, D), A_v.reshape(S, D), A_ssm_k, B_w1.T, B_w2,
          A_shift_k.T, A_ssm_D, B_b1, B_b2, jnp.asarray(Fm, bf16), jnp.asarray(Gm, bf16))
        return out.reshape(1, S, D)
    return f


_impl = make(depth=0, kvanchor=None, hdyn=False)


@jax.jit
def pallas_parallel_sum__ssm_conv_h3__dense_activation_gelu__prompt_kernel(
    A_q, A_k, A_v, A_shift_k, A_ssm_k, A_ssm_D, B_x, B_w1, B_b1, B_w2, B_b2
):
    return _impl(A_q, A_k, A_v, A_shift_k, A_ssm_k, A_ssm_D, B_x, B_w1, B_b1, B_w2, B_b2)
```

```python
import functools
import jax, jax.numpy as jnp, numpy as np
from jax import lax
from jax.experimental import pallas as pl
from jax.experimental.pallas import tpu as pltpu

S, D, F = 2048, 640, 1728
B = 128
NB = S // B
TM = 256
NSTEP = S // TM
NT = D // 128
R8 = B // 8
Z = NB
H0 = NB + 1
KO = 16
VO = 16 + S
FO = 16 + 2 * S
KVR = 2 * S + 64
f32 = jnp.float32
bf16 = jnp.bfloat16
u32 = jnp.uint32
NT_DIMS = (((1,), (1,)), ((), ()))

def dft_mats(fold):
    k = np.concatenate([np.arange(0, B, 2), np.arange(1, B, 2)]).astype(np.float64) + 0.5
    n = np.arange(B, dtype=np.float64)
    th = 2 * np.pi * np.outer(k, n) / (2 * B)
    Fu = np.concatenate([np.cos(th), -np.sin(th)], 0)
    if not fold:
        Fh = Fu
        Gm = np.concatenate([np.cos(th).T, -np.sin(th).T], 1) / B
    else:
        c = (B - 1) / 2
        ph = 2 * np.pi * np.outer(k, n - c) / (2 * B)
        Fh = np.concatenate([np.cos(ph), -np.sin(ph)], 0)
        Gm = np.concatenate([np.cos(ph).T[:B // 2], np.sin(ph).T[:B // 2]], 0) / B
    return Fu.astype(np.float32), Fh.astype(np.float32), Gm.astype(np.float32)

def pk(x):
    return pltpu.bitcast(x, u32)

def upk(x):
    return pltpu.bitcast(x, bf16)

def make(kvanchor='h', kvt=(2, 12), kvrows=32, kvfence=True, fold=True, idft_pos=5, order=True, w1b=(0, 768, 1728), w2b=(0, 1024, 1728)):
    def kern(z_ref, x_hbm, k_hbm, v_hbm, h_hbm, w1_hbm, w2_hbm, sk_hbm, sD_hbm, b1_hbm, b2_hbm, C_hbm,
             o_hbm,
             UH, x_v, o_v, KV, h_v, w1_v, w2_v, w1p, w2p, kvb_ref, Q_ref, xn_ref,
             sk_ref, sD_ref, b1_ref, b2_ref, C_ref,
             sem_t, sem_0, sem_h, sem_w1, sem_w2, sem_o, sem_b):
        Fu_ref = C_ref.at[0:2 * B]; Fh_ref = C_ref.at[2 * B:4 * B]; Gm_ref = C_ref.at[4 * B:5 * B]
        def rows(i):
            return pl.ds(pl.multiple_of(i * TM, TM), TM)
        cx = lambda i: pltpu.make_async_copy(x_hbm.at[rows(i)], x_v.at[rows(i)], sem_0.at[1] if (isinstance(i, int) and i == 0) else sem_t.at[i])
        ck = lambda i: pltpu.make_async_copy(k_hbm.at[rows(i)], KV.at[pl.ds(pl.multiple_of(KO + i * TM, 16), TM)], sem_0.at[i] if (isinstance(i, int) and i == 0) else sem_0.at[2] if (isinstance(i, int) and i == 1) else sem_t.at[i - 1])
        cv = lambda i: pltpu.make_async_copy(v_hbm.at[rows(i)], KV.at[pl.ds(pl.multiple_of(VO + i * TM, 16), TM)], sem_0.at[i] if (isinstance(i, int) and i == 0) else sem_0.at[2] if (isinstance(i, int) and i == 1) else sem_t.at[i - 1])
        ch = lambda c: pltpu.make_async_copy(h_hbm.at[pl.ds(c * 128, 128)], h_v.at[pl.ds(c * 128, 128)], sem_h.at[c])
        co = lambda i: pltpu.make_async_copy(o_v.at[rows(i)], o_hbm.at[rows(i)], sem_o)
        def chunks(bounds):
            return [(bounds[i], bounds[i + 1]) for i in range(len(bounds) - 1)]
        W1C = chunks(w1b); W2C = chunks(w2b)
        cw1 = lambda i: pltpu.make_async_copy(w1_hbm.at[W1C[i][0]:W1C[i][1]], w1_v.at[W1C[i][0]:W1C[i][1]], sem_w1.at[i])
        cw2 = lambda i: pltpu.make_async_copy(w2_hbm.at[W2C[i][0]:W2C[i][1]], w2_v.at[W2C[i][0]:W2C[i][1]], sem_w2.at[i])
        small = [(C_hbm, C_ref), (sD_hbm, sD_ref), (sk_hbm, sk_ref), (b1_hbm, b1_ref), (b2_hbm, b2_ref)]
        cs_ = lambda i: pltpu.make_async_copy(small[i][0], small[i][1], [sem_h.at[0], sem_h.at[0], sem_0.at[0], sem_0.at[1], sem_0.at[1]][i])

        def start_in_order(copies):
            for cp in copies:
                cp.start()
                if order:
                    pl.semaphore_signal(sem_b, 1)
                    pl.semaphore_wait(sem_b, 1)

        start_in_order([cs_(0), cs_(1), ch(0), ch(1), ch(2), cs_(2), ck(0), cv(0), ch(3), cx(0), ch(4), cs_(3), cs_(4)]
                       + [cw1(i) for i in range(len(W1C))] + [cw2(i) for i in range(len(W2C))]
                       + [ck(1), cv(1), cx(1)])
        for i_ in range(2, NSTEP):
            ck(i_).start(); cv(i_).start(); cx(i_).start()
            if i_ % 2 == 0:
                pl.semaphore_signal(sem_b, 1)
                pl.semaphore_wait(sem_b, 1)

        zero = z_ref[0]
        never = jnp.full((8, 128), zero, jnp.int32) != 0
        KV[0:16, :] = jnp.zeros((16, D), bf16)

        def kv_block(base, anchors=None):
            sk = sk_ref[...].astype(f32)
            nrc = TM // kvrows
            fr = pl.ds(pl.multiple_of(FO + zero * 64, 16), 8)
            for c in range(NT):
                cs = slice(c * 128, (c + 1) * 128)
                for rc in range(nrc):
                    if anchors is not None:
                        KV[fr, 0:128] = anchors[c * nrc + rc].astype(bf16)
                    r0 = pl.multiple_of(base + rc * kvrows, 16)
                    kext = KV[pl.ds(r0, kvrows + 16), cs].astype(f32)[8:]
                    vv = KV[pl.ds(pl.multiple_of(r0 + VO, 16), kvrows), cs].astype(f32)
                    ks = kext[8:] * sk[0:1, cs]
                    for j in range(1, 4):
                        ks = ks + pltpu.roll(kext, j, 0)[8:, :] * sk[j:j + 1, cs]
                    kv = (ks * vv).astype(bf16)
                    kvb_ref[rc * kvrows // 2:(rc + 1) * kvrows // 2, cs] = pk(kv)

        UH[Z] = jnp.zeros(UH.shape[1:], f32)
        hb = B // 2
        anchor0 = []
        for c in range(NT):
            with jax.named_scope("waith"):
                if c == 0:
                    cs_(0).wait(); cs_(1).wait()
                if c == 3:
                    cs_(2).wait(); ck(0).wait(); cv(0).wait()
                if c == 4:
                    cx(0).wait(); cs_(3).wait(); cs_(4).wait()
                ch(c).wait()
            Fh = Fh_ref[...]
            cs = slice(c * 128, (c + 1) * 128)
            hp_re = hp_im = None
            for a in range(NB):
                hh = lax.dot_general(Fh, h_v[cs, a * B:(a + 1) * B], NT_DIMS, preferred_element_type=f32)
                if a == 0:
                    hh = hh + Fh[:, 0:1].astype(f32) * sD_ref[...].astype(f32)[None, cs]
                hre = hh[:B]; him = hh[B:]
                if a == 0:
                    c_, d_ = hre, him
                else:
                    c_ = jnp.concatenate([hre[:hb] - hp_im[:hb], hre[hb:] + hp_im[hb:]], axis=0)
                    d_ = jnp.concatenate([him[:hb] + hp_re[:hb], him[hb:] - hp_re[hb:]], axis=0)
                UH[H0 + a, :, 0, :, cs] = c_.reshape(R8, 8, 128)
                UH[H0 + a, :, 1, :, cs] = (d_ - c_).reshape(R8, 8, 128)
                UH[H0 + a, :, 2, :, cs] = (c_ + d_).reshape(R8, 8, 128)
                hp_re, hp_im = hre, him
                if c == 3:
                    anchor0.extend([hre[0:8], hre[64:72], him[0:8]])
            if c == 3:
                nch = NT * TM // kvrows
                kv_block(zero * 64, [anchor0[3 + (i * 42) // nch] for i in range(nch)])

        def step(t, first):
            nlag = 2 if first else NB
            tn = jnp.minimum(t + 1, NSTEP - 1) if not first else 1
            Fu = Fu_ref[...]
            for j in range(2):
                kvb = upk(kvb_ref[j * (B // 2):(j + 1) * (B // 2), :])
                u = jnp.dot(Fu, kvb, preferred_element_type=f32)
                a = u[:B]; b = u[B:]
                UH[2 * t + j, :, 0] = (a + b).reshape(R8, 8, D)
                UH[2 * t + j, :, 1] = a.reshape(R8, 8, D)
                UH[2 * t + j, :, 2] = b.reshape(R8, 8, D)

            x = x_v[rows(t), :].astype(f32)
            m = jnp.mean(x, axis=-1, keepdims=True)
            xc = x - m
            var = jnp.mean(xc * xc, axis=-1, keepdims=True)
            xn = xc * lax.rsqrt(var + 1e-5)
            xn_ref[...] = pk(xn.astype(bf16))

            c1 = np.float32(np.sqrt(2 / np.pi)); c2 = np.float32(np.sqrt(2 / np.pi) * 0.044715)
            b1 = b1_ref[...].astype(f32)[None, :]
            def mlp1(w1, lo, hi):
                h = lax.dot_general(upk(xn_ref[...]), w1, NT_DIMS, preferred_element_type=f32) + b1[:, lo:hi]
                th = jnp.tanh(h * (c1 + c2 * (h * h)))
                return h, (h + h * th).astype(bf16)
            if first:
                gs = []
                for i, (lo, hi) in enumerate(W1C):
                    with jax.named_scope("waitw1"):
                        cw1(i).wait()
                    w1 = w1_v[lo:hi, :]
                    w1p[lo // 2:hi // 2, :] = pk(w1)
                    gs.append(mlp1(w1, lo, hi)[1])
                g = jnp.concatenate(gs, axis=1)
                o_a = None
                for i, (lo, hi) in enumerate(W2C):
                    with jax.named_scope("waitw2"):
                        cw2(i).wait()
                        if i == len(W2C) - 1:
                            ck(1).wait(); cv(1).wait()
                    w2 = w2_v[lo:hi, :]
                    w2p[lo // 2:hi // 2, :] = pk(w2)
                    p_ = jnp.dot(g[:, lo:hi], w2, preferred_element_type=f32)
                    o_a = p_ if o_a is None else p_ + o_a
            else:
                w2 = upk(w2p[...])
                h, g = mlp1(upk(w1p[...]), 0, F)
                o_a = jnp.dot(g, w2[:, :idft_pos * 128], preferred_element_type=f32)

            anchor = None
            nch = NT * TM // kvrows
            if first:
                pts = [(i * 64) // nch for i in range(nch)]
                anchor = [o_a[(p % 16) * 16:(p % 16) * 16 + 8, (p // 16) * 128:(p // 16 + 1) * 128] for p in pts]
            elif kvanchor == 'h':
                t0_, t1_ = kvt
                pts = [(t0_ * 16 + (i * (t1_ - t0_) * 16) // nch) for i in range(nch)]
                anchor = [h[(p % 16) * 16:(p % 16) * 16 + 8, (p // 16) * 128:(p // 16 + 1) * 128] for p in pts]
            elif kvanchor == 'o':
                t0_, t1_ = kvt
                pts = [(t0_ * 16 + (i * (t1_ - t0_) * 16) // nch) for i in range(nch)]
                anchor = [o_a[(p % 16) * 16:(p % 16) * 16 + 8, (p // 16) * 128:(p // 16 + 1) * 128] for p in pts]
            kv_block(tn * TM + (zero * 64 if first else 0), anchor)

            if first:
                uslot = [1, 0]
            else:
                uslot = [2 * t + 1 - l if l < 4 else jnp.where(2 * t + 1 - l >= 0, 2 * t + 1 - l, Z) for l in range(nlag)]
            for ci in range(NT):
                cs = slice(ci * 128, (ci + 1) * 128)
                for r2 in range(0, R8, 2):
                    ld = lambda s: [UH[s, r2:r2 + 2, c_, :, cs].reshape(16, 128) for c_ in range(3)]
                    acc1 = None; acc0 = None
                    ucur = ld(uslot[0])
                    for l in range(nlag):
                        hv = ld(H0 + l)
                        p1 = [hv[c_] * ucur[c_] for c_ in range(3)]
                        if l + 1 < nlag:
                            ucur = ld(uslot[l + 1])
                            p0 = [hv[c_] * ucur[c_] for c_ in range(3)]
                            acc0 = p0 if acc0 is None else [x_ + y_ for x_, y_ in zip(acc0, p0)]
                        acc1 = p1 if acc1 is None else [x_ + y_ for x_, y_ in zip(acc1, p1)]
                    w = []
                    for j, acc in ((0, acc0), (1, acc1)):
                        w.append(pk((acc[0] - acc[2]).astype(bf16)))
                        w.append(pk((acc[0] + acc[1]).astype(bf16)))
                    if not first:
                        s_ = (w[0] | w[1]) | (w[2] | w[3])
                        w = [jnp.where(never, s_, w_) for w_ in w]
                    for j in range(2):
                        col = slice(ci * 256 + j * 128, ci * 256 + (j + 1) * 128)
                        Q_ref[r2 * 4:r2 * 4 + 8, col] = w[2 * j]
                        Q_ref[B // 2 + r2 * 4:B // 2 + r2 * 4 + 8, col] = w[2 * j + 1]

            if not fold:
                yy = jnp.dot(Gm_ref[...], upk(Q_ref[...]), preferred_element_type=f32)
            else:
                idx = 7 - lax.broadcasted_iota(jnp.int32, (8, 128), 0)
                cols = []
                for c in range(NT):
                    qs = slice(c * 256, (c + 1) * 256)
                    cc = jnp.dot(Gm_ref[0:hb, :], upk(Q_ref[0:hb, qs]), preferred_element_type=f32)
                    ss = jnp.dot(Gm_ref[hb:, :], upk(Q_ref[hb:, qs]), preferred_element_type=f32)
                    lo = cc - ss
                    hi = cc + ss
                    hi = jnp.concatenate(
                        [jnp.concatenate([jnp.take_along_axis(hi[r * 8:(r + 1) * 8, j * 128:(j + 1) * 128], idx, axis=0) for j in range(2)], axis=1)
                         for r in reversed(range(hb // 8))], axis=0)
                    cols.append(jnp.concatenate([lo, hi], axis=0))
                yy = jnp.concatenate(cols, axis=1)
            y = jnp.concatenate([jnp.concatenate([yy[:, c * 256 + j * 128: c * 256 + (j + 1) * 128] for c in range(NT)], axis=1) for j in range(2)], axis=0)
            if idft_pos < NT and not first:
                o_b = jnp.dot(g, w2[:, idft_pos * 128:], preferred_element_type=f32)
                o = jnp.concatenate([o_a, o_b], axis=1)
            else:
                o = o_a

            xn = upk(xn_ref[...]).astype(f32)
            x = x_v[rows(t), :].astype(f32)
            out = (x + b2_ref[...].astype(f32)[None, :] + xn * y) + 0.5 * o
            o_v[rows(t), :] = out.astype(bf16)

        step(0, True)
        co(0).start()

        def body(t, carry):
            cx(t).wait()
            @pl.when(t + 1 < NSTEP)
            def _():
                ck(t + 1).wait(); cv(t + 1).wait()
            with jax.named_scope("step"):
                step(t, False)
            co(t).start()
            return carry
        lax.fori_loop(1, NSTEP, body, 0)
        with jax.named_scope("waito"):
            for i in range(NSTEP):
                co(i).wait()

    Fu, Fh, Gm = dft_mats(fold)
    @jax.jit
    def f(A_q, A_k, A_v, A_shift_k, A_ssm_k, A_ssm_D, B_x, B_w1, B_b1, B_w2, B_b2):
        anyspec = pl.BlockSpec(memory_space=pl.ANY)
        vm = pl.BlockSpec(memory_space=pltpu.VMEM)
        out = pl.pallas_call(
            kern,
            in_specs=[pl.BlockSpec(memory_space=pltpu.SMEM)] + [anyspec] * 11,
            out_specs=anyspec,
            out_shape=jax.ShapeDtypeStruct((S, D), bf16),
            scratch_shapes=[pltpu.VMEM((2 * NB + 1, R8, 3, 8, D), f32),
                            pltpu.VMEM((S, D), bf16), pltpu.VMEM((S, D), bf16),
                            pltpu.VMEM((KVR, D), bf16),
                            pltpu.VMEM((D, S), bf16), pltpu.VMEM((F, D), bf16), pltpu.VMEM((F, D), bf16),
                            pltpu.VMEM((F // 2, D), u32), pltpu.VMEM((F // 2, D), u32),
                            pltpu.VMEM((TM // 2, D), u32), pltpu.VMEM((B, 2 * D), u32), pltpu.VMEM((TM // 2, D), u32),
                            pltpu.VMEM((4, D), bf16), pltpu.VMEM((D,), bf16), pltpu.VMEM((F,), bf16), pltpu.VMEM((D,), bf16),
                            pltpu.VMEM((5 * B, B), bf16),
                            pltpu.SemaphoreType.DMA((NSTEP,)), pltpu.SemaphoreType.DMA((3,)),
                            pltpu.SemaphoreType.DMA((NT,)), pltpu.SemaphoreType.DMA((len(w1b) - 1,)), pltpu.SemaphoreType.DMA((len(w2b) - 1,)),
                            pltpu.SemaphoreType.DMA(()), pltpu.SemaphoreType.REGULAR],
            compiler_params=pltpu.CompilerParams(vmem_limit_bytes=110 * 1024 * 1024),
        )(jnp.zeros((1,), jnp.int32), A_q.reshape(S, D), A_k.reshape(S, D), A_v.reshape(S, D), A_ssm_k, B_w1.T, B_w2,
          A_shift_k.T, A_ssm_D, B_b1, B_b2, jnp.asarray(np.concatenate([Fu, Fh, Gm], 0), bf16))
        return out.reshape(1, S, D)
    return f


_impl = make()


@jax.jit
def pallas_parallel_sum__ssm_conv_h3__dense_activation_gelu__prompt_kernel(
    A_q, A_k, A_v, A_shift_k, A_ssm_k, A_ssm_D, B_x, B_w1, B_b1, B_w2, B_b2
):
    return _impl(A_q, A_k, A_v, A_shift_k, A_ssm_k, A_ssm_D, B_x, B_w1, B_b1, B_w2, B_b2)
```

```python
import functools
import jax, jax.numpy as jnp, numpy as np
from jax import lax
from jax.experimental import pallas as pl
from jax.experimental.pallas import tpu as pltpu

S, D, F = 2048, 640, 1728
B = 128
NB = S // B
TM = 256
NSTEP = S // TM
NT = D // 128
R8 = B // 8
HB = B // 2
Z = NB
DUM = NB + 1
H0 = NB + 2
KO = 16
VO = 16 + S
FO = 16 + 2 * S
KVR = 2 * S + 64
FM = 1664
f32 = jnp.float32
bf16 = jnp.bfloat16
u32 = jnp.uint32
NT_DIMS = (((1,), (1,)), ((), ()))
TN_DIMS = (((0,), (0,)), ((), ()))

def dft_mats():
    k = np.concatenate([np.arange(0, B, 2), np.arange(1, B, 2)]).astype(np.float64) + 0.5
    n = np.arange(B, dtype=np.float64)
    th = 2 * np.pi * np.outer(k, n) / (2 * B)
    Fu = np.concatenate([np.cos(th), -np.sin(th)], 0)
    c = (B - 1) / 2
    ph = 2 * np.pi * np.outer(k, n - c) / (2 * B)
    Fh = np.concatenate([np.cos(ph), -np.sin(ph)], 0)
    Gm = np.concatenate([np.cos(ph).T[:HB], np.sin(ph).T[:HB]], 0) / B
    return np.concatenate([Fh, Fu, Gm], 0).astype(np.float32)

def pk(x):
    return pltpu.bitcast(x, u32)

def upk(x):
    return pltpu.bitcast(x, bf16)

def make(kvrows=32, kvanchor='h', kvt=(2, 12), w1b=(0, 768, 1728), w2b=(0, 1024, 1728), nobc=True, rem=False, kvscr=True, mat=0, lnt=(1, 3), lnn=16):
    def kern(z_ref, x_hbm, k_hbm, v_hbm, h_hbm, w1_hbm, w2_hbm, sk_hbm, sD_hbm, b1_hbm, b2_hbm, C_hbm,
             o_hbm,
             UH, x_v, o_v, KV, h_v, w1_v, w2_v, w1p, w2p, kvb_ref, Q_ref, xn_ref, xb_ref, skb_ref, b1c_ref,
             sk_ref, sD_ref, b1_ref, b2_ref, C_ref,
             sem_t, sem_0, sem_h, sem_w1, sem_w2, sem_o, sem_b):
        Fh_ref = C_ref.at[0:2 * B]; Fu_ref = C_ref.at[2 * B:4 * B]; Gm_ref = C_ref.at[4 * B:5 * B]
        def rows(i):
            return pl.ds(pl.multiple_of(i * TM, TM), TM)
        st = lambda i: isinstance(i, int)
        cx = lambda i: pltpu.make_async_copy(x_hbm.at[rows(i)], x_v.at[rows(i)], sem_0.at[1] if (st(i) and i == 0) else sem_t.at[i])
        ck = lambda i: pltpu.make_async_copy(k_hbm.at[rows(i)], KV.at[pl.ds(pl.multiple_of(KO + i * TM, 16), TM)], sem_0.at[0] if (st(i) and i == 0) else sem_t.at[i])
        cv = lambda i: pltpu.make_async_copy(v_hbm.at[rows(i)], KV.at[pl.ds(pl.multiple_of(VO + i * TM, 16), TM)], sem_0.at[0] if (st(i) and i == 0) else sem_t.at[i])
        ch = lambda c: pltpu.make_async_copy(h_hbm.at[pl.ds(c * 128, 128)], h_v.at[pl.ds(c * 128, 128)], sem_h.at[c])
        co = lambda i: pltpu.make_async_copy(o_v.at[rows(i)], o_hbm.at[rows(i)], sem_o)
        def chunks(bounds):
            return [(bounds[i], bounds[i + 1]) for i in range(len(bounds) - 1)]
        W1C = chunks(w1b); W2C = chunks(w2b)
        cw1 = lambda i: pltpu.make_async_copy(w1_hbm.at[W1C[i][0]:W1C[i][1]], w1_v.at[W1C[i][0]:W1C[i][1]], sem_w1.at[i])
        cw2 = lambda i: pltpu.make_async_copy(w2_hbm.at[W2C[i][0]:W2C[i][1]], w2_v.at[W2C[i][0]:W2C[i][1]], sem_w2.at[i])
        small = [(C_hbm, C_ref, sem_h.at[0]), (sD_hbm, sD_ref, sem_h.at[0]), (sk_hbm, sk_ref, sem_0.at[0]),
                 (b1_hbm, b1_ref, sem_0.at[1]), (b2_hbm, b2_ref, sem_0.at[1])]
        cs_ = lambda i: pltpu.make_async_copy(*small[i])

        def bar():
            pl.semaphore_signal(sem_b, 1)
            pl.semaphore_wait(sem_b, 1)

        for cp in ([cs_(0), cs_(1), ch(0), ch(1), ch(2), cs_(2), ck(0), cv(0), ch(3), cx(0), ch(4), cs_(3), cs_(4)]
                   + [cw1(i) for i in range(len(W1C))] + [cw2(i) for i in range(len(W2C))]):
            cp.start(); bar()
        for i_ in range(1, NSTEP):
            ck(i_).start(); cv(i_).start(); cx(i_).start()
            if i_ in (1, 2, 4):
                bar()

        zero = z_ref[0]
        never = jnp.full((8, 128), zero, jnp.int32) != 0
        KV[0:16, :] = jnp.zeros((16, D), bf16)
        nch = NT * TM // kvrows

        def kv_block(base, anchors=None):
            nrc = TM // kvrows
            fr = pl.ds(pl.multiple_of(FO + zero * 64, 16), 8)
            cols = []
            for c in range(NT):
                cs = slice(c * 128, (c + 1) * 128)
                col = []
                if anchors is not None:
                    skb_ref[pl.ds(pl.multiple_of(32 + zero * 8, 8), 8), 0:128] = anchors[c * nrc]
                sk = [jnp.concatenate([skb_ref[8 * j:8 * j + 8, cs]] * (kvrows // 8), axis=0) for j in range(4)]
                for rc in range(nrc):
                    if anchors is not None:
                        KV[fr, 0:128] = anchors[c * nrc + rc].astype(bf16)
                    r0 = pl.multiple_of(base + rc * kvrows, 16)
                    kext = KV[pl.ds(r0, kvrows + 16), cs].astype(f32)[8:]
                    vv = KV[pl.ds(pl.multiple_of(r0 + VO, 16), kvrows), cs].astype(f32)
                    ks = kext[8:] * sk[0]
                    for j in range(1, 4):
                        ks = ks + pltpu.roll(kext, j, 0)[8:, :] * sk[j]
                    kv = (ks * vv).astype(bf16)
                    if kvscr:
                        kvb_ref[rc * kvrows // 2:(rc + 1) * kvrows // 2, cs] = pk(kv)
                    col.append(kv)
                cols.append(jnp.concatenate(col, axis=0))
            return jnp.concatenate(cols, axis=1)

        def u_dft(t, kvb=None):
            Fu = Fu_ref[...]
            for j in range(2):
                kj = upk(kvb_ref[j * HB:(j + 1) * HB, :]) if (kvb is None or kvscr) else kvb[j * B:(j + 1) * B]
                u = jnp.dot(Fu, kj, preferred_element_type=f32)
                a = u[:B]; b = u[B:]
                UH[2 * t + j, :, 0] = (a + b).reshape(R8, 8, D)
                UH[2 * t + j, :, 1] = a.reshape(R8, 8, D)
                UH[2 * t + j, :, 2] = b.reshape(R8, 8, D)

        def layernorm(t, anchors=None):
            outs = []
            n = len(anchors) if anchors is not None else 1
            rr = TM // n
            for i in range(n):
                if anchors is not None:
                    x_v[pl.ds(pl.multiple_of(S + zero * 64, 16), 8), 0:128] = anchors[i].astype(bf16)
                x = x_v[pl.ds(pl.multiple_of(t * TM + i * rr, 16), rr), :].astype(f32)
                m = jnp.mean(x, axis=-1, keepdims=True)
                xc = x - m
                var = jnp.mean(xc * xc, axis=-1, keepdims=True)
                xn = xc * lax.rsqrt(var + 1e-5)
                xn_ref[i * rr // 2:(i + 1) * rr // 2, :] = pk(xn.astype(bf16))

        c1 = np.float32(np.sqrt(2 / np.pi)); c2 = np.float32(np.sqrt(2 / np.pi) * 0.044715)
        def gelu2(h):
            return (h + h * jnp.tanh(h * (c1 + c2 * (h * h)))).astype(bf16)

        def mlp1(w1, lo, hi):
            b1 = b1_ref[...].astype(f32)[None, :]
            h = lax.dot_general(upk(xn_ref[...]), w1, NT_DIMS, preferred_element_type=f32) + b1[:, lo:hi]
            return h, gelu2(h)

        def pts_anchor(val, t0_, t1_, n=nch):
            pts = [(t0_ * 16 + (i * (t1_ - t0_) * 16) // n) for i in range(n)]
            return [val[(p % 16) * 16:(p % 16) * 16 + 8, (p // 16) * 128:(p // 16 + 1) * 128] for p in pts]

        def mac(t, anchor=None):
            if anchor is not None:
                UH[DUM + zero, 0, 0, :, 0:128] = anchor
            if st(t):
                nlag = 2 * t + 2
                uslot = [2 * t + 1 - l for l in range(nlag)]
            else:
                nlag = NB
                uslot = [2 * t + 1 - l if l < 4 else jnp.where(2 * t + 1 - l >= 0, 2 * t + 1 - l, Z) for l in range(nlag)]
            for ci in range(NT):
                cs = slice(ci * 128, (ci + 1) * 128)
                for r2 in range(0, R8, 2):
                    ld = lambda s: [UH[s, r2:r2 + 2, c_, :, cs].reshape(16, 128) for c_ in range(3)]
                    acc1 = None; acc0 = None
                    ucur = ld(uslot[0])
                    for l in range(nlag):
                        hv = ld(H0 + l)
                        p1 = [hv[c_] * ucur[c_] for c_ in range(3)]
                        if l + 1 < nlag:
                            ucur = ld(uslot[l + 1])
                            p0 = [hv[c_] * ucur[c_] for c_ in range(3)]
                            acc0 = p0 if acc0 is None else [x_ + y_ for x_, y_ in zip(acc0, p0)]
                        acc1 = p1 if acc1 is None else [x_ + y_ for x_, y_ in zip(acc1, p1)]
                    w = []
                    for j, acc in ((0, acc0), (1, acc1)):
                        w.append(pk((acc[0] - acc[2]).astype(bf16)))
                        w.append(pk((acc[0] + acc[1]).astype(bf16)))
                    if nlag > 2:
                        s_ = (w[0] | w[1]) | (w[2] | w[3])
                        w = [jnp.where(never, s_, w_) for w_ in w]
                    for j in range(2):
                        col = slice(ci * 256 + j * 128, ci * 256 + (j + 1) * 128)
                        Q_ref[r2 * 4:r2 * 4 + 8, col] = w[2 * j]
                        Q_ref[HB + r2 * 4:HB + r2 * 4 + 8, col] = w[2 * j + 1]

        def finish(t, o):
            idx = 7 - lax.broadcasted_iota(jnp.int32, (8, 128), 0)
            cols = []
            for c in range(NT):
                qs = slice(c * 256, (c + 1) * 256)
                cc = jnp.dot(Gm_ref[0:HB, :], upk(Q_ref[0:HB, qs]), preferred_element_type=f32)
                ss = jnp.dot(Gm_ref[HB:, :], upk(Q_ref[HB:, qs]), preferred_element_type=f32)
                lo = cc - ss
                hi = cc + ss
                hi = jnp.concatenate(
                    [jnp.concatenate([jnp.take_along_axis(hi[r * 8:(r + 1) * 8, j * 128:(j + 1) * 128], idx, axis=0) for j in range(2)], axis=1)
                     for r in reversed(range(HB // 8))], axis=0)
                cols.append(jnp.concatenate([lo, hi], axis=0))
            yy = jnp.concatenate(cols, axis=1)
            y = jnp.concatenate([jnp.concatenate([yy[:, c * 256 + j * 128: c * 256 + (j + 1) * 128] for c in range(NT)], axis=1) for j in range(2)], axis=0)
            xn = upk(xb_ref[...]).astype(f32)
            x = x_v[rows(t), :].astype(f32)
            out = (xn * y + o) + x
            o_v[rows(t), :] = out.astype(bf16)

        def mlp_full():
            if not rem:
                h, g = mlp1(upk(w1p[...]), 0, F)
                o = jnp.dot(g, upk(w2p[...]), preferred_element_type=f32) + b2_ref[...].astype(f32)[None, :]
            else:
                h, g = mlp1(upk(w1p[0:FM // 2, :]), 0, FM)
                ht = lax.dot_general(upk(w1p[FM // 2:, :]), upk(xn_ref[...]), NT_DIMS, preferred_element_type=f32)
                bc = b1c_ref[...]
                gt = gelu2(ht + jnp.concatenate([bc, bc], axis=1))
                g = jnp.concatenate([g, gt.T], axis=1)
                o = jnp.dot(g, upk(w2p[...]), preferred_element_type=f32) + b2_ref[...].astype(f32)[None, :]
            return h, o

        UH[Z] = jnp.zeros(UH.shape[1:], f32)
        anchor0 = []
        for c in range(NT):
            with jax.named_scope("waith"):
                if c == 0:
                    cs_(0).wait(); cs_(1).wait()
                if c == 3:
                    cs_(2).wait(); ck(0).wait(); cv(0).wait()
                if c == 4:
                    cx(0).wait(); cs_(3).wait(); cs_(4).wait()
                ch(c).wait()
            if c == 3:
                skf = sk_ref[...].astype(f32)
                for j in range(4):
                    skb_ref[8 * j:8 * j + 8, :] = jnp.broadcast_to(skf[j:j + 1, :], (8, D))
            Fh = Fh_ref[...]
            cs = slice(c * 128, (c + 1) * 128)
            hp_re = hp_im = None
            for a in range(NB):
                hh = lax.dot_general(Fh, h_v[cs, a * B:(a + 1) * B], NT_DIMS, preferred_element_type=f32)
                if a == 0:
                    hh = hh + Fh[:, 0:1].astype(f32) * sD_ref[...].astype(f32)[None, cs]
                hre = hh[:B]; him = hh[B:]
                if a == 0:
                    c_, d_ = hre, him
                else:
                    c_ = jnp.concatenate([hre[:HB] - hp_im[:HB], hre[HB:] + hp_im[HB:]], axis=0)
                    d_ = jnp.concatenate([him[:HB] + hp_re[:HB], him[HB:] - hp_re[HB:]], axis=0)
                UH[H0 + a, :, 0, :, cs] = c_.reshape(R8, 8, 128)
                UH[H0 + a, :, 1, :, cs] = (d_ - c_).reshape(R8, 8, 128)
                UH[H0 + a, :, 2, :, cs] = (c_ + d_).reshape(R8, 8, 128)
                hp_re, hp_im = hre, him
                if c == 3:
                    anchor0.extend([hre[0:8], hre[64:72], him[0:8]])
            if c == 3:
                kvb0 = kv_block(zero * 64, [anchor0[3 + (i * 42) // nch] for i in range(nch)])
        u_dft(0, kvb0)
        layernorm(0)
        xb_ref[...] = xn_ref[...]
        if rem:
            b1t = jnp.broadcast_to(b1_ref[...].astype(f32)[None, F - 128:], (128, 128)).T
            b1c_ref[...] = b1t[64:]
        gs = []
        for i, (lo, hi) in enumerate(W1C):
            with jax.named_scope("waitw1"):
                cw1(i).wait()
            w1 = w1_v[lo:hi, :]
            w1p[lo // 2:hi // 2, :] = pk(w1)
            gs.append(mlp1(w1, lo, hi)[1])
        g = jnp.concatenate(gs, axis=1)
        o = None
        for i, (lo, hi) in enumerate(W2C):
            with jax.named_scope("waitw2"):
                cw2(i).wait()
                if i == len(W2C) - 1:
                    ck(1).wait(); cv(1).wait(); cx(1).wait()
            w2 = (w2_v[lo:hi, :].astype(f32) * 0.5).astype(bf16)
            w2p[lo // 2:hi // 2, :] = pk(w2)
            p_ = jnp.dot(g[:, lo:hi], w2, preferred_element_type=f32)
            o = p_ + (b2_ref[...].astype(f32)[None, :] if o is None else o)
            if i == 0:
                mac(0, p_[0:8, 0:128])
        kvb = kv_block(TM + zero * 64, pts_anchor(o, 0, 4))
        layernorm(1, pts_anchor(o, 0, 3, n=16))
        finish(0, o)

        co(0).start()

        def body(t, carry):
            tn = jnp.minimum(t + 1, NSTEP - 1)
            @pl.when(t + 1 < NSTEP)
            def _():
                ck(t + 1).wait(); cv(t + 1).wait(); cx(t + 1).wait()
            with jax.named_scope("step"):
                u_dft(t)
                xb_ref[...] = xn_ref[...]
                h, o = mlp_full()
                anchor = None
                if kvanchor == 'h':
                    anchor = pts_anchor(h, *kvt)
                elif kvanchor == 'o':
                    anchor = pts_anchor(o, *kvt)
                kv_block(tn * TM, anchor)
                mac(t)
                layernorm(tn, pts_anchor(o, *lnt, n=lnn) if lnn else None)
                finish(t, o)
            co(t).start()
            return carry
        lax.fori_loop(1, NSTEP, body, 0)
        with jax.named_scope("waito"):
            for i in range(NSTEP):
                co(i).wait()

    C = dft_mats()
    @jax.jit
    def f(A_q, A_k, A_v, A_shift_k, A_ssm_k, A_ssm_D, B_x, B_w1, B_b1, B_w2, B_b2):
        anyspec = pl.BlockSpec(memory_space=pl.ANY)
        out = pl.pallas_call(
            kern,
            in_specs=[pl.BlockSpec(memory_space=pltpu.SMEM)] + [anyspec] * 11,
            out_specs=anyspec,
            out_shape=jax.ShapeDtypeStruct((S, D), bf16),
            scratch_shapes=[pltpu.VMEM((2 * NB + 2, R8, 3, 8, D), f32),
                            pltpu.VMEM((S + 64, D), bf16), pltpu.VMEM((S, D), bf16),
                            pltpu.VMEM((KVR, D), bf16),
                            pltpu.VMEM((D, S), bf16), pltpu.VMEM((F, D), bf16), pltpu.VMEM((F, D), bf16),
                            pltpu.VMEM((F // 2, D), u32), pltpu.VMEM((F // 2, D), u32),
                            pltpu.VMEM((TM // 2, D), u32), pltpu.VMEM((B, 2 * D), u32), pltpu.VMEM((TM // 2, D), u32), pltpu.VMEM((TM // 2, D), u32),
                            pltpu.VMEM((40, D), f32), pltpu.VMEM((64, 128), f32),
                            pltpu.VMEM((4, D), bf16), pltpu.VMEM((D,), bf16), pltpu.VMEM((F,), bf16), pltpu.VMEM((D,), bf16),
                            pltpu.VMEM((5 * B, B), bf16),
                            pltpu.SemaphoreType.DMA((NSTEP,)), pltpu.SemaphoreType.DMA((2,)),
                            pltpu.SemaphoreType.DMA((NT,)), pltpu.SemaphoreType.DMA((len(w1b) - 1,)), pltpu.SemaphoreType.DMA((len(w2b) - 1,)),
                            pltpu.SemaphoreType.DMA(()), pltpu.SemaphoreType.REGULAR],
            compiler_params=pltpu.CompilerParams(vmem_limit_bytes=110 * 1024 * 1024, disable_bounds_checks=nobc),
        )(jnp.zeros((1,), jnp.int32), A_q.reshape(S, D), A_k.reshape(S, D), A_v.reshape(S, D), A_ssm_k, B_w1.T, B_w2,
          A_shift_k.T, A_ssm_D, B_b1, B_b2, jnp.asarray(C, bf16))
        return out.reshape(1, S, D)
    return f


_impl = make(rem=True)


@jax.jit
def pallas_parallel_sum__ssm_conv_h3__dense_activation_gelu__prompt_kernel(
    A_q, A_k, A_v, A_shift_k, A_ssm_k, A_ssm_D, B_x, B_w1, B_b1, B_w2, B_b2
):
    return _impl(A_q, A_k, A_v, A_shift_k, A_ssm_k, A_ssm_D, B_x, B_w1, B_b1, B_w2, B_b2)
```

```python
import functools
import jax, jax.numpy as jnp, numpy as np
from jax import lax
from jax.experimental import pallas as pl
from jax.experimental.pallas import tpu as pltpu

S, D, F = 2048, 640, 1728
B = 128
NB = S // B
TM = 256
NSTEP = S // TM
NT = D // 128
R8 = B // 8
HB = B // 2
Z = NB
DUM = NB + 1
H0 = NB + 2
KO = 16
VO = 16 + S
FO = 16 + 2 * S
KVR = 2 * S + 64
FM = 1664
f32 = jnp.float32
bf16 = jnp.bfloat16
u32 = jnp.uint32
NT_DIMS = (((1,), (1,)), ((), ()))
TN_DIMS = (((0,), (0,)), ((), ()))

def dft_mats():
    k = np.concatenate([np.arange(0, B, 2), np.arange(1, B, 2)]).astype(np.float64) + 0.5
    n = np.arange(B, dtype=np.float64)
    th = 2 * np.pi * np.outer(k, n) / (2 * B)
    Fu = np.concatenate([np.cos(th), -np.sin(th)], 0)
    c = (B - 1) / 2
    ph = 2 * np.pi * np.outer(k, n - c) / (2 * B)
    Fh = np.concatenate([np.cos(ph), -np.sin(ph)], 0)
    Gm = np.concatenate([np.cos(ph).T[:HB], np.sin(ph).T[:HB]], 0) / B
    return np.concatenate([Fh, Fu, Gm], 0).astype(np.float32)

def pk(x):
    return pltpu.bitcast(x, u32)

def upk(x):
    return pltpu.bitcast(x, bf16)

def make(kvshift=False, kvrows=32, kvanchor='h', kvt=(2, 12), w1b=(0, 640, 1728), ln0c=4, ln0a=0, ln0n=48, fsd=2, fa=((0, 80), (40, 160), (100, 260), (8, 90)), nobc=True, kvscr=True, mat=0, lnt=(1, 3), lnn=16):
    def kern(z_ref, x_hbm, k_hbm, v_hbm, h_hbm, w1_hbm, w2_hbm, sk_hbm, sD_hbm, b1_hbm, b2_hbm, C_hbm,
             o_hbm,
             UH, x_v, o_v, KV, h_v, w1_v, w2_v, w1p, w2p, kvb_ref, Q_ref, xn_ref, xb_ref, x2_ref, skb_ref, ks_ref, b1c_ref,
             sk_ref, sD_ref, b1_ref, b2_ref, C_ref,
             sem_t, sem_0, sem_h, sem_w1, sem_o, sem_b):
        Fh_ref = C_ref.at[0:2 * B]; Fu_ref = C_ref.at[2 * B:4 * B]; Gm_ref = C_ref.at[4 * B:5 * B]
        def rows(i):
            return pl.ds(pl.multiple_of(i * TM, TM), TM)
        st = lambda i: isinstance(i, int)
        def bsem(i, kv):
            if not st(i) or i >= 3:
                return sem_t.at[i]
            if kv:
                return [sem_0.at[0], sem_0.at[3], sem_0.at[2]][i]
            return [sem_0.at[1], sem_w1.at[0], sem_0.at[2]][i]
        cx = lambda i: pltpu.make_async_copy(x_hbm.at[rows(i)], x_v.at[rows(i)], bsem(i, False))
        ck = lambda i: pltpu.make_async_copy(k_hbm.at[rows(i)], KV.at[pl.ds(pl.multiple_of(KO + i * TM, 16), TM)], bsem(i, True))
        cv = lambda i: pltpu.make_async_copy(v_hbm.at[rows(i)], KV.at[pl.ds(pl.multiple_of(VO + i * TM, 16), TM)], bsem(i, True))
        ch = lambda c: pltpu.make_async_copy(h_hbm.at[pl.ds(c * 128, 128)], h_v.at[pl.ds(c * 128, 128)], sem_h.at[c])
        co = lambda i: pltpu.make_async_copy(o_v.at[rows(i)], o_hbm.at[rows(i)], sem_o)
        def chunks(bounds):
            return [(bounds[i], bounds[i + 1]) for i in range(len(bounds) - 1)]
        W1C = chunks(w1b)
        cw1 = lambda i: pltpu.make_async_copy(w1_hbm.at[W1C[i][0]:W1C[i][1]], w1_v.at[W1C[i][0]:W1C[i][1]], sem_w1.at[i])
        cw2 = pltpu.make_async_copy(w2_hbm, w2_v, sem_0.at[0])
        small = [(C_hbm, C_ref, sem_h.at[0]), (sD_hbm, sD_ref, sem_h.at[0]), (sk_hbm, sk_ref, sem_0.at[0]),
                 (b1_hbm, b1_ref, sem_0.at[1]), (b2_hbm, b2_ref, sem_0.at[0])]
        cs_ = lambda i: pltpu.make_async_copy(*small[i])

        def bar():
            pl.semaphore_signal(sem_b, 1)
            pl.semaphore_wait(sem_b, 1)

        for cp in (([cs_(0), cs_(1), ch(0), ch(1), ch(2), ch(3), cx(0), cs_(3), ch(4), cx(1)] if ln0c == 4 else [cs_(0), cs_(1), ch(0), ch(1), ch(2), cx(0), cs_(3), ch(3), ch(4), cx(1)])
                   + [cw1(i) for i in range(len(W1C))] + [cs_(2), cs_(4), ck(0), cv(0), cw2, ck(1), cv(1)]):
            cp.start(); bar()
        ck(2).start(); cv(2).start(); cx(2).start(); bar()
        for i_ in range(3, NSTEP):
            ck(i_).start(); cv(i_).start(); cx(i_).start()
            if i_ in (3, 5):
                bar()

        zero = z_ref[0]
        never = jnp.full((8, 128), zero, jnp.int32) != 0
        KV[0:16, :] = jnp.zeros((16, D), bf16)
        nch = NT * TM // kvrows

        def kv_block(base, anchors=None):
            nrc = TM // kvrows
            fr = pl.ds(pl.multiple_of(FO + zero * 64, 16), 8)
            cols = []
            for c in range(NT):
                cs = slice(c * 128, (c + 1) * 128)
                col = []
                if anchors is not None:
                    skb_ref[pl.ds(pl.multiple_of(32 + zero * 8, 8), 8), 0:128] = anchors[c * nrc]
                sk = [jnp.concatenate([skb_ref[8 * j:8 * j + 8, cs]] * (kvrows // 8), axis=0) for j in range(4)]
                for rc in range(nrc):
                    if anchors is not None:
                        KV[fr, 0:128] = anchors[c * nrc + rc].astype(bf16)
                    r0 = pl.multiple_of(base + rc * kvrows, 16)
                    vv = KV[pl.ds(pl.multiple_of(r0 + VO, 16), kvrows), cs].astype(f32)
                    if kvshift:
                        o_ = 8 + rc * kvrows
                        if rc == 0:
                            ks_ref[c, 0:8, :] = KV[pl.ds(r0, 16), cs].astype(f32)[8:]
                        kf = KV[pl.ds(pl.multiple_of(r0 + 16, 16), kvrows), cs].astype(f32)
                        ks_ref[c, o_:o_ + kvrows, :] = kf
                        ks = kf * sk[0]
                        for j in range(1, 4):
                            ks = ks + ks_ref[c, o_ - j:o_ - j + kvrows, :] * sk[j]
                    else:
                        kext = KV[pl.ds(r0, kvrows + 16), cs].astype(f32)[8:]
                        ks = kext[8:] * sk[0]
                        for j in range(1, 4):
                            ks = ks + pltpu.roll(kext, j, 0)[8:, :] * sk[j]
                    kv = (ks * vv).astype(bf16)
                    if kvscr:
                        kvb_ref[rc * kvrows // 2:(rc + 1) * kvrows // 2, cs] = pk(kv)
                    col.append(kv)
                cols.append(jnp.concatenate(col, axis=0))
            return jnp.concatenate(cols, axis=1)

        def u_dft(t, kvb=None):
            Fu = Fu_ref[...]
            for j in range(2):
                kj = upk(kvb_ref[j * HB:(j + 1) * HB, :]) if (kvb is None or kvscr) else kvb[j * B:(j + 1) * B]
                u = jnp.dot(Fu, kj, preferred_element_type=f32)
                a = u[:B]; b = u[B:]
                UH[2 * t + j, :, 0] = (a + b).reshape(R8, 8, D)
                UH[2 * t + j, :, 1] = a.reshape(R8, 8, D)
                UH[2 * t + j, :, 2] = b.reshape(R8, 8, D)
            return b[B - 8:, D - 128:]

        def layernorm(t, anchors=None, dst=None, off=0):
            outs = []
            n = len(anchors) if anchors is not None else 1
            rr = TM // n
            for i in range(n):
                if anchors is not None:
                    x_v[pl.ds(pl.multiple_of(S + zero * 64, 16), 8), 0:128] = anchors[i].astype(bf16)
                x = x_v[pl.ds(pl.multiple_of(t * TM + i * rr, 16), rr), :].astype(f32)
                m = jnp.mean(x, axis=-1, keepdims=True)
                xc = x - m
                var = jnp.mean(xc * xc, axis=-1, keepdims=True)
                xn = xc * lax.rsqrt(var + 1e-5)
                (xn_ref if dst is None else dst)[off + i * rr // 2:off + (i + 1) * rr // 2, :] = pk(xn.astype(bf16))

        c1 = np.float32(2 * np.sqrt(2 / np.pi)); c2 = np.float32(8 * np.sqrt(2 / np.pi) * 0.044715)
        def gelu2(h):
            return (h + h * jnp.tanh(h * (c1 + c2 * (h * h)))).astype(bf16)

        def mlp1(xr, w1, lo, hi):
            b1 = b1_ref[...].astype(f32)[None, :] * 0.5
            h = lax.dot_general(upk(xr[...]), w1, NT_DIMS, preferred_element_type=f32) + b1[:, lo:hi]
            return h, gelu2(h)

        def mlp1_rem(xr, w1r):
            ht = lax.dot_general(w1r, upk(xr[...]), NT_DIMS, preferred_element_type=f32)
            bc = b1c_ref[...]
            return gelu2(ht + jnp.concatenate([bc] * (ht.shape[1] // 128), axis=1)).T

        def pts_anchor(val, t0_, t1_, n=nch):
            pts = [(t0_ * 16 + (i * (t1_ - t0_) * 16) // n) for i in range(n)]
            return [val[(p % 16) * 16:(p % 16) * 16 + 8, (p // 16) * 128:(p // 16 + 1) * 128] for p in pts]

        def mac(t, anchor=None, depth=0):
            pend = []
            if anchor is not None:
                UH[DUM + zero, 0, 0, :, 0:128] = anchor
            if st(t):
                nlag = 2 * t + 2
                uslot = [2 * t + 1 - l for l in range(nlag)]
            else:
                nlag = NB
                uslot = [2 * t + 1 - l if l < 6 else jnp.where(2 * t + 1 - l >= 0, 2 * t + 1 - l, Z) for l in range(nlag)]
            for ci in range(NT):
                cs = slice(ci * 128, (ci + 1) * 128)
                for r2 in range(0, R8, 2):
                    ld = lambda s: [UH[s, r2:r2 + 2, c_, :, cs].reshape(16, 128) for c_ in range(3)]
                    acc1 = None; acc0 = None
                    ucur = ld(uslot[0])
                    for l in range(nlag):
                        hv = ld(H0 + l)
                        p1 = [hv[c_] * ucur[c_] for c_ in range(3)]
                        if l + 1 < nlag:
                            ucur = ld(uslot[l + 1])
                            p0 = [hv[c_] * ucur[c_] for c_ in range(3)]
                            acc0 = p0 if acc0 is None else [x_ + y_ for x_, y_ in zip(acc0, p0)]
                        acc1 = p1 if acc1 is None else [x_ + y_ for x_, y_ in zip(acc1, p1)]
                    w = []
                    for j, acc in ((0, acc0), (1, acc1)):
                        w.append(pk((acc[0] - acc[2]).astype(bf16)))
                        w.append(pk((acc[0] + acc[1]).astype(bf16)))
                    if True:
                        s_ = (w[0] | w[1]) | (w[2] | w[3])
                        w = [jnp.where(never, s_, w_) for w_ in w]
                        if depth:
                            pend.append(s_)
                            if len(pend) >= depth:
                                UH[DUM + zero, 0, 0, :, 0:128] = pltpu.bitcast(pend.pop(0), f32)
                    for j in range(2):
                        col = slice(ci * 256 + j * 128, ci * 256 + (j + 1) * 128)
                        Q_ref[r2 * 4:r2 * 4 + 8, col] = w[2 * j]
                        Q_ref[HB + r2 * 4:HB + r2 * 4 + 8, col] = w[2 * j + 1]

        def idft():
            idx = 7 - lax.broadcasted_iota(jnp.int32, (8, 128), 0)
            cols = []
            for c in range(NT):
                qs = slice(c * 256, (c + 1) * 256)
                cc = jnp.dot(Gm_ref[0:HB, :], upk(Q_ref[0:HB, qs]), preferred_element_type=f32)
                ss = jnp.dot(Gm_ref[HB:, :], upk(Q_ref[HB:, qs]), preferred_element_type=f32)
                lo = cc - ss
                hi = cc + ss
                hi = jnp.concatenate(
                    [jnp.concatenate([jnp.take_along_axis(hi[r * 8:(r + 1) * 8, j * 128:(j + 1) * 128], idx, axis=0) for j in range(2)], axis=1)
                     for r in reversed(range(HB // 8))], axis=0)
                cols.append(jnp.concatenate([lo, hi], axis=0))
            yy = jnp.concatenate(cols, axis=1)
            y = jnp.concatenate([jnp.concatenate([yy[:, c * 256 + j * 128: c * 256 + (j + 1) * 128] for c in range(NT)], axis=1) for j in range(2)], axis=0)
            return y

        def combine(t, y, o, xb):
            xn = upk(xb[...]).astype(f32)
            x = x_v[rows(t), :].astype(f32)
            out = (xn * y + o) + x
            o_v[rows(t), :] = out.astype(bf16)

        def mlp_full():
            h, g = mlp1(xn_ref, upk(w1p[0:FM // 2, :]), 0, FM)
            g = jnp.concatenate([g, mlp1_rem(xn_ref, upk(w1p[FM // 2:, :]))], axis=1)
            o = jnp.dot(g, upk(w2p[...]), preferred_element_type=f32) + b2_ref[...].astype(f32)[None, :]
            return h, o

        UH[Z] = jnp.zeros(UH.shape[1:], f32)
        for c in range(NT):
            with jax.named_scope("waith"):
                if c == 0:
                    cs_(0).wait(); cs_(1).wait()
                if c == ln0c:
                    cx(0).wait(); cs_(3).wait()
                ch(c).wait()
            Fh = Fh_ref[...]
            cs = slice(c * 128, (c + 1) * 128)
            hp_re = hp_im = None
            anc = []
            for a in range(NB):
                hh = lax.dot_general(Fh, h_v[cs, a * B:(a + 1) * B], NT_DIMS, preferred_element_type=f32)
                if a == 0:
                    hh = hh + Fh[:, 0:1].astype(f32) * sD_ref[...].astype(f32)[None, cs]
                hre = hh[:B]; him = hh[B:]
                if a == 0:
                    c_, d_ = hre, him
                else:
                    c_ = jnp.concatenate([hre[:HB] - hp_im[:HB], hre[HB:] + hp_im[HB:]], axis=0)
                    d_ = jnp.concatenate([him[:HB] + hp_re[:HB], him[HB:] - hp_re[HB:]], axis=0)
                UH[H0 + a, :, 0, :, cs] = c_.reshape(R8, 8, 128)
                UH[H0 + a, :, 1, :, cs] = (d_ - c_).reshape(R8, 8, 128)
                UH[H0 + a, :, 2, :, cs] = (c_ + d_).reshape(R8, 8, 128)
                hp_re, hp_im = hre, him
                if a % 4 == 0:
                    anc.extend([hh[r * 16:r * 16 + 8] for r in range(16)])
            if c == ln0c:
                layernorm(0, [anc[ln0a + (i * ln0n) // 16] for i in range(16)], x2_ref, 0)
        b1t = jnp.broadcast_to(b1_ref[...].astype(f32)[None, F - 128:], (128, 128)).T
        b1c_ref[...] = b1t[64:] * 0.5
        gs = []
        for i, (lo, hi) in enumerate(W1C):
            with jax.named_scope("waitw1"):
                if i == 0:
                    cx(1).wait()
                cw1(i).wait()
            w1 = (w1_v[lo:hi, :].astype(f32) * 0.5).astype(bf16)
            w1p[lo // 2:hi // 2, :] = pk(w1)
            nt_ = ((hi if hi < F else FM) - lo) // 128
            def quarters(a_):
                return jnp.concatenate([mlp1(x2_ref.at[q * 64:(q + 1) * 64], upk(w1p[a_ // 2:(a_ + 128) // 2, :]), a_, a_ + 128)[1] for q in range(4)], axis=0)
            if i == 0:
                e_ = hi - 128 if nt_ % 2 else hi
                ha, ga = mlp1(x2_ref.at[0:TM // 2], w1[:e_ - lo], lo, e_)
                layernorm(1, None, x2_ref, TM // 2)
                hb_, gb = mlp1(x2_ref.at[TM // 2:TM], upk(w1p[lo // 2:e_ // 2, :]), lo, e_)
                gs.append(jnp.concatenate([ga, gb], axis=0))
                if e_ < hi:
                    gs.append(quarters(e_))
            elif hi == F:
                gr = mlp1_rem(x2_ref, w1[FM - lo:])
                e_ = FM - 128 * (nt_ % 4)
                gs.append(mlp1(x2_ref, w1[:e_ - lo], lo, e_)[1])
                for a_ in range(e_, FM, 128):
                    gs.append(quarters(a_))
                gs.append(gr)
            else:
                gs.append(mlp1(x2_ref, w1, lo, hi)[1])
        g2 = jnp.concatenate(gs, axis=1)

        def first_steps(t):
            g = g2[t * TM:(t + 1) * TM]
            b2 = b2_ref[...].astype(f32)[None, :]
            def w2cols(lo, hi):
                if t == 0:
                    w2 = w2_v[:, lo:hi]
                    w2p[:, lo:hi] = pk(w2)
                    return w2
                return upk(w2p[:, lo:hi])
            parts = []
            def mm(n):
                lo, hi = n * 128, (n + 1) * 128
                w2 = w2cols(lo, hi)
                acc = b2[:, lo:hi]
                for k0 in range(0, F, 512):
                    k1 = min(F, k0 + 512)
                    acc = jnp.dot(g[:, k0:k1], w2[k0:k1], preferred_element_type=f32) + acc
                    parts.extend([acc[r * 16:r * 16 + 8] for r in range(16)])
                return acc
            spread = lambda a_, b_, n_: [parts[a_ + (i * (b_ - a_)) // n_] for i in range(n_)]
            if t == 0:
                o0 = mm(0)
                o1 = mm(1)
                kv_block(zero * 64, spread(*fa[0], nch))
                ulast = u_dft(0)
                parts.clear()
                with jax.named_scope("waitk1"):
                    ck(1).wait(); cv(1).wait()
            else:
                ulast = u_dft(1)
                o0 = mm(0)
                o1 = mm(1)
            o2 = mm(2)
            o3 = mm(3)
            mac(t, parts[0] if t == 0 else ulast, fsd)
            y = idft()
            o4 = mm(4)
            kv_block((t + 1) * TM + zero * 64, spread(*fa[1 + t], nch))
            if t == 1:
                layernorm(2, spread(*fa[3], 16))
            combine(t, y, jnp.concatenate([o0, o1, o2, o3, o4], axis=1), x2_ref.at[t * TM // 2:(t + 1) * TM // 2])
            co(t).start()

        with jax.named_scope("waitw2"):
            cs_(2).wait(); cs_(4).wait(); ck(0).wait(); cv(0).wait(); cw2.wait()
        skf = sk_ref[...].astype(f32)
        for j in range(4):
            skb_ref[8 * j:8 * j + 8, :] = jnp.broadcast_to(skf[j:j + 1, :], (8, D))
        first_steps(0)
        with jax.named_scope("waitk1"):
            ck(2).wait(); cv(2).wait(); cx(2).wait()
        first_steps(1)

        def body(t, carry):
            tn = jnp.minimum(t + 1, NSTEP - 1)
            @pl.when(t + 1 < NSTEP)
            def _():
                ck(t + 1).wait(); cv(t + 1).wait(); cx(t + 1).wait()
            with jax.named_scope("step"):
                u_dft(t)
                xb_ref[...] = xn_ref[...]
                h, o = mlp_full()
                anchor = None
                if kvanchor == 'h':
                    anchor = pts_anchor(h, *kvt)
                elif kvanchor == 'o':
                    anchor = pts_anchor(o, *kvt)
                kv_block(tn * TM, anchor)
                mac(t)
                layernorm(tn, pts_anchor(o, *lnt, n=lnn) if lnn else None)
                combine(t, idft(), o, xb_ref)
            co(t).start()
            return carry
        lax.fori_loop(2, NSTEP, body, 0)
        with jax.named_scope("waito"):
            for i in range(NSTEP):
                co(i).wait()

    C = dft_mats()
    @jax.jit
    def f(A_q, A_k, A_v, A_shift_k, A_ssm_k, A_ssm_D, B_x, B_w1, B_b1, B_w2, B_b2):
        anyspec = pl.BlockSpec(memory_space=pl.ANY)
        out = pl.pallas_call(
            kern,
            in_specs=[pl.BlockSpec(memory_space=pltpu.SMEM)] + [anyspec] * 11,
            out_specs=anyspec,
            out_shape=jax.ShapeDtypeStruct((S, D), bf16),
            scratch_shapes=[pltpu.VMEM((2 * NB + 2, R8, 3, 8, D), f32),
                            pltpu.VMEM((S + 64, D), bf16), pltpu.VMEM((S, D), bf16),
                            pltpu.VMEM((KVR, D), bf16),
                            pltpu.VMEM((D, S), bf16), pltpu.VMEM((F, D), bf16), pltpu.VMEM((F, D), bf16),
                            pltpu.VMEM((F // 2, D), u32), pltpu.VMEM((F // 2, D), u32),
                            pltpu.VMEM((TM // 2, D), u32), pltpu.VMEM((B, 2 * D), u32), pltpu.VMEM((TM // 2, D), u32), pltpu.VMEM((TM // 2, D), u32),
                            pltpu.VMEM((TM, D), u32), pltpu.VMEM((40, D), f32), pltpu.VMEM((NT, TM + 8, 128), f32), pltpu.VMEM((64, 128), f32),
                            pltpu.VMEM((4, D), bf16), pltpu.VMEM((D,), bf16), pltpu.VMEM((F,), bf16), pltpu.VMEM((D,), bf16),
                            pltpu.VMEM((5 * B, B), bf16),
                            pltpu.SemaphoreType.DMA((NSTEP,)), pltpu.SemaphoreType.DMA((4,)),
                            pltpu.SemaphoreType.DMA((NT,)), pltpu.SemaphoreType.DMA((len(w1b) - 1,)),
                            pltpu.SemaphoreType.DMA(()), pltpu.SemaphoreType.REGULAR],
            compiler_params=pltpu.CompilerParams(vmem_limit_bytes=110 * 1024 * 1024, disable_bounds_checks=nobc),
        )(jnp.zeros((1,), jnp.int32), A_q.reshape(S, D), A_k.reshape(S, D), A_v.reshape(S, D), A_ssm_k, B_w1.T, B_w2,
          A_shift_k.T, A_ssm_D, B_b1, B_b2, jnp.asarray(C, bf16))
        return out.reshape(1, S, D)
    return f


_impl = make()


@jax.jit
def pallas_parallel_sum__ssm_conv_h3__dense_activation_gelu__prompt_kernel(
    A_q, A_k, A_v, A_shift_k, A_ssm_k, A_ssm_D, B_x, B_w1, B_b1, B_w2, B_b2
):
    return _impl(A_q, A_k, A_v, A_shift_k, A_ssm_k, A_ssm_D, B_x, B_w1, B_b1, B_w2, B_b2)
```

```python
import functools
import jax, jax.numpy as jnp, numpy as np
from jax import lax
from jax.experimental import pallas as pl
from jax.experimental.pallas import tpu as pltpu

S, D, F = 2048, 640, 1728
B = 128
NB = S // B
TM = 256
NSTEP = S // TM
NT = D // 128
R8 = B // 8
HB = B // 2
Z = NB
DUM = NB + 1
H0 = NB + 2
KO = 16
VO = 16 + S
FO = 16 + 2 * S
KVR = 2 * S + 64
FM = 1664
f32 = jnp.float32
bf16 = jnp.bfloat16
u32 = jnp.uint32
NT_DIMS = (((1,), (1,)), ((), ()))
TN_DIMS = (((0,), (0,)), ((), ()))

def dft_mats():
    k = np.concatenate([np.arange(0, B, 2), np.arange(1, B, 2)]).astype(np.float64) + 0.5
    n = np.arange(B, dtype=np.float64)
    th = 2 * np.pi * np.outer(k, n) / (2 * B)
    Fu = np.concatenate([np.cos(th), -np.sin(th)], 0)
    c = (B - 1) / 2
    ph = 2 * np.pi * np.outer(k, n - c) / (2 * B)
    Fh = np.concatenate([np.cos(ph), -np.sin(ph)], 0)
    Gm = np.concatenate([np.cos(ph).T[:HB], np.sin(ph).T[:HB]], 0) / B
    return np.concatenate([Fh, Fu, Gm], 0).astype(np.float32)

def pk(x):
    return pltpu.bitcast(x, u32)

def upk(x):
    return pltpu.bitcast(x, bf16)

def make(cp=dict(disable_semaphore_checks=True), la=((100, 200), (200, 260)), ipos=5, osplit=True, un=1, kvshift=False, kvrows=32, kvanchor='p', kvt=(2, 12), w1b=(0, 640, 1728), ln0c=4, ln0a=0, ln0n=48, fsd=(2, 1), fa=((0, 90), (70, 175), (120, 290), (8, 110)), nobc=True, kvscr=True, mat=0, lnt=(1, 3), lnn=16):
    def kern(z_ref, x_hbm, k_hbm, v_hbm, h_hbm, w1_hbm, w2_hbm, sk_hbm, sD_hbm, b1_hbm, b2_hbm, C_hbm,
             o_hbm,
             UH, x_v, o_v, KV, h_v, w1_v, w2_v, w1p, w2p, kvb_ref, QQ_ref, xn_ref, xb_ref, x2_ref, skb_ref, ks_ref, b1c_ref,
             sk_ref, sD_ref, b1_ref, b2_ref, C_ref,
             sem_t, sem_0, sem_h, sem_w1, sem_o, sem_b):
        Fh_ref = C_ref.at[0:2 * B]; Fu_ref = C_ref.at[2 * B:4 * B]; Gm_ref = C_ref.at[4 * B:5 * B]
        def rows(i):
            return pl.ds(pl.multiple_of(i * TM, TM), TM)
        st = lambda i: isinstance(i, int)
        def bsem(i, kv):
            if not st(i) or i >= 3:
                return sem_t.at[i]
            if kv:
                return [sem_0.at[0], sem_0.at[3], sem_0.at[2]][i]
            return [sem_0.at[1], sem_w1.at[0], sem_0.at[2]][i]
        cx = lambda i: pltpu.make_async_copy(x_hbm.at[rows(i)], x_v.at[rows(i)], bsem(i, False))
        ck = lambda i: pltpu.make_async_copy(k_hbm.at[rows(i)], KV.at[pl.ds(pl.multiple_of(KO + i * TM, 16), TM)], bsem(i, True))
        cv = lambda i: pltpu.make_async_copy(v_hbm.at[rows(i)], KV.at[pl.ds(pl.multiple_of(VO + i * TM, 16), TM)], bsem(i, True))
        ch = lambda c: pltpu.make_async_copy(h_hbm.at[pl.ds(c * 128, 128)], h_v.at[pl.ds(c * 128, 128)], sem_h.at[c])
        OC = [(0, 512), (512, D)] if osplit else [(0, D)]
        co = lambda i, p: pltpu.make_async_copy(o_v.at[rows(i), OC[p][0]:OC[p][1]], o_hbm.at[rows(i), OC[p][0]:OC[p][1]], sem_o)
        def chunks(bounds):
            return [(bounds[i], bounds[i + 1]) for i in range(len(bounds) - 1)]
        W1C = chunks(w1b)
        cw1 = lambda i: pltpu.make_async_copy(w1_hbm.at[W1C[i][0]:W1C[i][1]], w1_v.at[W1C[i][0]:W1C[i][1]], sem_w1.at[i])
        cw2 = pltpu.make_async_copy(w2_hbm, w2_v, sem_0.at[0])
        small = [(C_hbm, C_ref, sem_h.at[0]), (sD_hbm, sD_ref, sem_h.at[0]), (sk_hbm, sk_ref, sem_0.at[0]),
                 (b1_hbm, b1_ref, sem_0.at[1]), (b2_hbm, b2_ref, sem_0.at[0])]
        cs_ = lambda i: pltpu.make_async_copy(*small[i])

        def bar():
            pl.semaphore_signal(sem_b, 1)
            pl.semaphore_wait(sem_b, 1)

        for cp in (([cs_(0), cs_(1), ch(0), ch(1), ch(2), ch(3), cx(0), cs_(3), ch(4), cx(1)] if ln0c == 4 else [cs_(0), cs_(1), ch(0), ch(1), ch(2), cx(0), cs_(3), ch(3), ch(4), cx(1)])
                   + [cw1(i) for i in range(len(W1C))] + [cs_(2), cs_(4), ck(0), cv(0), cw2, ck(1), cv(1)]):
            cp.start(); bar()
        ck(2).start(); cv(2).start(); cx(2).start(); bar()
        for i_ in range(3, NSTEP):
            ck(i_).start(); cv(i_).start(); cx(i_).start()
            if i_ in (3, 5):
                bar()

        zero = jnp.clip(z_ref[0], 0, 1)
        never = jnp.full((8, 128), zero, jnp.int32) != 0
        KV[0:16, :] = jnp.zeros((16, D), bf16)
        nch = NT * TM // kvrows

        def kv_block(base, anchors=None):
            nrc = TM // kvrows
            fr = pl.ds(pl.multiple_of(FO + zero * 16, 16), 8)
            cols = []
            for c in range(NT):
                cs = slice(c * 128, (c + 1) * 128)
                col = []
                if anchors is not None:
                    skb_ref[pl.ds(pl.multiple_of(32 + zero * 8, 8), 8), 0:128] = anchors[c * nrc]
                sk = [jnp.concatenate([skb_ref[8 * j:8 * j + 8, cs]] * (kvrows // 8), axis=0) for j in range(4)]
                for rc in range(nrc):
                    if anchors is not None:
                        KV[fr, 0:128] = anchors[c * nrc + rc].astype(bf16)
                    r0 = base + rc * kvrows if st(base) else pl.multiple_of(base + rc * kvrows, 16)
                    vv = KV[pl.ds(r0 + VO if st(base) else pl.multiple_of(r0 + VO, 16), kvrows), cs].astype(f32)
                    if kvshift:
                        o_ = 8 + rc * kvrows
                        if rc == 0:
                            ks_ref[c, 0:8, :] = KV[pl.ds(r0, 16), cs].astype(f32)[8:]
                        kf = KV[pl.ds(pl.multiple_of(r0 + 16, 16), kvrows), cs].astype(f32)
                        ks_ref[c, o_:o_ + kvrows, :] = kf
                        ks = kf * sk[0]
                        for j in range(1, 4):
                            ks = ks + ks_ref[c, o_ - j:o_ - j + kvrows, :] * sk[j]
                    else:
                        kext = KV[pl.ds(r0, kvrows + 16), cs].astype(f32)[8:]
                        ks = kext[8:] * sk[0]
                        for j in range(1, 4):
                            ks = ks + pltpu.roll(kext, j, 0)[8:, :] * sk[j]
                    kv = (ks * vv).astype(bf16)
                    if kvscr:
                        kvb_ref[rc * kvrows // 2:(rc + 1) * kvrows // 2, cs] = pk(kv)
                    col.append(kv)
                cols.append(jnp.concatenate(col, axis=0))
            return jnp.concatenate(cols, axis=1)

        def u_dft(t, kvb=None):
            Fu = Fu_ref[...]
            for j in range(2):
                kj = upk(kvb_ref[j * HB:(j + 1) * HB, :]) if (kvb is None or kvscr) else kvb[j * B:(j + 1) * B]
                u = jnp.dot(Fu, kj, preferred_element_type=f32)
                a = u[:B]; b = u[B:]
                UH[2 * t + j, :, 0] = (a + b).reshape(R8, 8, D)
                UH[2 * t + j, :, 1] = a.reshape(R8, 8, D)
                UH[2 * t + j, :, 2] = b.reshape(R8, 8, D)
            return b[B - 8:, D - 128:]

        def layernorm(t, anchors=None, dst=None, off=0):
            outs = []
            n = len(anchors) if anchors is not None else 1
            rr = TM // n
            for i in range(n):
                if anchors is not None:
                    x_v[pl.ds(pl.multiple_of(S + zero * 16, 16), 8), 0:128] = anchors[i].astype(bf16)
                x = x_v[pl.ds(pl.multiple_of(t * TM + i * rr, 16), rr), :].astype(f32)
                m = jnp.mean(x, axis=-1, keepdims=True)
                xc = x - m
                var = jnp.mean(xc * xc, axis=-1, keepdims=True)
                xn = xc * lax.rsqrt(var + 1e-5)
                (xn_ref if dst is None else dst)[off + i * rr // 2:off + (i + 1) * rr // 2, :] = pk(xn.astype(bf16))

        c1 = np.float32(2 * np.sqrt(2 / np.pi)); c2 = np.float32(8 * np.sqrt(2 / np.pi) * 0.044715)
        def gelu2(h):
            return (h + h * jnp.tanh(h * (c1 + c2 * (h * h)))).astype(bf16)

        def mlp1(xr, w1, lo, hi):
            b1 = b1_ref[...].astype(f32)[None, :] * 0.5
            h = lax.dot_general(upk(xr[...]), w1, NT_DIMS, preferred_element_type=f32) + b1[:, lo:hi]
            return h, gelu2(h)

        def mlp1_rem(xr, w1r):
            ht = lax.dot_general(w1r, upk(xr[...]), NT_DIMS, preferred_element_type=f32)
            bc = b1c_ref[...]
            return gelu2(ht + jnp.concatenate([bc] * (ht.shape[1] // 128), axis=1)).T

        def pts_anchor(val, t0_, t1_, n=nch):
            pts = [(t0_ * 16 + (i * (t1_ - t0_) * 16) // n) for i in range(n)]
            return [val[(p % 16) * 16:(p % 16) * 16 + 8, (p // 16) * 128:(p // 16 + 1) * 128] for p in pts]

        def mac(t, anchor=None, depth=0, qi=0):
            Q_ref = QQ_ref.at[qi]
            pend = []
            if anchor is not None:
                UH[DUM, zero, 0, :, 0:128] = anchor
            if st(t):
                nlag = 2 * t + 2
                uslot = [2 * t + 1 - l for l in range(nlag)]
            else:
                nlag = NB
                uslot = [2 * t + 1 - l if l < 6 else jnp.where(2 * t + 1 - l >= 0, 2 * t + 1 - l, Z) for l in range(nlag)]
            for ci in range(NT):
                cs = slice(ci * 128, (ci + 1) * 128)
                for r2 in range(0, R8, 2):
                    ld = lambda s: [UH[s, r2:r2 + 2, c_, :, cs].reshape(16, 128) for c_ in range(3)]
                    acc1 = None; acc0 = None
                    ucur = ld(uslot[0])
                    for l in range(nlag):
                        hv = ld(H0 + l)
                        p1 = [hv[c_] * ucur[c_] for c_ in range(3)]
                        if l + 1 < nlag:
                            ucur = ld(uslot[l + 1])
                            p0 = [hv[c_] * ucur[c_] for c_ in range(3)]
                            acc0 = p0 if acc0 is None else [x_ + y_ for x_, y_ in zip(acc0, p0)]
                        acc1 = p1 if acc1 is None else [x_ + y_ for x_, y_ in zip(acc1, p1)]
                    w = []
                    for j, acc in ((0, acc0), (1, acc1)):
                        w.append(pk((acc[0] - acc[2]).astype(bf16)))
                        w.append(pk((acc[0] + acc[1]).astype(bf16)))
                    if True:
                        s_ = (w[0] | w[1]) | (w[2] | w[3])
                        w = [jnp.where(never, s_, w_) for w_ in w]
                        if depth:
                            pend.append(s_)
                            if len(pend) >= depth:
                                UH[DUM, zero, 0, :, 0:128] = pltpu.bitcast(pend.pop(0), f32)
                    for j in range(2):
                        col = slice(ci * 256 + j * 128, ci * 256 + (j + 1) * 128)
                        Q_ref[r2 * 4:r2 * 4 + 8, col] = w[2 * j]
                        Q_ref[HB + r2 * 4:HB + r2 * 4 + 8, col] = w[2 * j + 1]

        def idft(qi=0):
            Q_ref = QQ_ref.at[qi]
            idx = 7 - lax.broadcasted_iota(jnp.int32, (8, 128), 0)
            cols = []
            for c in range(NT):
                qs = slice(c * 256, (c + 1) * 256)
                cc = jnp.dot(Gm_ref[0:HB, :], upk(Q_ref[0:HB, qs]), preferred_element_type=f32)
                ss = jnp.dot(Gm_ref[HB:, :], upk(Q_ref[HB:, qs]), preferred_element_type=f32)
                lo = cc - ss
                hi = cc + ss
                hi = jnp.concatenate(
                    [jnp.concatenate([jnp.take_along_axis(hi[r * 8:(r + 1) * 8, j * 128:(j + 1) * 128], idx, axis=0) for j in range(2)], axis=1)
                     for r in reversed(range(HB // 8))], axis=0)
                cols.append(jnp.concatenate([lo, hi], axis=0))
            yy = jnp.concatenate(cols, axis=1)
            y = jnp.concatenate([jnp.concatenate([yy[:, c * 256 + j * 128: c * 256 + (j + 1) * 128] for c in range(NT)], axis=1) for j in range(2)], axis=0)
            return y

        def combine(t, y, o, xb):
            for p, (lo, hi) in enumerate(OC):
                xn = upk(xb[:, lo:hi]).astype(f32)
                x = x_v[rows(t), lo:hi].astype(f32)
                out = (xn * y[:, lo:hi] + o[:, lo:hi]) + x
                o_v[rows(t), lo:hi] = out.astype(bf16)
                co(t, p).start()

        def mlp_a():
            h, g = mlp1(xn_ref, upk(w1p[0:FM // 2, :]), 0, FM)
            g = jnp.concatenate([g, mlp1_rem(xn_ref, upk(w1p[FM // 2:, :]))], axis=1)
            return h, g

        def mlp_b(g, lo, hi):
            return jnp.dot(g, upk(w2p[:, lo:hi]), preferred_element_type=f32) + b2_ref[...].astype(f32)[None, lo:hi]

        UH[Z] = jnp.zeros(UH.shape[1:], f32)
        for c in range(NT):
            with jax.named_scope("waith"):
                if c == 0:
                    cs_(0).wait(); cs_(1).wait()
                if c == ln0c:
                    cx(0).wait(); cs_(3).wait()
                ch(c).wait()
            Fh = Fh_ref[...]
            cs = slice(c * 128, (c + 1) * 128)
            hp_re = hp_im = None
            anc = []
            for a in range(NB):
                hh = lax.dot_general(Fh, h_v[cs, a * B:(a + 1) * B], NT_DIMS, preferred_element_type=f32)
                if a == 0:
                    hh = hh + Fh[:, 0:1].astype(f32) * sD_ref[...].astype(f32)[None, cs]
                hre = hh[:B]; him = hh[B:]
                if a == 0:
                    c_, d_ = hre, him
                else:
                    c_ = jnp.concatenate([hre[:HB] - hp_im[:HB], hre[HB:] + hp_im[HB:]], axis=0)
                    d_ = jnp.concatenate([him[:HB] + hp_re[:HB], him[HB:] - hp_re[HB:]], axis=0)
                UH[H0 + a, :, 0, :, cs] = c_.reshape(R8, 8, 128)
                UH[H0 + a, :, 1, :, cs] = (d_ - c_).reshape(R8, 8, 128)
                UH[H0 + a, :, 2, :, cs] = (c_ + d_).reshape(R8, 8, 128)
                hp_re, hp_im = hre, him
                if a % 4 == 0:
                    anc.extend([hh[r * 16:r * 16 + 8] for r in range(16)])
            if c == ln0c:
                layernorm(0, [anc[ln0a + (i * ln0n) // 16] for i in range(16)], x2_ref, 0)
        b1t = jnp.broadcast_to(b1_ref[...].astype(f32)[None, F - 128:], (128, 128)).T
        b1c_ref[...] = b1t[64:] * 0.5
        gs = []
        for i, (lo, hi) in enumerate(W1C):
            with jax.named_scope("waitw1"):
                if i == 0:
                    cx(1).wait()
                cw1(i).wait()
            w1 = (w1_v[lo:hi, :].astype(f32) * 0.5).astype(bf16)
            w1p[lo // 2:hi // 2, :] = pk(w1)
            nt_ = ((hi if hi < F else FM) - lo) // 128
            def quarters(a_):
                return jnp.concatenate([mlp1(x2_ref.at[q * 64:(q + 1) * 64], upk(w1p[a_ // 2:(a_ + 128) // 2, :]), a_, a_ + 128)[1] for q in range(4)], axis=0)
            if i == 0:
                e_ = hi - 128 if nt_ % 2 else hi
                ha, ga = mlp1(x2_ref.at[0:TM // 2], w1[:e_ - lo], lo, e_)
                layernorm(1, None, x2_ref, TM // 2)
                hb_, gb = mlp1(x2_ref.at[TM // 2:TM], upk(w1p[lo // 2:e_ // 2, :]), lo, e_)
                gs.append(jnp.concatenate([ga, gb], axis=0))
                if e_ < hi:
                    gs.append(quarters(e_))
            elif hi == F:
                gr = mlp1_rem(x2_ref, w1[FM - lo:])
                e_ = FM - 128 * (nt_ % 4)
                gs.append(mlp1(x2_ref, w1[:e_ - lo], lo, e_)[1])
                for a_ in range(e_, FM, 128):
                    gs.append(quarters(a_))
                gs.append(gr)
            else:
                gs.append(mlp1(x2_ref, w1, lo, hi)[1])
        g2 = jnp.concatenate(gs, axis=1)

        def first_steps(t):
            g = g2[t * TM:(t + 1) * TM]
            b2 = b2_ref[...].astype(f32)[None, :]
            def w2cols(lo, hi):
                if t == 0:
                    w2 = w2_v[:, lo:hi]
                    w2p[:, lo:hi] = pk(w2)
                    return w2
                return upk(w2p[:, lo:hi])
            parts = []
            def mm(n):
                lo, hi = n * 128, (n + 1) * 128
                w2 = w2cols(lo, hi)
                acc = b2[:, lo:hi]
                for k0 in range(0, F, 512):
                    k1 = min(F, k0 + 512)
                    acc = jnp.dot(g[:, k0:k1], w2[k0:k1], preferred_element_type=f32) + acc
                    parts.extend([acc[r * 16:r * 16 + 8] for r in range(16)])
                return acc
            spread = lambda a_, b_, n_: [parts[a_ + (i * (b_ - a_)) // n_] for i in range(n_)]
            if t == 0:
                o0 = mm(0)
                o1 = mm(1)
                kv_block(0, spread(*fa[0], nch))
                ulast = u_dft(0)
                parts.clear()
                with jax.named_scope("waitk1"):
                    ck(1).wait(); cv(1).wait()
            else:
                ulast = u_dft(1)
                o0 = mm(0)
                o1 = mm(1)
            o2 = mm(2)
            o3 = mm(3)
            mac(t, parts[0] if t == 0 else ulast, fsd[t])
            y = idft()
            o4 = mm(4)
            kv_block((t + 1) * TM, spread(*fa[1 + t], nch))
            if t == 1:
                layernorm(2, spread(*fa[3], 16))
            combine(t, y, jnp.concatenate([o0, o1, o2, o3, o4], axis=1), x2_ref.at[t * TM // 2:(t + 1) * TM // 2])

        with jax.named_scope("waitw2"):
            cs_(2).wait(); cs_(4).wait(); ck(0).wait(); cv(0).wait(); cw2.wait()
        skf = sk_ref[...].astype(f32)
        for j in range(4):
            skb_ref[8 * j:8 * j + 8, :] = jnp.broadcast_to(skf[j:j + 1, :], (8, D))
        first_steps(0)
        with jax.named_scope("waitk1"):
            ck(2).wait(); cv(2).wait(); cx(2).wait()
        first_steps(1)

        def step(t, qi):
            tn = jnp.minimum(t + 1, NSTEP - 1)
            u_dft(t)
            xb_ref[...] = xn_ref[...]
            h, g = mlp_a()
            if kvanchor != 'p':
                o = mlp_b(g, 0, ipos * 128)
                anchor = pts_anchor(h if kvanchor == 'h' else o, *kvt)
                kv_block(tn * TM, anchor)
                mac(t, qi=qi)
                layernorm(tn, pts_anchor(o, *lnt, n=lnn) if lnn else None)
                y = idft(qi)
                if ipos < NT:
                    o = jnp.concatenate([o, mlp_b(g, ipos * 128, D)], axis=1)
            else:
                parts = []
                b2 = b2_ref[...].astype(f32)[None, :]
                def mm(n):
                    lo, hi = n * 128, (n + 1) * 128
                    acc = b2[:, lo:hi]
                    for k0 in range(0, F, 512):
                        k1 = min(F, k0 + 512)
                        acc = jnp.dot(g[:, k0:k1], upk(w2p[k0 // 2:k1 // 2, lo:hi]), preferred_element_type=f32) + acc
                        parts.extend([acc[r * 16:r * 16 + 8] for r in range(16)])
                    return acc
                spread = lambda a_, b_, n_: [parts[a_ + (i * (b_ - a_)) // n_] for i in range(n_)]
                os_ = [mm(n) for n in range(ipos)]
                mac(t, qi=qi)
                y = idft(qi)
                os_ += [mm(n) for n in range(ipos, NT)]
                kv_block(tn * TM, spread(*la[0], nch))
                layernorm(tn, spread(*la[1], 16))
                o = jnp.concatenate(os_, axis=1)
            combine(t, y, o, xb_ref)

        def body(i, carry):
            t = i * un
            for j in range(un):
                if j < un - 1:
                    ck(t + j + 1).wait(); cv(t + j + 1).wait(); cx(t + j + 1).wait()
                else:
                    @pl.when(t + j + 1 < NSTEP)
                    def _():
                        ck(t + j + 1).wait(); cv(t + j + 1).wait(); cx(t + j + 1).wait()
            with jax.named_scope("step"):
                for j in range(un):
                    step(t + j, j)
            return carry
        lax.fori_loop(2 // un, NSTEP // un, body, 0)
        with jax.named_scope("waito"):
            for i in range(NSTEP):
                for p in range(len(OC)):
                    co(i, p).wait()

    C = dft_mats()
    @jax.jit
    def f(A_q, A_k, A_v, A_shift_k, A_ssm_k, A_ssm_D, B_x, B_w1, B_b1, B_w2, B_b2):
        anyspec = pl.BlockSpec(memory_space=pl.ANY)
        out = pl.pallas_call(
            kern,
            in_specs=[pl.BlockSpec(memory_space=pltpu.SMEM)] + [anyspec] * 11,
            out_specs=anyspec,
            out_shape=jax.ShapeDtypeStruct((S, D), bf16),
            scratch_shapes=[pltpu.VMEM((2 * NB + 2, R8, 3, 8, D), f32),
                            pltpu.VMEM((S + 64, D), bf16), pltpu.VMEM((S, D), bf16),
                            pltpu.VMEM((KVR, D), bf16),
                            pltpu.VMEM((D, S), bf16), pltpu.VMEM((F, D), bf16), pltpu.VMEM((F, D), bf16),
                            pltpu.VMEM((F // 2, D), u32), pltpu.VMEM((F // 2, D), u32),
                            pltpu.VMEM((TM // 2, D), u32), pltpu.VMEM((2, B, 2 * D), u32), pltpu.VMEM((TM // 2, D), u32), pltpu.VMEM((TM // 2, D), u32),
                            pltpu.VMEM((TM, D), u32), pltpu.VMEM((48, D), f32), pltpu.VMEM((NT, TM + 8, 128), f32), pltpu.VMEM((64, 128), f32),
                            pltpu.VMEM((4, D), bf16), pltpu.VMEM((D,), bf16), pltpu.VMEM((F,), bf16), pltpu.VMEM((D,), bf16),
                            pltpu.VMEM((5 * B, B), bf16),
                            pltpu.SemaphoreType.DMA((NSTEP,)), pltpu.SemaphoreType.DMA((4,)),
                            pltpu.SemaphoreType.DMA((NT,)), pltpu.SemaphoreType.DMA((len(w1b) - 1,)),
                            pltpu.SemaphoreType.DMA(()), pltpu.SemaphoreType.REGULAR],
            compiler_params=pltpu.CompilerParams(vmem_limit_bytes=110 * 1024 * 1024, disable_bounds_checks=nobc, **cp),
        )(jnp.zeros((1,), jnp.int32), A_q.reshape(S, D), A_k.reshape(S, D), A_v.reshape(S, D), A_ssm_k, B_w1.T, B_w2,
          A_shift_k.T, A_ssm_D, B_b1, B_b2, jnp.asarray(C, bf16))
        return out.reshape(1, S, D)
    return f


_impl = make()


@jax.jit
def pallas_parallel_sum__ssm_conv_h3__dense_activation_gelu__prompt_kernel(
    A_q, A_k, A_v, A_shift_k, A_ssm_k, A_ssm_D, B_x, B_w1, B_b1, B_w2, B_b2
):
    return _impl(A_q, A_k, A_v, A_shift_k, A_ssm_k, A_ssm_D, B_x, B_w1, B_b1, B_w2, B_b2)
```

```python
import functools
import jax, jax.numpy as jnp, numpy as np
from jax import lax
from jax.experimental import pallas as pl
from jax.experimental.pallas import tpu as pltpu

S, D, F = 2048, 640, 1728
B = 128
NB = S // B
TM = 256
NSTEP = S // TM
NT = D // 128
R8 = B // 8
HB = B // 2
Z = NB
DUM = NB + 1
H0 = NB + 2
KO = 16
VO = 16 + S
FO = 16 + 2 * S
KVR = 2 * S + 64
FM = 1664
f32 = jnp.float32
bf16 = jnp.bfloat16
u32 = jnp.uint32
NT_DIMS = (((1,), (1,)), ((), ()))
TN_DIMS = (((0,), (0,)), ((), ()))

def dft_mats():
    k = np.concatenate([np.arange(0, B, 2), np.arange(1, B, 2)]).astype(np.float64) + 0.5
    n = np.arange(B, dtype=np.float64)
    th = 2 * np.pi * np.outer(k, n) / (2 * B)
    Fu = np.concatenate([np.cos(th), -np.sin(th)], 0)
    c = (B - 1) / 2
    ph = 2 * np.pi * np.outer(k, n - c) / (2 * B)
    Fh = np.concatenate([np.cos(ph), -np.sin(ph)], 0)
    Gm = np.concatenate([np.cos(ph).T[:HB], np.sin(ph).T[:HB]], 0) / B
    il = lambda M: np.stack([M[:B].reshape(R8, 8, B), M[B:].reshape(R8, 8, B)], axis=1).reshape(2 * B, B)
    return np.concatenate([il(Fh), il(Fu), Gm], 0).astype(np.float32)

def pk(x):
    return pltpu.bitcast(x, u32)

def upk(x):
    return pltpu.bitcast(x, bf16)

def make(mf=None, cp=dict(disable_semaphore_checks=True), la=((100, 200), (200, 260)), ipos=5, osplit=True, un=1, kvshift=False, kvrows=32, kvanchor='p', kvt=(2, 12), w1b=(0, 256, 512, 1280, 1728), nh1=3, w2k=512, ln2='fb', hstep=1, fsa=(0, 11), ra=((0, 180), (60, 220), (120, 290), (8, 110)), ln0c=4, ln0a=0, ln0n=48, fsd=(2, 1), fa=((0, 90), (8, 170), (120, 290), (8, 110)), nobc=True, kvscr=True, mat=0, lnt=(1, 3), lnn=16):
    def kern(z_ref, x_hbm, k_hbm, v_hbm, h_hbm, w1_hbm, w2_hbm, sk_hbm, sD_hbm, b1_hbm, b2_hbm, C_hbm,
             o_hbm,
             UH, x_v, o_v, KV, h_v, w1_v, w2_v, w1p, w2p, kvb_ref, kvb2_ref, QQ_ref, xn_ref, xb_ref, x2_ref, skb_ref, ks_ref, b1c_ref,
             sk_ref, sD_ref, b1_ref, b2_ref, C_ref,
             sem_t, sem_0, sem_w1, sem_o, sem_b):
        Fh_ref = C_ref.at[0:2 * B]; Fu_ref = C_ref.at[2 * B:4 * B]; Gm_ref = C_ref.at[4 * B:5 * B]
        def rows(i):
            return pl.ds(pl.multiple_of(i * TM, TM), TM)
        st = lambda i: isinstance(i, int)
        def bsem(i, kv):
            if not st(i) or i >= 3:
                return sem_t.at[i]
            if kv:
                return sem_0.at[i] if i < 2 else sem_t.at[2]
            return [sem_w1.at[0], sem_w1.at[1], sem_0.at[0] if ln2 == 'r5' else sem_t.at[2]][i]
        cx = lambda i: pltpu.make_async_copy(x_hbm.at[rows(i)], x_v.at[rows(i)], bsem(i, False))
        ck = lambda i: pltpu.make_async_copy(k_hbm.at[rows(i)], KV.at[pl.ds(pl.multiple_of(KO + i * TM, 16), TM)], bsem(i, True))
        cv = lambda i: pltpu.make_async_copy(v_hbm.at[rows(i)], KV.at[pl.ds(pl.multiple_of(VO + i * TM, 16), TM)], bsem(i, True))
        ch = lambda c: pltpu.make_async_copy(h_hbm.at[pl.ds(c * 128, 128)], h_v.at[pl.ds(c * 128, 128)], sem_w1.at[3] if c < nh1 else sem_0.at[0])
        OC = [(0, 512), (512, D)] if osplit else [(0, D)]
        co = lambda i, p: pltpu.make_async_copy(o_v.at[rows(i), OC[p][0]:OC[p][1]], o_hbm.at[rows(i), OC[p][0]:OC[p][1]], sem_o)
        def chunks(bounds):
            return [(bounds[i], bounds[i + 1]) for i in range(len(bounds) - 1)]
        W1C = chunks(w1b); W2C = chunks((0, w2k, F))
        cw1 = lambda i: pltpu.make_async_copy(w1_hbm.at[W1C[i][0]:W1C[i][1]], w1_v.at[W1C[i][0]:W1C[i][1]], sem_w1.at[i])
        cw2 = lambda i: pltpu.make_async_copy(w2_hbm.at[W2C[i][0]:W2C[i][1]], w2_v.at[W2C[i][0]:W2C[i][1]], sem_0.at[i])
        small = [(C_hbm.at[0:2 * B], C_ref.at[0:2 * B], sem_w1.at[3]), (sD_hbm, sD_ref, sem_w1.at[3]), (sk_hbm, sk_ref, sem_0.at[0]),
                 (b1_hbm, b1_ref, sem_w1.at[0]), (b2_hbm, b2_ref, sem_0.at[0]), (C_hbm.at[2 * B:5 * B], C_ref.at[2 * B:5 * B], sem_0.at[1])]
        cs_ = lambda i: pltpu.make_async_copy(*small[i])

        def bar():
            pl.semaphore_signal(sem_b, 1)
            pl.semaphore_wait(sem_b, 1)

        for cp in [cx(0), cs_(3), cw1(0), cx(1), cw1(1), cw1(2), cw1(3), cs_(0), cs_(1), ch(0), ch(1), ch(2),
                   ch(3), ch(4), cs_(4), cw2(0), cs_(2), ck(0), cv(0)] + ([cx(2)] if ln2 == 'r5' else []):
            cp.start(); bar()
        for cp in [cw2(1), cs_(5), ck(1), cv(1)]:
            cp.start()
        bar()
        if ln2 != 'r5':
            cx(2).start()
        ck(2).start(); cv(2).start(); bar()
        for i_ in range(3, NSTEP):
            ck(i_).start(); cv(i_).start(); cx(i_).start()
            if i_ in (3, 5):
                bar()

        zero = jnp.clip(z_ref[0], 0, 1)
        never = jnp.full((8, 128), zero, jnp.int32) != 0
        KV[0:16, :] = jnp.zeros((16, D), bf16)
        nch = NT * TM // kvrows

        def kv_block(base, anchors=None, dst=None):
            nrc = TM // kvrows
            fr = pl.ds(pl.multiple_of(FO + zero * 16, 16), 8)
            cols = []
            for c in range(NT):
                cs = slice(c * 128, (c + 1) * 128)
                col = []
                if anchors is not None:
                    skb_ref[pl.ds(pl.multiple_of(32 + zero * 8, 8), 8), 0:128] = anchors[c * nrc]
                sk = [jnp.concatenate([skb_ref[8 * j:8 * j + 8, cs]] * (kvrows // 8), axis=0) for j in range(4)]
                for rc in range(nrc):
                    if anchors is not None:
                        KV[fr, 0:128] = anchors[c * nrc + rc].astype(bf16)
                    r0 = base + rc * kvrows if st(base) else pl.multiple_of(base + rc * kvrows, 16)
                    vv = KV[pl.ds(r0 + VO if st(base) else pl.multiple_of(r0 + VO, 16), kvrows), cs].astype(f32)
                    if kvshift:
                        o_ = 8 + rc * kvrows
                        if rc == 0:
                            ks_ref[c, 0:8, :] = KV[pl.ds(r0, 16), cs].astype(f32)[8:]
                        kf = KV[pl.ds(pl.multiple_of(r0 + 16, 16), kvrows), cs].astype(f32)
                        ks_ref[c, o_:o_ + kvrows, :] = kf
                        ks = kf * sk[0]
                        for j in range(1, 4):
                            ks = ks + ks_ref[c, o_ - j:o_ - j + kvrows, :] * sk[j]
                    else:
                        kext = KV[pl.ds(r0, kvrows + 16), cs].astype(f32)[8:]
                        ks = kext[8:] * sk[0]
                        for j in range(1, 4):
                            ks = ks + pltpu.roll(kext, j, 0)[8:, :] * sk[j]
                    kv = (ks * vv).astype(bf16)
                    if kvscr:
                        (kvb_ref if dst is None else dst)[rc * kvrows // 2:(rc + 1) * kvrows // 2, cs] = pk(kv)
                    col.append(kv)
                cols.append(jnp.concatenate(col, axis=0))
            return jnp.concatenate(cols, axis=1)

        def u_dft(t, src=None):
            Fu = Fu_ref[...]
            for j in range(2):
                kj = upk((kvb_ref if src is None else src)[j * HB:(j + 1) * HB, :])
                u = jnp.dot(Fu, kj, preferred_element_type=f32)
                u = u.reshape(R8, 2, 8, D)
                a = u[:, 0]; b = u[:, 1]
                UH[2 * t + j, :, 0] = a + b
                UH[2 * t + j, :, 1] = a
                UH[2 * t + j, :, 2] = b
            return b[R8 - 1, :, D - 128:]

        def layernorm(t, anchors=None, dst=None, off=0):
            outs = []
            n = len(anchors) if anchors is not None else 1
            rr = TM // n
            for i in range(n):
                if anchors is not None:
                    x_v[pl.ds(pl.multiple_of(S + zero * 16, 16), 8), 0:128] = anchors[i].astype(bf16)
                x = x_v[pl.ds(pl.multiple_of(t * TM + i * rr, 16), rr), :].astype(f32)
                m = jnp.mean(x, axis=-1, keepdims=True)
                xc = x - m
                var = jnp.mean(xc * xc, axis=-1, keepdims=True)
                xn = xc * lax.rsqrt(var + 1e-5)
                (xn_ref if dst is None else dst)[off + i * rr // 2:off + (i + 1) * rr // 2, :] = pk(xn.astype(bf16))

        c1 = np.float32(2 * np.sqrt(2 / np.pi)); c2 = np.float32(8 * np.sqrt(2 / np.pi) * 0.044715)
        def gelu2(h):
            return (h + h * jnp.tanh(h * (c1 + c2 * (h * h)))).astype(bf16)

        def mlp1(xr, w1, lo, hi):
            b1 = b1_ref[...].astype(f32)[None, :] * 0.5
            h = lax.dot_general(upk(xr[...]), w1, NT_DIMS, preferred_element_type=f32) + b1[:, lo:hi]
            return h, gelu2(h)

        def mlp1_rem(xr, w1r):
            ht = lax.dot_general(w1r, upk(xr[...]), NT_DIMS, preferred_element_type=f32)
            bc = b1c_ref[...]
            return gelu2(ht + jnp.concatenate([bc] * (ht.shape[1] // 128), axis=1)).T

        def pts_anchor(val, t0_, t1_, n=nch):
            pts = [(t0_ * 16 + (i * (t1_ - t0_) * 16) // n) for i in range(n)]
            return [val[(p % 16) * 16:(p % 16) * 16 + 8, (p // 16) * 128:(p // 16 + 1) * 128] for p in pts]

        def mac(t, anchor=None, depth=0, qi=0):
            Q_ref = QQ_ref.at[qi]
            pend = []
            if anchor is not None:
                UH[DUM, zero, 0, :, 0:128] = anchor
            if st(t):
                nlag = 2 * t + 2
                uslot = [2 * t + 1 - l for l in range(nlag)]
            else:
                nlag = NB
                uslot = [2 * t + 1 - l if l < 6 else jnp.where(2 * t + 1 - l >= 0, 2 * t + 1 - l, Z) for l in range(nlag)]
            for ci in range(NT):
                cs = slice(ci * 128, (ci + 1) * 128)
                for r2 in range(0, R8, 2):
                    ld = lambda s: [UH[s, r2:r2 + 2, c_, :, cs].reshape(16, 128) for c_ in range(3)]
                    acc1 = None; acc0 = None
                    ucur = ld(uslot[0])
                    for l in range(nlag):
                        hv = ld(H0 + l)
                        p1 = [hv[c_] * ucur[c_] for c_ in range(3)]
                        if l + 1 < nlag:
                            ucur = ld(uslot[l + 1])
                            p0 = [hv[c_] * ucur[c_] for c_ in range(3)]
                            acc0 = p0 if acc0 is None else [x_ + y_ for x_, y_ in zip(acc0, p0)]
                        acc1 = p1 if acc1 is None else [x_ + y_ for x_, y_ in zip(acc1, p1)]
                    w = []
                    for j, acc in ((0, acc0), (1, acc1)):
                        w.append(pk((acc[0] - acc[2]).astype(bf16)))
                        w.append(pk((acc[0] + acc[1]).astype(bf16)))
                    if True:
                        s_ = (w[0] | w[1]) | (w[2] | w[3])
                        w = [jnp.where(never, s_, w_) for w_ in w]
                        if depth:
                            pend.append(s_)
                            if len(pend) >= depth:
                                UH[DUM, zero, 0, :, 0:128] = pltpu.bitcast(pend.pop(0), f32)
                    for j in range(2):
                        col = slice(ci * 256 + j * 128, ci * 256 + (j + 1) * 128)
                        Q_ref[r2 * 4:r2 * 4 + 8, col] = w[2 * j]
                        Q_ref[HB + r2 * 4:HB + r2 * 4 + 8, col] = w[2 * j + 1]

        def idft(qi=0):
            Q_ref = QQ_ref.at[qi]
            idx = 7 - lax.broadcasted_iota(jnp.int32, (8, 128), 0)
            cols = []
            for c in range(NT):
                qs = slice(c * 256, (c + 1) * 256)
                cc = jnp.dot(Gm_ref[0:HB, :], upk(Q_ref[0:HB, qs]), preferred_element_type=f32)
                ss = jnp.dot(Gm_ref[HB:, :], upk(Q_ref[HB:, qs]), preferred_element_type=f32)
                lo = cc - ss
                hi = cc + ss
                hi = jnp.concatenate(
                    [jnp.concatenate([jnp.take_along_axis(hi[r * 8:(r + 1) * 8, j * 128:(j + 1) * 128], idx, axis=0) for j in range(2)], axis=1)
                     for r in reversed(range(HB // 8))], axis=0)
                cols.append(jnp.concatenate([lo, hi], axis=0))
            yy = jnp.concatenate(cols, axis=1)
            y = jnp.concatenate([jnp.concatenate([yy[:, c * 256 + j * 128: c * 256 + (j + 1) * 128] for c in range(NT)], axis=1) for j in range(2)], axis=0)
            return y

        def combine(t, y, o, xb):
            for p, (lo, hi) in enumerate(OC):
                xn = upk(xb[:, lo:hi]).astype(f32)
                x = x_v[rows(t), lo:hi].astype(f32)
                out = (xn * y[:, lo:hi] + o[:, lo:hi]) + x
                o_v[rows(t), lo:hi] = out.astype(bf16)
                co(t, p).start()

        def mlp_a():
            h, g = mlp1(xn_ref, upk(w1p[0:FM // 2, :]), 0, FM)
            gr_ = mlp1_rem(xn_ref, upk(w1p[FM // 2:, :]))
            if kvanchor == 'p':
                return h, (g, jnp.concatenate([g[:, 1536:], gr_], axis=1))
            return h, jnp.concatenate([g, gr_], axis=1)

        def mlp_b(g, lo, hi):
            return jnp.dot(g, upk(w2p[:, lo:hi]), preferred_element_type=f32) + b2_ref[...].astype(f32)[None, lo:hi]

        UH[Z] = jnp.zeros(UH.shape[1:], f32)
        def h_rounds(c):
            cs = slice(c * 128, (c + 1) * 128)
            hp_re = hp_im = None
            for a in range(NB):
                Fh = Fh_ref[...]
                hh = lax.dot_general(Fh, h_v[cs, a * B:(a + 1) * B], NT_DIMS, preferred_element_type=f32)
                if a == 0:
                    hh = hh + Fh[:, 0:1].astype(f32) * sD_ref[...].astype(f32)[None, cs]
                h4 = hh.reshape(R8, 2, 8, 128)
                hre = h4[:, 0]; him = h4[:, 1]
                if a == 0:
                    c_, d_ = hre, him
                else:
                    c_ = jnp.concatenate([hre[:R8 // 2] - hp_im[:R8 // 2], hre[R8 // 2:] + hp_im[R8 // 2:]], axis=0)
                    d_ = jnp.concatenate([him[:R8 // 2] + hp_re[:R8 // 2], him[R8 // 2:] - hp_re[R8 // 2:]], axis=0)
                UH[H0 + a, :, 0, :, cs] = c_
                UH[H0 + a, :, 1, :, cs] = d_ - c_
                UH[H0 + a, :, 2, :, cs] = c_ + d_
                hp_re, hp_im = hre, him
                if a % 4 == 3:
                    yield hh

        G = {}
        def mlp1_piece(q0, q1, n0, n1, split):
            for q in range(q0, q1, split):
                g_ = mlp1(x2_ref.at[q * 64:(q + split) * 64], upk(w1p[n0 * 64:n1 * 64, :]), n0 * 128, n1 * 128)[1]
                for qq in range(split):
                    for n in range(n0, n1):
                        G[(q + qq, n)] = g_[qq * 128:(qq + 1) * 128, (n - n0) * 128:(n - n0 + 1) * 128]

        def w1_load(i):
            lo, hi = W1C[i]
            w1p[lo // 2:hi // 2, :] = pk((w1_v[lo:hi, :].astype(f32) * 0.5).astype(bf16))

        n1, n2, n3 = W1C[0][1] // 128, W1C[1][1] // 128, W1C[2][1] // 128
        with jax.named_scope("w1"):
            cx(0).wait(); cs_(3).wait(); cw1(0).wait()
        w1_load(0)
        layernorm(0, None, x2_ref, 0)
        for q in range(2):
            for n in range(n1):
                mlp1_piece(q, q + 1, n, n + 1, 1)
        b1t = jnp.broadcast_to(b1_ref[...].astype(f32)[None, F - 128:], (128, 128)).T
        b1c_ref[...] = b1t[64:] * 0.5
        with jax.named_scope("w2"):
            cx(1).wait(); cw1(1).wait()
        w1_load(1)
        mlp1_piece(0, 2, n1, n2, 1)
        layernorm(1, None, x2_ref, TM // 2)
        mlp1_piece(2, 4, 0, n2, 2)
        with jax.named_scope("w3"):
            cw1(2).wait()
        w1_load(2)
        e_ = n3 - (n3 - n2) % 4
        mlp1_piece(0, 4, n2, e_, 4)
        for n in range(e_, n3, 2):
            mlp1_piece(0, 4, n, min(n + 2, n3), 2 if n + 2 <= n3 else 1)
        with jax.named_scope("w4"):
            cw1(3).wait(); cs_(0).wait(); cs_(1).wait()
            for c in range(nh1):
                ch(c).wait()
        w1_load(3)
        gr = mlp1_rem(x2_ref, upk(w1p[FM // 2:, :]))
        import itertools
        rounds = itertools.chain(*[h_rounds(c) for c in range(nh1)])
        nr = 4 * nh1
        pieces = [(q, n) for n in range(n3, FM // 128) for q in range(4)]
        done = 0
        for i, (q, n) in enumerate(pieces):
            for _ in range((i + 1) * nr // len(pieces) - done):
                next(rounds); done += 1
            mlp1_piece(q, q + 1, n, n + 1, 1)
        with jax.named_scope("w5"):
            for c in range(nh1, NT):
                ch(c).wait()
            cs_(4).wait(); cw2(0).wait(); cs_(2).wait(); ck(0).wait(); cv(0).wait()
            if ln2 == 'r5':
                cx(2).wait()
        skf = sk_ref[...].astype(f32)
        for j in range(4):
            skb_ref[8 * j:8 * j + 8, :] = jnp.broadcast_to(skf[j:j + 1, :], (8, D))
        def gslice(t, k0, k1):
            rws = []
            for q in (2 * t, 2 * t + 1):
                tiles = [G[(q, n)] for n in range(k0 // 128, min(k1, FM) // 128)]
                if k1 > FM:
                    tiles.append(gr[q * 128:(q + 1) * 128])
                rws.append(jnp.concatenate(tiles, axis=1))
            return jnp.concatenate(rws, axis=0)
        b2 = b2_ref[...].astype(f32)[None, :]
        parts = []
        def mmk(t, n, k0, k1, acc, fresh):
            lo, hi = n * 128, (n + 1) * 128
            if fresh:
                w2 = w2_v[k0:k1, lo:hi]
                w2p[k0 // 2:k1 // 2, lo:hi] = pk(w2)
            else:
                w2 = upk(w2p[k0 // 2:k1 // 2, lo:hi])
            acc = jnp.dot(gslice(t, k0, k1), w2, preferred_element_type=f32) + (b2[:, lo:hi] if acc is None else acc)
            parts.extend([acc[r * 16:r * 16 + 8] for r in range(16)])
            return acc
        rounds = itertools.chain(*[h_rounds(c) for c in range(nh1, NT)])
        nr = 4 * (NT - nh1)
        pieces = [(n, hf) for n in range(NT) for hf in range(2)]
        oh0 = {}
        done = 0
        for i, (n, hf) in enumerate(pieces):
            for _ in range(min(nr, ((i + 1) * nr + len(pieces) - 2) // (len(pieces) - 1)) - done):
                hh = next(rounds); done += 1
                parts.extend([hh[r * 16:r * 16 + 8] for r in range(0, 16, hstep)])
            lo, hi = n * 128, (n + 1) * 128
            if hf == 0:
                w2 = w2_v[0:w2k, lo:hi]
                w2p[0:w2k // 2, lo:hi] = pk(w2)
            else:
                w2 = upk(w2p[0:w2k // 2, lo:hi])
            acc = jnp.dot(gslice(0, 0, w2k)[hf * 128:(hf + 1) * 128], w2, preferred_element_type=f32) + b2[:, lo:hi]
            parts.extend([acc[r * 16:r * 16 + 8] for r in range(8)])
            oh0[(n, hf)] = acc
        o0 = [jnp.concatenate([oh0[(n, 0)], oh0[(n, 1)]], axis=0) for n in range(NT)]
        spread = lambda a_, b_, n_: [parts[a_ + (i * (b_ - a_)) // n_] for i in range(n_)]
        kv_block(0, spread(*ra[0], nch))
        if ln2 == 'r5':
            layernorm(2, spread(*ra[3], 16))

        with jax.named_scope("w6"):
            cw2(1).wait(); cs_(5).wait(); ck(1).wait(); cv(1).wait()
        parts.clear()
        KG = [(k0, min(F, k0 + 512)) for k0 in range(0, F, 512)]
        rest = [(n, k0, k1) for n in range(NT) for k0, k1 in KG if k0 >= w2k]
        def run0(lst):
            for n, k0, k1 in lst:
                o0[n] = mmk(0, n, k0, k1, o0[n], True)
        def mm1(n, acc=None, ga=0, gb=4):
            for k0, k1 in KG[ga:gb]:
                acc = mmk(1, n, k0, k1, acc, False)
            return acc
        ul0 = u_dft(0)
        run0(rest[:fsa[1]])
        mac(0, ul0, fsd[0], 0)
        y0 = idft(0)
        run0(rest[fsa[1]:])
        if ln2 == 'fa':
            layernorm(2, spread(*ra[3], 16))
        kv_block(TM, spread(*ra[1], nch))
        combine(0, y0, jnp.concatenate(o0, axis=1), x2_ref.at[0:TM // 2])
        with jax.named_scope("w7"):
            ck(2).wait(); cv(2).wait()
            if ln2 != 'r5':
                cx(2).wait()
        ul1 = u_dft(1)
        parts.clear()
        o1 = [mm1(n) for n in range(3)]
        oh = mm1(3, None, 0, 3)
        mac(1, ul1, fsd[1], 0)
        y1 = idft(0)
        o1.append(mm1(3, oh, 3, 4))
        o1.append(mm1(4))
        if ln2 == 'fb':
            layernorm(2, spread(*ra[3], 16))
        kv_block(2 * TM, spread(*ra[2], nch))
        combine(1, y1, jnp.concatenate(o1, axis=1), x2_ref.at[TM // 2:TM])

        def step(t, qi):
            tn = jnp.minimum(t + 1, NSTEP - 1)
            ul = u_dft(t)
            xb_ref[...] = xn_ref[...]
            h, g = mlp_a()
            if kvanchor != 'p':
                o = mlp_b(g, 0, ipos * 128)
                anchor = pts_anchor(h if kvanchor == 'h' else o, *kvt)
                kv_block(tn * TM, anchor)
                mac(t, qi=qi)
                layernorm(tn, pts_anchor(o, *lnt, n=lnn) if lnn else None)
                y = idft(qi)
                if ipos < NT:
                    o = jnp.concatenate([o, mlp_b(g, ipos * 128, D)], axis=1)
            else:
                parts = []
                b2 = b2_ref[...].astype(f32)[None, :]
                def mm(n):
                    lo, hi = n * 128, (n + 1) * 128
                    acc = b2[:, lo:hi]
                    for k0 in range(0, F, 512):
                        k1 = min(F, k0 + 512)
                        acc = jnp.dot(g[0][:, k0:k1] if k1 < F else g[1], upk(w2p[k0 // 2:k1 // 2, lo:hi]), preferred_element_type=f32) + acc
                        parts.extend([acc[r * 16:r * 16 + 8] for r in range(16)])
                    return acc
                spread = lambda a_, b_, n_: [parts[a_ + (i * (b_ - a_)) // n_] for i in range(n_)]
                os_ = [mm(n) for n in range(ipos)]
                mac(t, (h[0:8, 0:128] if mf == 'h' else ul) if (mf and qi > 0) else None, qi=qi)
                y = idft(qi)
                os_ += [mm(n) for n in range(ipos, NT)]
                kv_block(tn * TM, spread(*la[0], nch))
                layernorm(tn, spread(*la[1], 16))
                o = jnp.concatenate(os_, axis=1)
            combine(t, y, o, xb_ref)

        def body(i, carry):
            t = i * un
            for j in range(un):
                if j < un - 1:
                    ck(t + j + 1).wait(); cv(t + j + 1).wait(); cx(t + j + 1).wait()
                else:
                    @pl.when(t + j + 1 < NSTEP)
                    def _():
                      with jax.named_scope('lw'):
                        ck(t + j + 1).wait(); cv(t + j + 1).wait(); cx(t + j + 1).wait()
            with jax.named_scope("step"):
                for j in range(un):
                    step(t + j, j)
            return carry
        lax.fori_loop(2 // un, NSTEP // un, body, 0)
        with jax.named_scope("waito"):
            for i in range(NSTEP):
                for p in range(len(OC)):
                    co(i, p).wait()

    C = dft_mats()
    @jax.jit
    def f(A_q, A_k, A_v, A_shift_k, A_ssm_k, A_ssm_D, B_x, B_w1, B_b1, B_w2, B_b2):
        anyspec = pl.BlockSpec(memory_space=pl.ANY)
        out = pl.pallas_call(
            kern,
            in_specs=[pl.BlockSpec(memory_space=pltpu.SMEM)] + [anyspec] * 11,
            out_specs=anyspec,
            out_shape=jax.ShapeDtypeStruct((S, D), bf16),
            scratch_shapes=[pltpu.VMEM((2 * NB + 2, R8, 3, 8, D), f32),
                            pltpu.VMEM((S + 64, D), bf16), pltpu.VMEM((S, D), bf16),
                            pltpu.VMEM((KVR, D), bf16),
                            pltpu.VMEM((D, S), bf16), pltpu.VMEM((F, D), bf16), pltpu.VMEM((F, D), bf16),
                            pltpu.VMEM((F // 2, D), u32), pltpu.VMEM((F // 2, D), u32),
                            pltpu.VMEM((TM // 2, D), u32), pltpu.VMEM((TM // 2, D), u32), pltpu.VMEM((2, B, 2 * D), u32), pltpu.VMEM((TM // 2, D), u32), pltpu.VMEM((TM // 2, D), u32),
                            pltpu.VMEM((TM, D), u32), pltpu.VMEM((48, D), f32), pltpu.VMEM((NT, TM + 8, 128), f32), pltpu.VMEM((64, 128), f32),
                            pltpu.VMEM((4, D), bf16), pltpu.VMEM((D,), bf16), pltpu.VMEM((F,), bf16), pltpu.VMEM((D,), bf16),
                            pltpu.VMEM((5 * B, B), bf16),
                            pltpu.SemaphoreType.DMA((NSTEP,)), pltpu.SemaphoreType.DMA((2,)),
                            pltpu.SemaphoreType.DMA((len(w1b) - 1,)),
                            pltpu.SemaphoreType.DMA(()), pltpu.SemaphoreType.REGULAR],
            compiler_params=pltpu.CompilerParams(vmem_limit_bytes=110 * 1024 * 1024, disable_bounds_checks=nobc, **cp),
        )(jnp.zeros((1,), jnp.int32), A_q.reshape(S, D), A_k.reshape(S, D), A_v.reshape(S, D), A_ssm_k, B_w1.T, B_w2,
          A_shift_k.T, A_ssm_D, B_b1, B_b2, jnp.asarray(C, bf16))
        return out.reshape(1, S, D)
    return f


_impl = make()


@jax.jit
def pallas_parallel_sum__ssm_conv_h3__dense_activation_gelu__prompt_kernel(
    A_q, A_k, A_v, A_shift_k, A_ssm_k, A_ssm_D, B_x, B_w1, B_b1, B_w2, B_b2
):
    return _impl(A_q, A_k, A_v, A_shift_k, A_ssm_k, A_ssm_D, B_x, B_w1, B_b1, B_w2, B_b2)
```

```python
import itertools

import jax
import jax.numpy as jnp
import numpy as np
from jax import lax
from jax.experimental import pallas as pl
from jax.experimental.pallas import tpu as pltpu

S, D, F = 2048, 640, 1728
B = 128
NB = S // B
TM = 256
NSTEP = S // TM
NT = D // 128
R8 = B // 8
HB = B // 2
FM = 1664
KG = [(k0, min(F, k0 + 512)) for k0 in range(0, F, 512)]
Z, DUM, H0 = NB, NB + 1, NB + 2
KO, VO, FO, KVR = 16, 16 + S, 16 + 2 * S, 2 * S + 64
KVROWS = 32
NCH = NT * TM // KVROWS
f32, bf16, u32 = jnp.float32, jnp.bfloat16, jnp.uint32
NT_DIMS = (((1,), (1,)), ((), ()))


def dft_mats():
    k = np.concatenate([np.arange(0, B, 2), np.arange(1, B, 2)]).astype(np.float64) + 0.5
    n = np.arange(B, dtype=np.float64)
    c = (B - 1) / 2
    th = 2 * np.pi * np.outer(k, n - c / 2) / (2 * B)
    ph = 2 * np.pi * np.outer(k, n - c) / (2 * B)
    fwd = np.stack([np.cos(th).reshape(R8, 8, B), -np.sin(th).reshape(R8, 8, B)], axis=1).reshape(2 * B, B)
    inv = np.concatenate([np.cos(ph).T[:HB], np.sin(ph).T[:HB]], 0) / B
    return np.concatenate([fwd, inv], 0).astype(np.float32)


def pk(x):
    return pltpu.bitcast(x, u32)


def upk(x):
    return pltpu.bitcast(x, bf16)


def row_anchors(val, n=16):
    return [val[r * 16:r * 16 + 8] for r in range(n)]


def spread(parts, lo, hi, n):
    return [parts[lo + (i * (hi - lo)) // n] for i in range(n)]


def make(w1b=(0, 256, 512, 1408, 1728), nh1=3, la=((100, 200), (200, 260)),
         ra=((0, 180), (60, 220), (120, 290), (8, 110)), fsd=(2, 1), checks=False):
    W1C = list(zip(w1b[:-1], w1b[1:]))
    W2C = [(0, 512), (512, F)]

    def kern(z_ref, x_hbm, k_hbm, v_hbm, h_hbm, w1_hbm, w2_hbm, sk_hbm, sD_hbm, b1_hbm, b2_hbm, C_hbm,
             o_hbm,
             UH, x_v, o_v, KV, h_v, w1_v, w2_v, w1p, w2p, kvb_ref, Q_ref, xn_ref, xb_ref, x2_ref,
             skb_ref, b1c_ref, sk_ref, sD_ref, b1_ref, b2_ref, C_ref,
             sem_t, sem_a, sem_b, sem_o, sem_bar):
        F_ref, G_ref = C_ref.at[0:2 * B], C_ref.at[2 * B:3 * B]
        static = lambda i: isinstance(i, int)
        al = lambda i, m: i if static(i) else pl.multiple_of(i, m)
        rows = lambda i: pl.ds(al(i * TM, TM), TM)

        def copy(src, dst, sem):
            return pltpu.make_async_copy(src, dst, sem)

        xsem = lambda i: sem_a.at[i] if static(i) and i < 2 else sem_t.at[i - 2]
        ksem = lambda i: sem_b.at[i] if static(i) and i < 2 else sem_t.at[i - 2]
        cx = lambda i: copy(x_hbm.at[rows(i)], x_v.at[rows(i)], xsem(i))
        ck = lambda i: copy(k_hbm.at[rows(i)], KV.at[pl.ds(al(KO + i * TM, 16), TM)], ksem(i))
        cv = lambda i: copy(v_hbm.at[rows(i)], KV.at[pl.ds(al(VO + i * TM, 16), TM)], ksem(i))
        ch = lambda c: copy(h_hbm.at[c * 128:(c + 1) * 128], h_v.at[c * 128:(c + 1) * 128],
                            sem_a.at[3] if c < nh1 else sem_b.at[0])
        cw1 = lambda i: copy(w1_hbm.at[W1C[i][0]:W1C[i][1]], w1_v.at[W1C[i][0]:W1C[i][1]], sem_a.at[i])
        cw2 = lambda i: copy(w2_hbm.at[W2C[i][0]:W2C[i][1]], w2_v.at[W2C[i][0]:W2C[i][1]], sem_b.at[i])
        co = lambda i, c: copy(o_v.at[rows(i), c * 128:(c + 1) * 128], o_hbm.at[rows(i), c * 128:(c + 1) * 128], sem_o)
        cF = copy(C_hbm.at[0:2 * B], F_ref, sem_a.at[3])
        cG = copy(C_hbm.at[2 * B:3 * B], G_ref, sem_b.at[1])
        cD = copy(sD_hbm, sD_ref, sem_a.at[3])
        csk = copy(sk_hbm, sk_ref, sem_b.at[0])
        cb1 = copy(b1_hbm, b1_ref, sem_a.at[0])
        cb2 = copy(b2_hbm, b2_ref, sem_b.at[0])

        def wait(name, copies):
            with jax.named_scope(name):
                for cp in copies:
                    cp.wait()

        def bar():
            pl.semaphore_signal(sem_bar, 1)
            pl.semaphore_wait(sem_bar, 1)

        g1, g2, g3 = [cx(0), cb1, cw1(0)], [cx(1), cw1(1)], [cw1(2)]
        g4 = [cw1(3), cF, cD] + [ch(c) for c in range(nh1)]
        g5 = [ch(c) for c in range(nh1, NT)] + [cb2, cw2(0), csk, ck(0), cv(0)]
        g6 = [cw2(1), cG, ck(1), cv(1)]
        blk = lambda i: [cx(i), ck(i), cv(i)]
        for cp in g1 + g2 + g3 + g4 + g5:
            cp.start()
            bar()
        for i, grp in enumerate([g6] + [blk(i) for i in range(2, NSTEP)]):
            for cp in grp:
                cp.start()
            if i in (0, 1, 2, 4):
                bar()

        zero = jnp.clip(z_ref[0], 0, 1)
        never = jnp.full((8, 128), zero, jnp.int32) != 0
        KV[0:16, :] = jnp.zeros((16, D), bf16)
        UH[Z] = jnp.zeros(UH.shape[1:], f32)

        def kv_block(t, anchors):
            nrc = TM // KVROWS
            for c in range(NT):
                cs = slice(c * 128, (c + 1) * 128)
                skb_ref[pl.ds(pl.multiple_of(32 + zero * 8, 8), 8), 0:128] = anchors[c * nrc]
                sk = [jnp.concatenate([skb_ref[8 * j:8 * j + 8, cs]] * (KVROWS // 8), axis=0) for j in range(4)]
                for rc in range(nrc):
                    KV[pl.ds(pl.multiple_of(FO + zero * 16, 16), 8), 0:128] = anchors[c * nrc + rc].astype(bf16)
                    r0 = t * TM + rc * KVROWS
                    vv = KV[pl.ds(al(r0 + VO, 16), KVROWS), cs].astype(f32)
                    kext = KV[pl.ds(al(r0, 16), KVROWS + 16), cs].astype(f32)[8:]
                    ks = kext[8:] * sk[0]
                    for j in range(1, 4):
                        ks = ks + pltpu.roll(kext, j, 0)[8:, :] * sk[j]
                    kvb_ref[rc * KVROWS // 2:(rc + 1) * KVROWS // 2, cs] = pk((ks * vv).astype(bf16))

        def u_dft(t):
            fm = F_ref[...]
            for j in range(2):
                u = jnp.dot(fm, upk(kvb_ref[j * HB:(j + 1) * HB, :]), preferred_element_type=f32)
                u = u.reshape(R8, 2, 8, D)
                a, b = u[:, 0], u[:, 1]
                UH[2 * t + j, :, 0] = a + b
                UH[2 * t + j, :, 1] = a
                UH[2 * t + j, :, 2] = b
            return b[R8 - 1, :, D - 128:]

        def h_rounds(c):
            cs = slice(c * 128, (c + 1) * 128)
            hp_re = hp_im = None
            for a in range(NB):
                fm = F_ref[...]
                hh = lax.dot_general(fm, h_v[cs, a * B:(a + 1) * B], NT_DIMS, preferred_element_type=f32)
                if a == 0:
                    hh = hh + fm[:, 0:1].astype(f32) * sD_ref[...].astype(f32)[None, cs]
                h4 = hh.reshape(R8, 2, 8, 128)
                hre, him = h4[:, 0], h4[:, 1]
                if a == 0:
                    c_, d_ = hre, him
                else:
                    e = R8 // 2
                    c_ = jnp.concatenate([hre[:e] - hp_im[:e], hre[e:] + hp_im[e:]], axis=0)
                    d_ = jnp.concatenate([him[:e] + hp_re[:e], him[e:] - hp_re[e:]], axis=0)
                UH[H0 + a, :, 0, :, cs] = c_
                UH[H0 + a, :, 1, :, cs] = d_ - c_
                UH[H0 + a, :, 2, :, cs] = c_ + d_
                hp_re, hp_im = hre, him
                if a % 4 == 3:
                    yield hh

        def layernorm(t, dst, anchors=None):
            n = 1 if anchors is None else len(anchors)
            rr = TM // n
            for i in range(n):
                if anchors is not None:
                    x_v[pl.ds(pl.multiple_of(S + zero * 16, 16), 8), 0:128] = anchors[i].astype(bf16)
                x = x_v[pl.ds(al(t * TM + i * rr, 16), rr), :].astype(f32)
                m = jnp.mean(x, axis=-1, keepdims=True)
                xc = x - m
                var = jnp.mean(xc * xc, axis=-1, keepdims=True)
                xn = xc * lax.rsqrt(var + 1e-5)
                dst[i * rr // 2:(i + 1) * rr // 2, :] = pk(xn.astype(bf16))

        c1 = np.float32(2 * np.sqrt(2 / np.pi))
        c2 = np.float32(8 * np.sqrt(2 / np.pi) * 0.044715)

        def gelu(h):
            return (h + h * jnp.tanh(h * (c1 + c2 * (h * h)))).astype(bf16)

        def mlp1(xr, lo, hi):
            b1 = b1_ref[...].astype(f32)[None, :] * 0.5
            h = lax.dot_general(upk(xr[...]), upk(w1p[lo // 2:hi // 2, :]), NT_DIMS, preferred_element_type=f32)
            return gelu(h + b1[:, lo:hi])

        def mlp1_rem(xr):
            ht = lax.dot_general(upk(w1p[FM // 2:, :]), upk(xr[...]), NT_DIMS, preferred_element_type=f32)
            return gelu(ht + jnp.concatenate([b1c_ref[...]] * (ht.shape[1] // 128), axis=1)).T

        def mac(t, anchor=None, depth=0):
            if anchor is not None:
                UH[DUM, zero, 0, :, 0:128] = anchor
            if static(t):
                uslot = [2 * t + 1 - l for l in range(2 * t + 2)]
            else:
                uslot = [2 * t + 1 - l if l < 6 else jnp.where(2 * t + 1 - l >= 0, 2 * t + 1 - l, Z)
                         for l in range(NB)]
            nlag = len(uslot)
            pend = []
            for ci in range(NT):
                cs = slice(ci * 128, (ci + 1) * 128)
                for r2 in range(0, R8, 2):
                    ld = lambda s: [UH[s, r2:r2 + 2, c_, :, cs].reshape(16, 128) for c_ in range(3)]
                    add = lambda acc, p: p if acc is None else [x_ + y_ for x_, y_ in zip(acc, p)]
                    acc0 = acc1 = None
                    ucur = ld(uslot[0])
                    for l in range(nlag):
                        hv = ld(H0 + l)
                        p1 = [hv[c_] * ucur[c_] for c_ in range(3)]
                        if l + 1 < nlag:
                            ucur = ld(uslot[l + 1])
                            acc0 = add(acc0, [hv[c_] * ucur[c_] for c_ in range(3)])
                        acc1 = add(acc1, p1)
                    w = []
                    for acc in (acc0, acc1):
                        w.append(pk((acc[0] - acc[2]).astype(bf16)))
                        w.append(pk((acc[0] + acc[1]).astype(bf16)))
                    tie = (w[0] | w[1]) | (w[2] | w[3])
                    w = [jnp.where(never, tie, w_) for w_ in w]
                    if depth:
                        pend.append(tie)
                        if len(pend) >= depth:
                            UH[DUM, zero, 0, :, 0:128] = pltpu.bitcast(pend.pop(0), f32)
                    for j in range(2):
                        col = slice(ci * 256 + j * 128, ci * 256 + (j + 1) * 128)
                        Q_ref[r2 * 4:r2 * 4 + 8, col] = w[2 * j]
                        Q_ref[HB + r2 * 4:HB + r2 * 4 + 8, col] = w[2 * j + 1]

        def idft():
            flip = 7 - lax.broadcasted_iota(jnp.int32, (8, 128), 0)
            ys = []
            for c in range(NT):
                qs = slice(c * 256, (c + 1) * 256)
                cc = jnp.dot(G_ref[0:HB, :], upk(Q_ref[0:HB, qs]), preferred_element_type=f32)
                ss = jnp.dot(G_ref[HB:, :], upk(Q_ref[HB:, qs]), preferred_element_type=f32)
                lo, hi = cc - ss, cc + ss
                pieces = []
                for j in range(2):
                    js = slice(j * 128, (j + 1) * 128)
                    pieces.append(lo[:, js])
                    pieces += [jnp.take_along_axis(hi[r * 8:(r + 1) * 8, js], flip, axis=0)
                               for r in reversed(range(HB // 8))]
                ys.append(jnp.concatenate(pieces, axis=0))
            return ys

        def combine(t, ys, os_, xb):
            for c in range(NT):
                cs = slice(c * 128, (c + 1) * 128)
                out = (upk(xb[:, cs]).astype(f32) * ys[c] + os_[c]) + x_v[rows(t), cs].astype(f32)
                o_v[rows(t), cs] = out.astype(bf16)
                co(t, c).start()

        G = {}

        def mlp1_piece(q0, q1, n0, n1, split):
            for q in range(q0, q1, split):
                g_ = mlp1(x2_ref.at[q * 64:(q + split) * 64], n0 * 128, n1 * 128)
                for qq in range(split):
                    for n in range(n0, n1):
                        G[(q + qq, n)] = g_[qq * 128:(qq + 1) * 128, (n - n0) * 128:(n - n0 + 1) * 128]

        def w1_load(i):
            lo, hi = W1C[i]
            w1p[lo // 2:hi // 2, :] = pk((w1_v[lo:hi, :].astype(f32) * 0.5).astype(bf16))

        n1, n2, n3 = (W1C[i][1] // 128 for i in range(3))
        wait("w1", g1)
        w1_load(0)
        layernorm(0, x2_ref.at[0:TM // 2])
        for q in range(2):
            for n in range(n1):
                mlp1_piece(q, q + 1, n, n + 1, 1)
        b1t = jnp.broadcast_to(b1_ref[...].astype(f32)[None, F - 128:], (128, 128)).T
        b1c_ref[...] = b1t[64:] * 0.5

        wait("w2", g2)
        w1_load(1)
        mlp1_piece(0, 2, n1, n2, 1)
        layernorm(1, x2_ref.at[TM // 2:TM])
        mlp1_piece(2, 4, 0, n2, 2)

        wait("w3", g3)
        w1_load(2)
        e = n3 - (n3 - n2) % 4
        mlp1_piece(0, 4, n2, e, 4)
        for n in range(e, n3, 2):
            mlp1_piece(0, 4, n, min(n + 2, n3), 2 if n + 2 <= n3 else 1)

        wait("w4", g4)
        w1_load(3)
        gr = mlp1_rem(x2_ref)
        rounds = itertools.chain(*[h_rounds(c) for c in range(nh1)])
        pieces = [(q, n) for n in range(n3, FM // 128) for q in range(4)]
        done = 0
        for i, (q, n) in enumerate(pieces):
            for _ in range((i + 1) * 4 * nh1 // len(pieces) - done):
                next(rounds)
                done += 1
            mlp1_piece(q, q + 1, n, n + 1, 1)

        wait("w5", g5)
        skf = sk_ref[...].astype(f32)
        for j in range(4):
            skb_ref[8 * j:8 * j + 8, :] = jnp.broadcast_to(skf[j:j + 1, :], (8, D))
        b2 = b2_ref[...].astype(f32)[None, :]
        parts = []

        def gslice(qs, k0, k1):
            rws = []
            for q in qs:
                tiles = [G[(q, n)] for n in range(k0 // 128, min(k1, FM) // 128)]
                if k1 > FM:
                    tiles.append(gr[q * 128:(q + 1) * 128])
                rws.append(jnp.concatenate(tiles, axis=1))
            return jnp.concatenate(rws, axis=0)

        def mmk(qs, n, k0, k1, acc, fresh):
            cs = slice(n * 128, (n + 1) * 128)
            if fresh:
                w2 = w2_v[k0:k1, cs]
                w2p[k0 // 2:k1 // 2, cs] = pk(w2)
            else:
                w2 = upk(w2p[k0 // 2:k1 // 2, cs])
            acc = jnp.dot(gslice(qs, k0, k1), w2, preferred_element_type=f32) + (b2[:, cs] if acc is None else acc)
            parts.extend(row_anchors(acc, 8 * len(qs)))
            return acc

        rounds = itertools.chain(*[h_rounds(c) for c in range(nh1, NT)])
        nr = 4 * (NT - nh1)
        o0 = []
        done = 0
        for i in range(2 * NT):
            for _ in range(min(nr, ((i + 1) * nr + 2 * NT - 2) // (2 * NT - 1)) - done):
                parts.extend(row_anchors(next(rounds)))
                done += 1
            o0.append(mmk([i % 2], i // 2, *KG[0], None, i % 2 == 0))
        o0 = [jnp.concatenate(o0[2 * n:2 * n + 2], axis=0) for n in range(NT)]
        kv_block(0, spread(parts, *ra[0], NCH))

        wait("w6", g6)
        parts.clear()
        rest = [(n, g) for n in range(NT) for g in KG[1:]]
        ul = u_dft(0)
        for n, g in rest[:11]:
            o0[n] = mmk([0, 1], n, *g, o0[n], True)
        mac(0, ul, fsd[0])
        ys = idft()
        for n, g in rest[11:]:
            o0[n] = mmk([0, 1], n, *g, o0[n], True)
        kv_block(1, spread(parts, *ra[1], NCH))
        combine(0, ys, o0, x2_ref.at[0:TM // 2])

        wait("w7", blk(2))
        parts.clear()
        rest = [(n, g) for n in range(NT) for g in KG]
        o1 = [None] * NT
        ul = u_dft(1)
        for n, g in rest[:15]:
            o1[n] = mmk([2, 3], n, *g, o1[n], False)
        mac(1, ul, fsd[1])
        ys = idft()
        for n, g in rest[15:]:
            o1[n] = mmk([2, 3], n, *g, o1[n], False)
        layernorm(2, xn_ref, spread(parts, *ra[3], 16))
        kv_block(2, spread(parts, *ra[2], NCH))
        combine(1, ys, o1, x2_ref.at[TM // 2:TM])

        def body(t, carry):
            @pl.when(t + 1 < NSTEP)
            def _():
                wait("lw", blk(t + 1))

            with jax.named_scope("step"):
                tn = jnp.minimum(t + 1, NSTEP - 1)
                u_dft(t)
                xb_ref[...] = xn_ref[...]
                g = mlp1(xn_ref, 0, FM)
                glast = jnp.concatenate([g[:, KG[-1][0]:], mlp1_rem(xn_ref)], axis=1)
                b2 = b2_ref[...].astype(f32)[None, :]
                parts, os_ = [], []
                for n in range(NT):
                    cs = slice(n * 128, (n + 1) * 128)
                    acc = b2[:, cs]
                    for k0, k1 in KG:
                        acc = jnp.dot(g[:, k0:k1] if k1 < F else glast, upk(w2p[k0 // 2:k1 // 2, cs]),
                                      preferred_element_type=f32) + acc
                        parts.extend(row_anchors(acc))
                    os_.append(acc)
                mac(t)
                ys = idft()
                kv_block(tn, spread(parts, *la[0], NCH))
                layernorm(tn, xn_ref, spread(parts, *la[1], 16))
                combine(t, ys, os_, xb_ref)
            return carry

        lax.fori_loop(2, NSTEP, body, 0)
        wait("wo", [co(i, c) for i in range(NSTEP) for c in range(NT)])

    consts = dft_mats()

    @jax.jit
    def f(A_q, A_k, A_v, A_shift_k, A_ssm_k, A_ssm_D, B_x, B_w1, B_b1, B_w2, B_b2):
        vm = pltpu.VMEM
        dma = pltpu.SemaphoreType.DMA
        out = pl.pallas_call(
            kern,
            in_specs=[pl.BlockSpec(memory_space=pltpu.SMEM)] + [pl.BlockSpec(memory_space=pl.ANY)] * 11,
            out_specs=pl.BlockSpec(memory_space=pl.ANY),
            out_shape=jax.ShapeDtypeStruct((S, D), bf16),
            scratch_shapes=[
                vm((2 * NB + 2, R8, 3, 8, D), f32), vm((S + 64, D), bf16), vm((S, D), bf16), vm((KVR, D), bf16),
                vm((D, S), bf16), vm((F, D), bf16), vm((F, D), bf16),
                vm((F // 2, D), u32), vm((F // 2, D), u32),
                vm((TM // 2, D), u32), vm((B, 2 * D), u32), vm((TM // 2, D), u32), vm((TM // 2, D), u32),
                vm((TM, D), u32), vm((48, D), f32), vm((64, 128), f32),
                vm((4, D), bf16), vm((D,), bf16), vm((F,), bf16), vm((D,), bf16), vm((3 * B, B), bf16),
                dma((NSTEP - 2,)), dma((4,)), dma((2,)), dma(()), pltpu.SemaphoreType.REGULAR,
            ],
            compiler_params=pltpu.CompilerParams(
                vmem_limit_bytes=110 * 1024 * 1024,
                disable_bounds_checks=not checks, disable_semaphore_checks=not checks),
        )(jnp.zeros((1,), jnp.int32), A_q.reshape(S, D), A_k.reshape(S, D), A_v.reshape(S, D), A_ssm_k,
          B_w1.T, B_w2, A_shift_k.T, A_ssm_D, B_b1, B_b2, jnp.asarray(consts, bf16))
        return out.reshape(1, S, D)

    return f


_impl = make()


@jax.jit
def pallas_parallel_sum__ssm_conv_h3__dense_activation_gelu__prompt_kernel(
    A_q, A_k, A_v, A_shift_k, A_ssm_k, A_ssm_D, B_x, B_w1, B_b1, B_w2, B_b2
):
    return _impl(A_q, A_k, A_v, A_shift_k, A_ssm_k, A_ssm_D, B_x, B_w1, B_b1, B_w2, B_b2)
```

```python
import itertools

import jax
import jax.numpy as jnp
import numpy as np
from jax import lax
from jax.experimental import pallas as pl
from jax.experimental.pallas import tpu as pltpu

S, D, F = 2048, 640, 1728
B = 128
NB = S // B
TM = 256
NSTEP = S // TM
NT = D // 128
R8 = B // 8
HB = B // 2
FM = 1664
KG = [(k0, min(F, k0 + 512)) for k0 in range(0, F, 512)]
Z, DUM, H0 = NB, NB + 1, NB + 2
KO, VO, FO, KVR = 16, 16 + S, 16 + 2 * S, 2 * S + 64
f32, bf16, u32 = jnp.float32, jnp.bfloat16, jnp.uint32
NT_DIMS = (((1,), (1,)), ((), ()))


def dft_mats():
    k = np.concatenate([np.arange(0, B, 2), np.arange(1, B, 2)]).astype(np.float64) + 0.5
    n = np.arange(B, dtype=np.float64)
    c = (B - 1) / 2
    th = 2 * np.pi * np.outer(k, n - c / 2) / (2 * B)
    ph = 2 * np.pi * np.outer(k, n - c) / (2 * B)
    fwd = np.stack([np.cos(th).reshape(R8, 8, B), -np.sin(th).reshape(R8, 8, B)], axis=1).reshape(2 * B, B)
    inv = np.concatenate([np.cos(ph).T[:HB], np.sin(ph).T[:HB]], 0) / B
    return np.concatenate([fwd, inv], 0).astype(np.float32)


def pk(x):
    return pltpu.bitcast(x, u32)


def upk(x):
    return pltpu.bitcast(x, bf16)


def row_anchors(val, n=16):
    return [val[r * 16:r * 16 + 8] for r in range(n)]


def spread(parts, lo, hi, n):
    return [parts[lo + (i * (hi - lo)) // n] for i in range(n)]


def make(w1b=(0, 256, 512, 1408, 1728), nh1=3, la=((112, 200), (205, 260)),
         ra=((20, 180), (80, 225), (60, 300), (8, 60)), fsd=(1, 1), checks=False, KVROWS=16, NLN=8, r1=0):
    NCH = NT * TM // KVROWS
    W1C = list(zip(w1b[:-1], w1b[1:]))
    W2C = [(0, 512), (512, F)]

    def kern(z_ref, x_hbm, k_hbm, v_hbm, h_hbm, w1_hbm, w2_hbm, sk_hbm, sD_hbm, b1_hbm, b2_hbm, C_hbm,
             o_hbm,
             UH, x_v, o_v, KV, h_v, w1_v, w2_v, w1p, w2p, kvb_ref, Q_ref, xn_ref, xb_ref, x2_ref,
             skb_ref, b1c_ref, sk_ref, sD_ref, b1_ref, b2_ref, C_ref,
             sem_t, sem_a, sem_b, sem_o, sem_bar):
        F_ref, G_ref = C_ref.at[0:2 * B], C_ref.at[2 * B:3 * B]
        static = lambda i: isinstance(i, int)
        al = lambda i, m: i if static(i) else pl.multiple_of(i, m)
        rows = lambda i: pl.ds(al(i * TM, TM), TM)

        def copy(src, dst, sem):
            return pltpu.make_async_copy(src, dst, sem)

        xsem = lambda i: sem_a.at[i] if static(i) and i < 2 else sem_t.at[i - 2]
        ksem = lambda i: sem_b.at[i] if static(i) and i < 2 else sem_t.at[i - 2]
        cx = lambda i: copy(x_hbm.at[rows(i)], x_v.at[rows(i)], xsem(i))
        ck = lambda i: copy(k_hbm.at[rows(i)], KV.at[pl.ds(al(KO + i * TM, 16), TM)], ksem(i))
        cv = lambda i: copy(v_hbm.at[rows(i)], KV.at[pl.ds(al(VO + i * TM, 16), TM)], ksem(i))
        ch = lambda c: copy(h_hbm.at[c * 128:(c + 1) * 128], h_v.at[c * 128:(c + 1) * 128],
                            sem_a.at[3] if c < nh1 else sem_b.at[0])
        cw1 = lambda i: copy(w1_hbm.at[W1C[i][0]:W1C[i][1]], w1_v.at[W1C[i][0]:W1C[i][1]], sem_a.at[i])
        cw2 = lambda i: copy(w2_hbm.at[W2C[i][0]:W2C[i][1]], w2_v.at[W2C[i][0]:W2C[i][1]], sem_b.at[i])
        co = lambda i, c: copy(o_v.at[rows(i), c * 128:(c + 1) * 128], o_hbm.at[rows(i), c * 128:(c + 1) * 128], sem_o)
        cF = copy(C_hbm.at[0:2 * B], F_ref, sem_a.at[3])
        cG = copy(C_hbm.at[2 * B:3 * B], G_ref, sem_b.at[1])
        cD = copy(sD_hbm, sD_ref, sem_a.at[3])
        csk = copy(sk_hbm, sk_ref, sem_b.at[0])
        cb1 = copy(b1_hbm, b1_ref, sem_a.at[0])
        cb2 = copy(b2_hbm, b2_ref, sem_b.at[0])

        def wait(name, copies):
            with jax.named_scope(name):
                for cp in copies:
                    cp.wait()

        def bar():
            pl.semaphore_signal(sem_bar, 1)
            pl.semaphore_wait(sem_bar, 1)

        g1, g2, g3 = [cx(0), cb1, cw1(0)], [cx(1), cw1(1)], [cw1(2)]
        g4 = [cw1(3), cF, cD] + [ch(c) for c in range(nh1)]
        g5 = [ch(c) for c in range(nh1, NT)] + [cb2, cw2(0), csk, ck(0), cv(0)]
        g6 = [cw2(1), cG, ck(1), cv(1)]
        blk = lambda i: [cx(i), ck(i), cv(i)]
        for cp in g1 + g2 + g3 + g4 + g5:
            cp.start()
            bar()
        for i, grp in enumerate([g6] + [blk(i) for i in range(2, NSTEP)]):
            for cp in grp:
                cp.start()
            if i in (0, 1, 2, 4):
                bar()

        zero = jnp.clip(z_ref[0], 0, 1)
        never = jnp.full((8, 128), zero, jnp.int32) != 0
        KV[0:16, :] = jnp.zeros((16, D), bf16)
        UH[Z] = jnp.zeros(UH.shape[1:], f32)

        def kv_block(t, anchors):
            nrc = TM // KVROWS
            for c in range(NT):
                cs = slice(c * 128, (c + 1) * 128)
                skb_ref[pl.ds(pl.multiple_of(32 + zero * 8, 8), 8), 0:128] = anchors[c * nrc]
                sk = [jnp.concatenate([skb_ref[8 * j:8 * j + 8, cs]] * (KVROWS // 8), axis=0) for j in range(4)]
                for rc in range(nrc):
                    KV[pl.ds(pl.multiple_of(FO + zero * 16, 16), 8), 0:128] = anchors[c * nrc + rc].astype(bf16)
                    r0 = t * TM + rc * KVROWS
                    vv = KV[pl.ds(al(r0 + VO, 16), KVROWS), cs].astype(f32)
                    kext = KV[pl.ds(al(r0, 16), KVROWS + 16), cs].astype(f32)[8:]
                    ks = kext[8:] * sk[0]
                    for j in range(1, 4):
                        ks = ks + pltpu.roll(kext, j, 0)[8:, :] * sk[j]
                    kvb_ref[rc * KVROWS // 2:(rc + 1) * KVROWS // 2, cs] = pk((ks * vv).astype(bf16))

        def u_dft(t):
            fm = F_ref[...]
            for j in range(2):
                u = jnp.dot(fm, upk(kvb_ref[j * HB:(j + 1) * HB, :]), preferred_element_type=f32)
                u = u.reshape(R8, 2, 8, D)
                a, b = u[:, 0], u[:, 1]
                UH[2 * t + j, :, 0] = a + b
                UH[2 * t + j, :, 1] = a
                UH[2 * t + j, :, 2] = b
            return b[R8 - 1, :, D - 128:]

        def h_rounds(c):
            cs = slice(c * 128, (c + 1) * 128)
            hp_re = hp_im = None
            for a in range(NB):
                fm = F_ref[...]
                hh = lax.dot_general(fm, h_v[cs, a * B:(a + 1) * B], NT_DIMS, preferred_element_type=f32)
                if a == 0:
                    hh = hh + fm[:, 0:1].astype(f32) * sD_ref[...].astype(f32)[None, cs]
                h4 = hh.reshape(R8, 2, 8, 128)
                hre, him = h4[:, 0], h4[:, 1]
                if a == 0:
                    c_, d_ = hre, him
                else:
                    e = R8 // 2
                    c_ = jnp.concatenate([hre[:e] - hp_im[:e], hre[e:] + hp_im[e:]], axis=0)
                    d_ = jnp.concatenate([him[:e] + hp_re[:e], him[e:] - hp_re[e:]], axis=0)
                UH[H0 + a, :, 0, :, cs] = c_
                UH[H0 + a, :, 1, :, cs] = d_ - c_
                UH[H0 + a, :, 2, :, cs] = c_ + d_
                hp_re, hp_im = hre, him
                if a % 4 == 3:
                    yield hh

        def layernorm(t, dst, anchors=None):
            n = 1 if anchors is None else len(anchors)
            rr = TM // n
            for i in range(n):
                if anchors is not None:
                    x_v[pl.ds(pl.multiple_of(S + zero * 16, 16), 8), 0:128] = anchors[i].astype(bf16)
                x = x_v[pl.ds(al(t * TM + i * rr, 16), rr), :].astype(f32)
                m = jnp.mean(x, axis=-1, keepdims=True)
                xc = x - m
                var = jnp.mean(xc * xc, axis=-1, keepdims=True)
                xn = xc * lax.rsqrt(var + 1e-5)
                dst[i * rr // 2:(i + 1) * rr // 2, :] = pk(xn.astype(bf16))

        c1 = np.float32(2 * np.sqrt(2 / np.pi))
        c2 = np.float32(8 * np.sqrt(2 / np.pi) * 0.044715)

        def gelu(h):
            return (h + h * jnp.tanh(h * (c1 + c2 * (h * h)))).astype(bf16)

        def mlp1(xr, lo, hi):
            b1 = b1_ref[...].astype(f32)[None, :] * 0.5
            h = lax.dot_general(upk(xr[...]), upk(w1p[lo // 2:hi // 2, :]), NT_DIMS, preferred_element_type=f32)
            return gelu(h + b1[:, lo:hi])

        def mlp1_rem(xr):
            ht = lax.dot_general(upk(w1p[FM // 2:, :]), upk(xr[...]), NT_DIMS, preferred_element_type=f32)
            return gelu(ht + jnp.concatenate([b1c_ref[...]] * (ht.shape[1] // 128), axis=1)).T

        def mac(t, anchor=None, depth=0):
            if anchor is not None:
                UH[DUM, zero, 0, :, 0:128] = anchor
            if static(t):
                uslot = [2 * t + 1 - l for l in range(2 * t + 2)]
            else:
                uslot = [2 * t + 1 - l if l < 6 else jnp.where(2 * t + 1 - l >= 0, 2 * t + 1 - l, Z)
                         for l in range(NB)]
            nlag = len(uslot)
            pend = []
            for ci in range(NT):
                cs = slice(ci * 128, (ci + 1) * 128)
                for r2 in range(0, R8, 2):
                    ld = lambda s: [UH[s, r2:r2 + 2, c_, :, cs].reshape(16, 128) for c_ in range(3)]
                    add = lambda acc, p: p if acc is None else [x_ + y_ for x_, y_ in zip(acc, p)]
                    acc0 = acc1 = None
                    ucur = ld(uslot[0])
                    for l in range(nlag):
                        hv = ld(H0 + l)
                        p1 = [hv[c_] * ucur[c_] for c_ in range(3)]
                        if l + 1 < nlag:
                            ucur = ld(uslot[l + 1])
                            acc0 = add(acc0, [hv[c_] * ucur[c_] for c_ in range(3)])
                        acc1 = add(acc1, p1)
                    w = []
                    for acc in (acc0, acc1):
                        w.append(pk((acc[0] - acc[2]).astype(bf16)))
                        w.append(pk((acc[0] + acc[1]).astype(bf16)))
                    tie = (w[0] | w[1]) | (w[2] | w[3])
                    w = [jnp.where(never, tie, w_) for w_ in w]
                    if depth:
                        pend.append(tie)
                        if len(pend) >= depth:
                            UH[DUM, zero, 0, :, 0:128] = pltpu.bitcast(pend.pop(0), f32)
                    for j in range(2):
                        col = slice(ci * 256 + j * 128, ci * 256 + (j + 1) * 128)
                        Q_ref[r2 * 4:r2 * 4 + 8, col] = w[2 * j]
                        Q_ref[HB + r2 * 4:HB + r2 * 4 + 8, col] = w[2 * j + 1]

        def idft():
            flip = 7 - lax.broadcasted_iota(jnp.int32, (8, 128), 0)
            ys = []
            for c in range(NT):
                qs = slice(c * 256, (c + 1) * 256)
                cc = jnp.dot(G_ref[0:HB, :], upk(Q_ref[0:HB, qs]), preferred_element_type=f32)
                ss = jnp.dot(G_ref[HB:, :], upk(Q_ref[HB:, qs]), preferred_element_type=f32)
                lo, hi = cc - ss, cc + ss
                pieces = []
                for j in range(2):
                    js = slice(j * 128, (j + 1) * 128)
                    pieces.append(lo[:, js])
                    pieces += [jnp.take_along_axis(hi[r * 8:(r + 1) * 8, js], flip, axis=0)
                               for r in reversed(range(HB // 8))]
                ys.append(jnp.concatenate(pieces, axis=0))
            return ys

        def combine(t, ys, os_, xb):
            for c in range(NT):
                cs = slice(c * 128, (c + 1) * 128)
                out = (upk(xb[:, cs]).astype(f32) * ys[c] + os_[c]) + x_v[rows(t), cs].astype(f32)
                o_v[rows(t), cs] = out.astype(bf16)
                co(t, c).start()

        G = {}

        def mlp1_piece(q0, q1, n0, n1, split):
            for q in range(q0, q1, split):
                g_ = mlp1(x2_ref.at[q * 64:(q + split) * 64], n0 * 128, n1 * 128)
                for qq in range(split):
                    for n in range(n0, n1):
                        G[(q + qq, n)] = g_[qq * 128:(qq + 1) * 128, (n - n0) * 128:(n - n0 + 1) * 128]

        def w1_load(i):
            lo, hi = W1C[i]
            w1p[lo // 2:hi // 2, :] = pk((w1_v[lo:hi, :].astype(f32) * 0.5).astype(bf16))

        n1, n2, n3 = (W1C[i][1] // 128 for i in range(3))
        wait("w1", g1)
        w1_load(0)
        if r1 == 0:
            layernorm(0, x2_ref.at[0:TM // 2])
            for q in range(2):
                for n in range(n1):
                    mlp1_piece(q, q + 1, n, n + 1, 1)
        elif r1 == 1:
            layernorm(0, x2_ref.at[0:TM // 2])
            for n in range(n1):
                for q in range(2):
                    mlp1_piece(q, q + 1, n, n + 1, 1)
        elif r1 == 2:
            layernorm(0, x2_ref.at[0:TM // 2])
            mlp1_piece(0, 2, 0, n1, 1)

        wait("w2", g2)
        w1_load(1)
        mlp1_piece(0, 2, n1, n2, 1)
        layernorm(1, x2_ref.at[TM // 2:TM])
        mlp1_piece(2, 4, 0, n2, 2)

        wait("w3", g3)
        w1_load(2)
        b1t = jnp.broadcast_to(b1_ref[...].astype(f32)[None, F - 128:], (128, 128)).T
        b1c_ref[...] = b1t[64:] * 0.5
        e = n3 - (n3 - n2) % 4
        mlp1_piece(0, 4, n2, e, 4)
        for n in range(e, n3, 2):
            mlp1_piece(0, 4, n, min(n + 2, n3), 2 if n + 2 <= n3 else 1)

        wait("w4", g4)
        w1_load(3)
        gr = mlp1_rem(x2_ref)
        rounds = itertools.chain(*[h_rounds(c) for c in range(nh1)])
        pieces = [(q, n) for n in range(n3, FM // 128) for q in range(4)]
        done = 0
        for i, (q, n) in enumerate(pieces):
            for _ in range((i + 1) * 4 * nh1 // len(pieces) - done):
                next(rounds)
                done += 1
            mlp1_piece(q, q + 1, n, n + 1, 1)

        wait("w5", g5)
        skf = sk_ref[...].astype(f32)
        for j in range(4):
            skb_ref[8 * j:8 * j + 8, :] = jnp.broadcast_to(skf[j:j + 1, :], (8, D))
        b2 = b2_ref[...].astype(f32)[None, :]
        parts = []

        def gslice(qs, k0, k1):
            rws = []
            for q in qs:
                tiles = [G[(q, n)] for n in range(k0 // 128, min(k1, FM) // 128)]
                if k1 > FM:
                    tiles.append(gr[q * 128:(q + 1) * 128])
                rws.append(jnp.concatenate(tiles, axis=1))
            return jnp.concatenate(rws, axis=0)

        def mmk(qs, n, k0, k1, acc, fresh):
            cs = slice(n * 128, (n + 1) * 128)
            if fresh:
                w2 = w2_v[k0:k1, cs]
                w2p[k0 // 2:k1 // 2, cs] = pk(w2)
            else:
                w2 = upk(w2p[k0 // 2:k1 // 2, cs])
            acc = jnp.dot(gslice(qs, k0, k1), w2, preferred_element_type=f32) + (b2[:, cs] if acc is None else acc)
            parts.extend(row_anchors(acc, 8 * len(qs)))
            return acc

        rounds = itertools.chain(*[h_rounds(c) for c in range(nh1, NT)])
        nr = 4 * (NT - nh1)
        o0 = []
        done = 0
        for i in range(2 * NT):
            for _ in range(min(nr, ((i + 1) * nr + 2 * NT - 2) // (2 * NT - 1)) - done):
                parts.extend(row_anchors(next(rounds)))
                done += 1
            o0.append(mmk([i % 2], i // 2, *KG[0], None, i % 2 == 0))
        o0 = [jnp.concatenate(o0[2 * n:2 * n + 2], axis=0) for n in range(NT)]
        kv_block(0, spread(parts, *ra[0], NCH))

        wait("w6", g6)
        parts.clear()
        rest = [(n, g) for n in range(NT) for g in KG[1:]]
        ul = u_dft(0)
        for n, g in rest[:11]:
            o0[n] = mmk([0, 1], n, *g, o0[n], True)
        mac(0, ul, fsd[0])
        ys = idft()
        for n, g in rest[11:]:
            o0[n] = mmk([0, 1], n, *g, o0[n], True)
        kv_block(1, spread(parts, *ra[1], NCH))
        combine(0, ys, o0, x2_ref.at[0:TM // 2])

        wait("w7", blk(2))
        parts.clear()
        rest = [(n, g) for n in range(NT) for g in KG]
        o1 = [None] * NT
        ul = u_dft(1)
        for n, g in rest[:15]:
            o1[n] = mmk([2, 3], n, *g, o1[n], False)
        mac(1, ul, fsd[1])
        ys = idft()
        for n, g in rest[15:]:
            o1[n] = mmk([2, 3], n, *g, o1[n], False)
        layernorm(2, xn_ref, spread(parts, *ra[3], NLN))
        kv_block(2, spread(parts, *ra[2], NCH))
        combine(1, ys, o1, x2_ref.at[TM // 2:TM])

        def body(t, carry):
            @pl.when(t + 1 < NSTEP)
            def _():
                wait("lw", blk(t + 1))

            with jax.named_scope("step"):
                tn = jnp.minimum(t + 1, NSTEP - 1)
                u_dft(t)
                xb_ref[...] = xn_ref[...]
                g = mlp1(xn_ref, 0, FM)
                glast = jnp.concatenate([g[:, KG[-1][0]:], mlp1_rem(xn_ref)], axis=1)
                b2 = b2_ref[...].astype(f32)[None, :]
                parts, os_ = [], []
                for n in range(NT):
                    cs = slice(n * 128, (n + 1) * 128)
                    acc = b2[:, cs]
                    for k0, k1 in KG:
                        acc = jnp.dot(g[:, k0:k1] if k1 < F else glast, upk(w2p[k0 // 2:k1 // 2, cs]),
                                      preferred_element_type=f32) + acc
                        parts.extend(row_anchors(acc))
                    os_.append(acc)
                mac(t)
                ys = idft()
                kv_block(tn, spread(parts, *la[0], NCH))
                layernorm(tn, xn_ref, spread(parts, *la[1], NLN))
                combine(t, ys, os_, xb_ref)
            return carry

        lax.fori_loop(2, NSTEP, body, 0)
        wait("wo", [co(i, c) for i in range(NSTEP) for c in range(NT)])

    consts = dft_mats()

    @jax.jit
    def f(A_q, A_k, A_v, A_shift_k, A_ssm_k, A_ssm_D, B_x, B_w1, B_b1, B_w2, B_b2):
        vm = pltpu.VMEM
        dma = pltpu.SemaphoreType.DMA
        out = pl.pallas_call(
            kern,
            in_specs=[pl.BlockSpec(memory_space=pltpu.SMEM)] + [pl.BlockSpec(memory_space=pl.ANY)] * 11,
            out_specs=pl.BlockSpec(memory_space=pl.ANY),
            out_shape=jax.ShapeDtypeStruct((S, D), bf16),
            scratch_shapes=[
                vm((2 * NB + 2, R8, 3, 8, D), f32), vm((S + 64, D), bf16), vm((S, D), bf16), vm((KVR, D), bf16),
                vm((D, S), bf16), vm((F, D), bf16), vm((F, D), bf16),
                vm((F // 2, D), u32), vm((F // 2, D), u32),
                vm((TM // 2, D), u32), vm((B, 2 * D), u32), vm((TM // 2, D), u32), vm((TM // 2, D), u32),
                vm((TM, D), u32), vm((48, D), f32), vm((64, 128), f32),
                vm((4, D), bf16), vm((D,), bf16), vm((F,), bf16), vm((D,), bf16), vm((3 * B, B), bf16),
                dma((NSTEP - 2,)), dma((4,)), dma((2,)), dma(()), pltpu.SemaphoreType.REGULAR,
            ],
            compiler_params=pltpu.CompilerParams(
                vmem_limit_bytes=110 * 1024 * 1024,
                disable_bounds_checks=not checks, disable_semaphore_checks=not checks),
        )(jnp.zeros((1,), jnp.int32), A_q.reshape(S, D), A_k.reshape(S, D), A_v.reshape(S, D), A_ssm_k,
          B_w1.T, B_w2, A_shift_k.T, A_ssm_D, B_b1, B_b2, jnp.asarray(consts, bf16))
        return out.reshape(1, S, D)

    return f


_impl = make()


@jax.jit
def pallas_parallel_sum__ssm_conv_h3__dense_activation_gelu__prompt_kernel(
    A_q, A_k, A_v, A_shift_k, A_ssm_k, A_ssm_D, B_x, B_w1, B_b1, B_w2, B_b2
):
    return _impl(A_q, A_k, A_v, A_shift_k, A_ssm_k, A_ssm_D, B_x, B_w1, B_b1, B_w2, B_b2)
```

```python
import itertools

import jax
import jax.numpy as jnp
import numpy as np
from jax import lax
from jax.experimental import pallas as pl
from jax.experimental.pallas import tpu as pltpu

S, D, F = 2048, 640, 1728
B = 128
NB = S // B
TM = 256
NSTEP = S // TM
NT = D // 128
R8 = B // 8
HB = B // 2
FM = 1664
KG = [(k0, min(F, k0 + 512)) for k0 in range(0, F, 512)]
Z, DUM, H0 = NB, NB + 1, NB + 2
KO, VO, FO, KVR = 16, 16 + S, 16 + 2 * S, 2 * S + 64
f32, bf16, u32 = jnp.float32, jnp.bfloat16, jnp.uint32
NT_DIMS = (((1,), (1,)), ((), ()))


def dft_mats():
    k = np.concatenate([np.arange(0, B, 2), np.arange(1, B, 2)]).astype(np.float64) + 0.5
    n = np.arange(B, dtype=np.float64)
    c = (B - 1) / 2
    th = 2 * np.pi * np.outer(k, n - c / 2) / (2 * B)
    ph = 2 * np.pi * np.outer(k, n - c) / (2 * B)
    fwd = np.stack([np.cos(th).reshape(R8, 8, B), -np.sin(th).reshape(R8, 8, B)], axis=1).reshape(2 * B, B)
    inv = np.concatenate([np.cos(ph).T[:HB], np.sin(ph).T[:HB]], 0) / B
    return np.concatenate([fwd, inv], 0).astype(np.float32)


def pk(x):
    return pltpu.bitcast(x, u32)


def upk(x):
    return pltpu.bitcast(x, bf16)


def row_anchors(val, n=16):
    return [val[r * 16:r * 16 + 8] for r in range(n)]


def spread(parts, lo, hi, n):
    return [parts[lo + (i * (hi - lo)) // n] for i in range(n)]


def make(w1b=(0, 256, 512, 1408, 1728), nh1=3, la=((112, 200), (205, 250)),
         ra=((20, 200), (75, 220), (70, 305), (8, 50)), fsd=(1, 1), checks=False, KVROWS=16, NLN=(8, 4)):
    NCH = NT * TM // KVROWS
    W1C = list(zip(w1b[:-1], w1b[1:]))
    W2C = [(0, 512), (512, F)]

    def kern(z_ref, x_hbm, k_hbm, v_hbm, h_hbm, w1_hbm, w2_hbm, sk_hbm, sD_hbm, b1_hbm, b2_hbm, C_hbm,
             o_hbm,
             UH, x_v, o_v, KV, h_v, w1_v, w2_v, w1p, w2p, kvb_ref, Q_ref, xn_ref, xb_ref, x2_ref,
             skb_ref, b1c_ref, sk_ref, sD_ref, b1_ref, b2_ref, C_ref,
             sem_t, sem_a, sem_b, sem_o, sem_bar):
        F_ref, G_ref = C_ref.at[0:2 * B], C_ref.at[2 * B:3 * B]
        static = lambda i: isinstance(i, int)
        al = lambda i, m: i if static(i) else pl.multiple_of(i, m)
        rows = lambda i: pl.ds(al(i * TM, TM), TM)

        def copy(src, dst, sem):
            return pltpu.make_async_copy(src, dst, sem)

        xsem = lambda i: sem_a.at[i] if static(i) and i < 2 else sem_t.at[i - 2]
        ksem = lambda i: sem_b.at[i] if static(i) and i < 2 else sem_t.at[i - 2]
        cx = lambda i: copy(x_hbm.at[rows(i)], x_v.at[rows(i)], xsem(i))
        ck = lambda i: copy(k_hbm.at[rows(i)], KV.at[pl.ds(al(KO + i * TM, 16), TM)], ksem(i))
        cv = lambda i: copy(v_hbm.at[rows(i)], KV.at[pl.ds(al(VO + i * TM, 16), TM)], ksem(i))
        ch = lambda c: copy(h_hbm.at[c * 128:(c + 1) * 128], h_v.at[c * 128:(c + 1) * 128],
                            sem_a.at[3] if c < nh1 else sem_b.at[0])
        cw1 = lambda i: copy(w1_hbm.at[W1C[i][0]:W1C[i][1]], w1_v.at[W1C[i][0]:W1C[i][1]], sem_a.at[i])
        cw2 = lambda i: copy(w2_hbm.at[W2C[i][0]:W2C[i][1]], w2_v.at[W2C[i][0]:W2C[i][1]], sem_b.at[i])
        co = lambda i, c: copy(o_v.at[rows(i), c * 128:(c + 1) * 128], o_hbm.at[rows(i), c * 128:(c + 1) * 128], sem_o)
        cF = copy(C_hbm.at[0:2 * B], F_ref, sem_a.at[3])
        cG = copy(C_hbm.at[2 * B:3 * B], G_ref, sem_b.at[1])
        cD = copy(sD_hbm, sD_ref, sem_a.at[3])
        csk = copy(sk_hbm, sk_ref, sem_b.at[0])
        cb1 = copy(b1_hbm, b1_ref, sem_a.at[0])
        cb2 = copy(b2_hbm, b2_ref, sem_b.at[0])

        def wait(name, copies):
            with jax.named_scope(name):
                for cp in copies:
                    cp.wait()

        def bar():
            pl.semaphore_signal(sem_bar, 1)
            pl.semaphore_wait(sem_bar, 1)

        g1, g2, g3 = [cx(0), cb1, cw1(0)], [cx(1), cw1(1)], [cw1(2)]
        g4 = [cw1(3), cF, cD] + [ch(c) for c in range(nh1)]
        g5 = [ch(c) for c in range(nh1, NT)] + [cb2, cw2(0), csk, ck(0), cv(0)]
        g6 = [cw2(1), cG, ck(1), cv(1)]
        blk = lambda i: [cx(i), ck(i), cv(i)]
        for cp in g1 + g2 + g3 + g4 + g5:
            cp.start()
            bar()
        for i, grp in enumerate([g6] + [blk(i) for i in range(2, NSTEP)]):
            for cp in grp:
                cp.start()
            if i in (0, 1, 2, 4):
                bar()

        zero = jnp.clip(z_ref[0], 0, 1)
        never = jnp.full((8, 128), zero, jnp.int32) != 0
        KV[0:16, :] = jnp.zeros((16, D), bf16)
        UH[Z] = jnp.zeros(UH.shape[1:], f32)

        def kv_block(t, anchors):
            nrc = TM // KVROWS
            for c in range(NT):
                cs = slice(c * 128, (c + 1) * 128)
                skb_ref[pl.ds(pl.multiple_of(32 + zero * 8, 8), 8), 0:128] = anchors[c * nrc]
                sk = [jnp.concatenate([skb_ref[8 * j:8 * j + 8, cs]] * (KVROWS // 8), axis=0) for j in range(4)]
                for rc in range(nrc):
                    KV[pl.ds(pl.multiple_of(FO + zero * 16, 16), 8), 0:128] = anchors[c * nrc + rc].astype(bf16)
                    r0 = t * TM + rc * KVROWS
                    vv = KV[pl.ds(al(r0 + VO, 16), KVROWS), cs].astype(f32)
                    kext = KV[pl.ds(al(r0, 16), KVROWS + 16), cs].astype(f32)[8:]
                    ks = kext[8:] * sk[0]
                    for j in range(1, 4):
                        ks = ks + pltpu.roll(kext, j, 0)[8:, :] * sk[j]
                    kvb_ref[rc * KVROWS // 2:(rc + 1) * KVROWS // 2, cs] = pk((ks * vv).astype(bf16))

        def u_dft(t):
            fm = F_ref[...]
            for j in range(2):
                u = jnp.dot(fm, upk(kvb_ref[j * HB:(j + 1) * HB, :]), preferred_element_type=f32)
                u = u.reshape(R8, 2, 8, D)
                a, b = u[:, 0], u[:, 1]
                UH[2 * t + j, :, 0] = a + b
                UH[2 * t + j, :, 1] = a
                UH[2 * t + j, :, 2] = b
            return b[R8 - 1, :, D - 128:]

        def h_rounds(c):
            cs = slice(c * 128, (c + 1) * 128)
            hp_re = hp_im = None
            for a in range(NB):
                fm = F_ref[...]
                hh = lax.dot_general(fm, h_v[cs, a * B:(a + 1) * B], NT_DIMS, preferred_element_type=f32)
                if a == 0:
                    hh = hh + fm[:, 0:1].astype(f32) * sD_ref[...].astype(f32)[None, cs]
                h4 = hh.reshape(R8, 2, 8, 128)
                hre, him = h4[:, 0], h4[:, 1]
                if a == 0:
                    c_, d_ = hre, him
                else:
                    e = R8 // 2
                    c_ = jnp.concatenate([hre[:e] - hp_im[:e], hre[e:] + hp_im[e:]], axis=0)
                    d_ = jnp.concatenate([him[:e] + hp_re[:e], him[e:] - hp_re[e:]], axis=0)
                UH[H0 + a, :, 0, :, cs] = c_
                UH[H0 + a, :, 1, :, cs] = d_ - c_
                UH[H0 + a, :, 2, :, cs] = c_ + d_
                hp_re, hp_im = hre, him
                if a % 4 == 3:
                    yield hh

        def layernorm(t, dst, anchors=None):
            n = 1 if anchors is None else len(anchors)
            rr = TM // n
            for i in range(n):
                if anchors is not None:
                    x_v[pl.ds(pl.multiple_of(S + zero * 16, 16), 8), 0:128] = anchors[i].astype(bf16)
                x = x_v[pl.ds(al(t * TM + i * rr, 16), rr), :].astype(f32)
                m = jnp.mean(x, axis=-1, keepdims=True)
                xc = x - m
                var = jnp.mean(xc * xc, axis=-1, keepdims=True)
                xn = xc * lax.rsqrt(var + 1e-5)
                dst[i * rr // 2:(i + 1) * rr // 2, :] = pk(xn.astype(bf16))

        c1 = np.float32(2 * np.sqrt(2 / np.pi))
        c2 = np.float32(8 * np.sqrt(2 / np.pi) * 0.044715)

        def gelu(h):
            return (h + h * jnp.tanh(h * (c1 + c2 * (h * h)))).astype(bf16)

        def mlp1(xr, lo, hi):
            b1 = b1_ref[...].astype(f32)[None, :] * 0.5
            h = lax.dot_general(upk(xr[...]), upk(w1p[lo // 2:hi // 2, :]), NT_DIMS, preferred_element_type=f32)
            return gelu(h + b1[:, lo:hi])

        def mlp1_rem(xr):
            ht = lax.dot_general(upk(w1p[FM // 2:, :]), upk(xr[...]), NT_DIMS, preferred_element_type=f32)
            return gelu(ht + jnp.concatenate([b1c_ref[...]] * (ht.shape[1] // 128), axis=1)).T

        def mac(t, anchor=None, depth=0):
            if anchor is not None:
                UH[DUM, zero, 0, :, 0:128] = anchor
            if static(t):
                uslot = [2 * t + 1 - l for l in range(2 * t + 2)]
            else:
                uslot = [2 * t + 1 - l if l < 6 else jnp.where(2 * t + 1 - l >= 0, 2 * t + 1 - l, Z)
                         for l in range(NB)]
            nlag = len(uslot)
            pend = []
            for ci in range(NT):
                cs = slice(ci * 128, (ci + 1) * 128)
                for r2 in range(0, R8, 2):
                    ld = lambda s: [UH[s, r2:r2 + 2, c_, :, cs].reshape(16, 128) for c_ in range(3)]
                    add = lambda acc, p: p if acc is None else [x_ + y_ for x_, y_ in zip(acc, p)]
                    acc0 = acc1 = None
                    ucur = ld(uslot[0])
                    for l in range(nlag):
                        hv = ld(H0 + l)
                        p1 = [hv[c_] * ucur[c_] for c_ in range(3)]
                        if l + 1 < nlag:
                            ucur = ld(uslot[l + 1])
                            acc0 = add(acc0, [hv[c_] * ucur[c_] for c_ in range(3)])
                        acc1 = add(acc1, p1)
                    w = []
                    for acc in (acc0, acc1):
                        w.append(pk((acc[0] - acc[2]).astype(bf16)))
                        w.append(pk((acc[0] + acc[1]).astype(bf16)))
                    tie = (w[0] | w[1]) | (w[2] | w[3])
                    w = [jnp.where(never, tie, w_) for w_ in w]
                    if depth:
                        pend.append(tie)
                        if len(pend) >= depth:
                            UH[DUM, zero, 0, :, 0:128] = pltpu.bitcast(pend.pop(0), f32)
                    for j in range(2):
                        col = slice(ci * 256 + j * 128, ci * 256 + (j + 1) * 128)
                        Q_ref[r2 * 4:r2 * 4 + 8, col] = w[2 * j]
                        Q_ref[HB + r2 * 4:HB + r2 * 4 + 8, col] = w[2 * j + 1]

        def idft():
            flip = 7 - lax.broadcasted_iota(jnp.int32, (8, 128), 0)
            ys = []
            for c in range(NT):
                qs = slice(c * 256, (c + 1) * 256)
                cc = jnp.dot(G_ref[0:HB, :], upk(Q_ref[0:HB, qs]), preferred_element_type=f32)
                ss = jnp.dot(G_ref[HB:, :], upk(Q_ref[HB:, qs]), preferred_element_type=f32)
                lo, hi = cc - ss, cc + ss
                pieces = []
                for j in range(2):
                    js = slice(j * 128, (j + 1) * 128)
                    pieces.append(lo[:, js])
                    pieces += [jnp.take_along_axis(hi[r * 8:(r + 1) * 8, js], flip, axis=0)
                               for r in reversed(range(HB // 8))]
                ys.append(jnp.concatenate(pieces, axis=0))
            return ys

        def combine(t, ys, os_, xb):
            for c in range(NT):
                cs = slice(c * 128, (c + 1) * 128)
                out = (upk(xb[:, cs]).astype(f32) * ys[c] + os_[c]) + x_v[rows(t), cs].astype(f32)
                o_v[rows(t), cs] = out.astype(bf16)
                co(t, c).start()

        G = {}

        def mlp1_piece(q0, q1, n0, n1, split):
            for q in range(q0, q1, split):
                g_ = mlp1(x2_ref.at[q * 64:(q + split) * 64], n0 * 128, n1 * 128)
                for qq in range(split):
                    for n in range(n0, n1):
                        G[(q + qq, n)] = g_[qq * 128:(qq + 1) * 128, (n - n0) * 128:(n - n0 + 1) * 128]

        def w1_load(i):
            lo, hi = W1C[i]
            w1p[lo // 2:hi // 2, :] = pk((w1_v[lo:hi, :].astype(f32) * 0.5).astype(bf16))

        n1, n2, n3 = (W1C[i][1] // 128 for i in range(3))
        wait("w1", g1)
        w1_load(0)
        layernorm(0, x2_ref.at[0:TM // 2])
        for q in range(2):
            for n in range(n1):
                mlp1_piece(q, q + 1, n, n + 1, 1)

        wait("w2", g2)
        w1_load(1)
        mlp1_piece(0, 2, n1, n2, 1)
        layernorm(1, x2_ref.at[TM // 2:TM])
        mlp1_piece(2, 4, 0, n2, 2)

        wait("w3", g3)
        w1_load(2)
        b1t = jnp.broadcast_to(b1_ref[...].astype(f32)[None, F - 128:], (128, 128)).T
        b1c_ref[...] = b1t[64:] * 0.5
        e = n3 - (n3 - n2) % 4
        mlp1_piece(0, 4, n2, e, 4)
        for n in range(e, n3, 2):
            mlp1_piece(0, 4, n, min(n + 2, n3), 2 if n + 2 <= n3 else 1)

        wait("w4", g4)
        w1_load(3)
        gr = mlp1_rem(x2_ref)
        rounds = itertools.chain(*[h_rounds(c) for c in range(nh1)])
        pieces = [(q, n) for n in range(n3, FM // 128) for q in range(4)]
        done = 0
        for i, (q, n) in enumerate(pieces):
            for _ in range((i + 1) * 4 * nh1 // len(pieces) - done):
                next(rounds)
                done += 1
            mlp1_piece(q, q + 1, n, n + 1, 1)

        wait("w5", g5)
        skf = sk_ref[...].astype(f32)
        for j in range(4):
            skb_ref[8 * j:8 * j + 8, :] = jnp.broadcast_to(skf[j:j + 1, :], (8, D))
        b2 = b2_ref[...].astype(f32)[None, :]
        parts = []

        def gslice(qs, k0, k1):
            rws = []
            for q in qs:
                tiles = [G[(q, n)] for n in range(k0 // 128, min(k1, FM) // 128)]
                if k1 > FM:
                    tiles.append(gr[q * 128:(q + 1) * 128])
                rws.append(jnp.concatenate(tiles, axis=1))
            return jnp.concatenate(rws, axis=0)

        def mmk(qs, n, k0, k1, acc, fresh):
            cs = slice(n * 128, (n + 1) * 128)
            if fresh:
                w2 = w2_v[k0:k1, cs]
                w2p[k0 // 2:k1 // 2, cs] = pk(w2)
            else:
                w2 = upk(w2p[k0 // 2:k1 // 2, cs])
            acc = jnp.dot(gslice(qs, k0, k1), w2, preferred_element_type=f32) + (b2[:, cs] if acc is None else acc)
            parts.extend(row_anchors(acc, 8 * len(qs)))
            return acc

        rounds = itertools.chain(*[h_rounds(c) for c in range(nh1, NT)])
        nr = 4 * (NT - nh1)
        o0 = []
        done = 0
        for i in range(2 * NT):
            for _ in range(min(nr, ((i + 1) * nr + 2 * NT - 2) // (2 * NT - 1)) - done):
                parts.extend(row_anchors(next(rounds)))
                done += 1
            o0.append(mmk([i % 2], i // 2, *KG[0], None, i % 2 == 0))
        o0 = [jnp.concatenate(o0[2 * n:2 * n + 2], axis=0) for n in range(NT)]
        kv_block(0, spread(parts, *ra[0], NCH))

        wait("w6", g6)
        parts.clear()
        rest = [(n, g) for n in range(NT) for g in KG[1:]]
        ul = u_dft(0)
        for n, g in rest[:11]:
            o0[n] = mmk([0, 1], n, *g, o0[n], True)
        mac(0, ul, fsd[0])
        ys = idft()
        for n, g in rest[11:]:
            o0[n] = mmk([0, 1], n, *g, o0[n], True)
        kv_block(1, spread(parts, *ra[1], NCH))
        combine(0, ys, o0, x2_ref.at[0:TM // 2])

        wait("w7", blk(2))
        parts.clear()
        rest = [(n, g) for n in range(NT) for g in KG]
        o1 = [None] * NT
        ul = u_dft(1)
        for n, g in rest[:15]:
            o1[n] = mmk([2, 3], n, *g, o1[n], False)
        mac(1, ul, fsd[1])
        ys = idft()
        for n, g in rest[15:]:
            o1[n] = mmk([2, 3], n, *g, o1[n], False)
        layernorm(2, xn_ref, spread(parts, *ra[3], NLN[0]))
        kv_block(2, spread(parts, *ra[2], NCH))
        combine(1, ys, o1, x2_ref.at[TM // 2:TM])

        def body(t, carry):
            @pl.when(t + 1 < NSTEP)
            def _():
                wait("lw", blk(t + 1))

            with jax.named_scope("step"):
                tn = jnp.minimum(t + 1, NSTEP - 1)
                u_dft(t)
                xb_ref[...] = xn_ref[...]
                g = mlp1(xn_ref, 0, FM)
                glast = jnp.concatenate([g[:, KG[-1][0]:], mlp1_rem(xn_ref)], axis=1)
                b2 = b2_ref[...].astype(f32)[None, :]
                parts, os_ = [], []
                for n in range(NT):
                    cs = slice(n * 128, (n + 1) * 128)
                    acc = b2[:, cs]
                    for k0, k1 in KG:
                        acc = jnp.dot(g[:, k0:k1] if k1 < F else glast, upk(w2p[k0 // 2:k1 // 2, cs]),
                                      preferred_element_type=f32) + acc
                        parts.extend(row_anchors(acc))
                    os_.append(acc)
                mac(t)
                ys = idft()
                kv_block(tn, spread(parts, *la[0], NCH))
                layernorm(tn, xn_ref, spread(parts, *la[1], NLN[1]))
                combine(t, ys, os_, xb_ref)
            return carry

        lax.fori_loop(2, NSTEP, body, 0)
        wait("wo", [co(i, c) for i in range(NSTEP) for c in range(NT)])

    consts = dft_mats()

    @jax.jit
    def f(A_q, A_k, A_v, A_shift_k, A_ssm_k, A_ssm_D, B_x, B_w1, B_b1, B_w2, B_b2):
        vm = pltpu.VMEM
        dma = pltpu.SemaphoreType.DMA
        out = pl.pallas_call(
            kern,
            in_specs=[pl.BlockSpec(memory_space=pltpu.SMEM)] + [pl.BlockSpec(memory_space=pl.ANY)] * 11,
            out_specs=pl.BlockSpec(memory_space=pl.ANY),
            out_shape=jax.ShapeDtypeStruct((S, D), bf16),
            scratch_shapes=[
                vm((2 * NB + 2, R8, 3, 8, D), f32), vm((S + 64, D), bf16), vm((S, D), bf16), vm((KVR, D), bf16),
                vm((D, S), bf16), vm((F, D), bf16), vm((F, D), bf16),
                vm((F // 2, D), u32), vm((F // 2, D), u32),
                vm((TM // 2, D), u32), vm((B, 2 * D), u32), vm((TM // 2, D), u32), vm((TM // 2, D), u32),
                vm((TM, D), u32), vm((48, D), f32), vm((64, 128), f32),
                vm((4, D), bf16), vm((D,), bf16), vm((F,), bf16), vm((D,), bf16), vm((3 * B, B), bf16),
                dma((NSTEP - 2,)), dma((4,)), dma((2,)), dma(()), pltpu.SemaphoreType.REGULAR,
            ],
            compiler_params=pltpu.CompilerParams(
                vmem_limit_bytes=110 * 1024 * 1024,
                disable_bounds_checks=not checks, disable_semaphore_checks=not checks),
        )(jnp.zeros((1,), jnp.int32), A_q.reshape(S, D), A_k.reshape(S, D), A_v.reshape(S, D), A_ssm_k,
          B_w1.T, B_w2, A_shift_k.T, A_ssm_D, B_b1, B_b2, jnp.asarray(consts, bf16))
        return out.reshape(1, S, D)

    return f


_impl = make()


@jax.jit
def pallas_parallel_sum__ssm_conv_h3__dense_activation_gelu__prompt_kernel(
    A_q, A_k, A_v, A_shift_k, A_ssm_k, A_ssm_D, B_x, B_w1, B_b1, B_w2, B_b2
):
    return _impl(A_q, A_k, A_v, A_shift_k, A_ssm_k, A_ssm_D, B_x, B_w1, B_b1, B_w2, B_b2)
```

```python
import itertools

import jax
import jax.numpy as jnp
import numpy as np
from jax import lax
from jax.experimental import pallas as pl
from jax.experimental.pallas import tpu as pltpu

S, D, F = 2048, 640, 1728
B = 128
NB = S // B
TM = 256
NSTEP = S // TM
NT = D // 128
R8 = B // 8
HB = B // 2
FM = 1664
KG = [(k0, min(F, k0 + 512)) for k0 in range(0, F, 512)]
Z, DUM, H0 = NB, NB + 1, NB + 2
KO, VO, FO, KVR = 16, 16 + S, 16 + 2 * S, 2 * S + 64
f32, bf16, u32 = jnp.float32, jnp.bfloat16, jnp.uint32
NT_DIMS = (((1,), (1,)), ((), ()))


def dft_mats():
    k = np.concatenate([np.arange(0, B, 2), np.arange(1, B, 2)]).astype(np.float64) + 0.5
    n = np.arange(B, dtype=np.float64)
    c = (B - 1) / 2
    th = 2 * np.pi * np.outer(k, n - c / 2) / (2 * B)
    ph = 2 * np.pi * np.outer(k, n - c) / (2 * B)
    fwd = np.stack([np.cos(th).reshape(R8, 8, B), -np.sin(th).reshape(R8, 8, B)], axis=1).reshape(2 * B, B)
    inv = np.concatenate([np.cos(ph).T[:HB], np.sin(ph).T[:HB]], 0) / B
    return np.concatenate([fwd, inv], 0).astype(np.float32)


def pk(x):
    return pltpu.bitcast(x, u32)


def upk(x):
    return pltpu.bitcast(x, bf16)


def row_anchors(val, n=16):
    return [val[r * 16:r * 16 + 8] for r in range(n)]


def spread(parts, lo, hi, n):
    return [parts[lo + (i * (hi - lo)) // n] for i in range(n)]


def make(w1b=(0, 384, 640, 1536, 1728), nh1=3, la=((112, 200), (205, 250)),
         ra=((20, 210), (75, 220), (60, 290), (8, 50)), fsd=(1, 1), checks=False, KVROWS=16, NLN=(8, 4), npull=1, fs1=11):
    NCH = NT * TM // KVROWS
    W1C = list(zip(w1b[:-1], w1b[1:]))
    W2C = [(0, 512), (512, F)]

    def kern(z_ref, x_hbm, k_hbm, v_hbm, h_hbm, w1_hbm, w2_hbm, sk_hbm, sD_hbm, b1_hbm, b2_hbm, C_hbm,
             o_hbm,
             UH, x_v, o_v, KV, h_v, w1_v, w2_v, w1p, w2p, kvb_ref, Q_ref, xn_ref, xb_ref, x2_ref,
             skb_ref, b1c_ref, sk_ref, sD_ref, b1_ref, b2_ref, C_ref,
             sem_t, sem_a, sem_b, sem_o, sem_bar):
        F_ref, G_ref = C_ref.at[0:2 * B], C_ref.at[2 * B:3 * B]
        static = lambda i: isinstance(i, int)
        al = lambda i, m: i if static(i) else pl.multiple_of(i, m)
        rows = lambda i: pl.ds(al(i * TM, TM), TM)

        def copy(src, dst, sem):
            return pltpu.make_async_copy(src, dst, sem)

        xsem = lambda i: sem_a.at[4 - 3 * i] if static(i) and i < 2 else sem_t.at[i - 2]
        ksem = lambda i: sem_b.at[i] if static(i) and i < 2 else sem_t.at[i - 2]
        cx = lambda i: copy(x_hbm.at[rows(i)], x_v.at[rows(i)], xsem(i))
        ck = lambda i: copy(k_hbm.at[rows(i)], KV.at[pl.ds(al(KO + i * TM, 16), TM)], ksem(i))
        cv = lambda i: copy(v_hbm.at[rows(i)], KV.at[pl.ds(al(VO + i * TM, 16), TM)], ksem(i))
        ch = lambda c: copy(h_hbm.at[c * 128:(c + 1) * 128], h_v.at[c * 128:(c + 1) * 128],
                            sem_a.at[3] if c < nh1 else sem_b.at[0])
        cw1 = lambda i: copy(w1_hbm.at[W1C[i][0]:W1C[i][1]], w1_v.at[W1C[i][0]:W1C[i][1]], sem_a.at[i])
        cw2 = lambda i: copy(w2_hbm.at[W2C[i][0]:W2C[i][1]], w2_v.at[W2C[i][0]:W2C[i][1]], sem_b.at[i])
        co = lambda i, c: copy(o_v.at[rows(i), c * 128:(c + 1) * 128], o_hbm.at[rows(i), c * 128:(c + 1) * 128], sem_o)
        cF = copy(C_hbm.at[0:2 * B], F_ref, sem_a.at[3])
        cG = copy(C_hbm.at[2 * B:3 * B], G_ref, sem_b.at[1])
        cD = copy(sD_hbm, sD_ref, sem_a.at[3])
        csk = copy(sk_hbm, sk_ref, sem_b.at[0])
        cb1 = copy(b1_hbm, b1_ref, sem_a.at[0])
        cb2 = copy(b2_hbm, b2_ref, sem_b.at[0])

        def wait(name, copies):
            with jax.named_scope(name):
                for cp in copies:
                    cp.wait()

        def bar():
            pl.semaphore_signal(sem_bar, 1)
            pl.semaphore_wait(sem_bar, 1)

        g0, g1, g2, g3 = [cx(0)], [cb1, cw1(0)], [cx(1), cw1(1)], [cw1(2)]
        g4 = [cw1(3), cF, cD] + [ch(c) for c in range(nh1)]
        g5 = [ch(c) for c in range(nh1, NT)] + [cb2, cw2(0), csk, ck(0), cv(0)]
        g6 = [cw2(1), cG, ck(1), cv(1)]
        blk = lambda i: [cx(i), ck(i), cv(i)]
        for cp in g0 + g1 + g2 + g3 + g4 + g5:
            cp.start()
            bar()
        for i, grp in enumerate([g6] + [blk(i) for i in range(2, NSTEP)]):
            for cp in grp:
                cp.start()
            if i in (0, 1, 2, 4):
                bar()

        zero = jnp.clip(z_ref[0], 0, 1)
        never = jnp.full((8, 128), zero, jnp.int32) != 0
        KV[0:16, :] = jnp.zeros((16, D), bf16)
        UH[Z] = jnp.zeros(UH.shape[1:], f32)

        def kv_block(t, anchors):
            nrc = TM // KVROWS
            for c in range(NT):
                cs = slice(c * 128, (c + 1) * 128)
                skb_ref[pl.ds(pl.multiple_of(32 + zero * 8, 8), 8), 0:128] = anchors[c * nrc]
                sk = [jnp.concatenate([skb_ref[8 * j:8 * j + 8, cs]] * (KVROWS // 8), axis=0) for j in range(4)]
                for rc in range(nrc):
                    KV[pl.ds(pl.multiple_of(FO + zero * 16, 16), 8), 0:128] = anchors[c * nrc + rc].astype(bf16)
                    r0 = t * TM + rc * KVROWS
                    vv = KV[pl.ds(al(r0 + VO, 16), KVROWS), cs].astype(f32)
                    kext = KV[pl.ds(al(r0, 16), KVROWS + 16), cs].astype(f32)[8:]
                    ks = kext[8:] * sk[0]
                    for j in range(1, 4):
                        ks = ks + pltpu.roll(kext, j, 0)[8:, :] * sk[j]
                    kvb_ref[rc * KVROWS // 2:(rc + 1) * KVROWS // 2, cs] = pk((ks * vv).astype(bf16))

        def u_dft(t):
            fm = F_ref[...]
            for j in range(2):
                u = jnp.dot(fm, upk(kvb_ref[j * HB:(j + 1) * HB, :]), preferred_element_type=f32)
                u = u.reshape(R8, 2, 8, D)
                a, b = u[:, 0], u[:, 1]
                UH[2 * t + j, :, 0] = a + b
                UH[2 * t + j, :, 1] = a
                UH[2 * t + j, :, 2] = b
            return b[R8 - 1, :, D - 128:]

        def h_rounds(c):
            cs = slice(c * 128, (c + 1) * 128)
            hp_re = hp_im = None
            for a in range(NB):
                fm = F_ref[...]
                hh = lax.dot_general(fm, h_v[cs, a * B:(a + 1) * B], NT_DIMS, preferred_element_type=f32)
                if a == 0:
                    hh = hh + fm[:, 0:1].astype(f32) * sD_ref[...].astype(f32)[None, cs]
                h4 = hh.reshape(R8, 2, 8, 128)
                hre, him = h4[:, 0], h4[:, 1]
                if a == 0:
                    c_, d_ = hre, him
                else:
                    e = R8 // 2
                    c_ = jnp.concatenate([hre[:e] - hp_im[:e], hre[e:] + hp_im[e:]], axis=0)
                    d_ = jnp.concatenate([him[:e] + hp_re[:e], him[e:] - hp_re[e:]], axis=0)
                UH[H0 + a, :, 0, :, cs] = c_
                UH[H0 + a, :, 1, :, cs] = d_ - c_
                UH[H0 + a, :, 2, :, cs] = c_ + d_
                hp_re, hp_im = hre, him
                if a % 4 == 3:
                    yield hh

        def layernorm(t, dst, anchors=None):
            n = 1 if anchors is None else len(anchors)
            rr = TM // n
            for i in range(n):
                if anchors is not None:
                    x_v[pl.ds(pl.multiple_of(S + zero * 16, 16), 8), 0:128] = anchors[i].astype(bf16)
                x = x_v[pl.ds(al(t * TM + i * rr, 16), rr), :].astype(f32)
                m = jnp.mean(x, axis=-1, keepdims=True)
                xc = x - m
                var = jnp.mean(xc * xc, axis=-1, keepdims=True)
                xn = xc * lax.rsqrt(var + 1e-5)
                dst[i * rr // 2:(i + 1) * rr // 2, :] = pk(xn.astype(bf16))

        c1 = np.float32(2 * np.sqrt(2 / np.pi))
        c2 = np.float32(8 * np.sqrt(2 / np.pi) * 0.044715)

        def gelu(h):
            return (h + h * jnp.tanh(h * (c1 + c2 * (h * h)))).astype(bf16)

        def mlp1(xr, lo, hi):
            b1 = b1_ref[...].astype(f32)[None, :] * 0.5
            h = lax.dot_general(upk(xr[...]), upk(w1p[lo // 2:hi // 2, :]), NT_DIMS, preferred_element_type=f32)
            return gelu(h + b1[:, lo:hi])

        def mlp1_rem(xr):
            ht = lax.dot_general(upk(w1p[FM // 2:, :]), upk(xr[...]), NT_DIMS, preferred_element_type=f32)
            return gelu(ht + jnp.concatenate([b1c_ref[...]] * (ht.shape[1] // 128), axis=1)).T

        def mac(t, anchor=None, depth=0):
            if anchor is not None:
                UH[DUM, zero, 0, :, 0:128] = anchor
            if static(t):
                uslot = [2 * t + 1 - l for l in range(2 * t + 2)]
            else:
                uslot = [2 * t + 1 - l if l < 6 else jnp.where(2 * t + 1 - l >= 0, 2 * t + 1 - l, Z)
                         for l in range(NB)]
            nlag = len(uslot)
            pend = []
            for ci in range(NT):
                cs = slice(ci * 128, (ci + 1) * 128)
                for r2 in range(0, R8, 2):
                    ld = lambda s: [UH[s, r2:r2 + 2, c_, :, cs].reshape(16, 128) for c_ in range(3)]
                    add = lambda acc, p: p if acc is None else [x_ + y_ for x_, y_ in zip(acc, p)]
                    acc0 = acc1 = None
                    ucur = ld(uslot[0])
                    for l in range(nlag):
                        hv = ld(H0 + l)
                        p1 = [hv[c_] * ucur[c_] for c_ in range(3)]
                        if l + 1 < nlag:
                            ucur = ld(uslot[l + 1])
                            acc0 = add(acc0, [hv[c_] * ucur[c_] for c_ in range(3)])
                        acc1 = add(acc1, p1)
                    w = []
                    for acc in (acc0, acc1):
                        w.append(pk((acc[0] - acc[2]).astype(bf16)))
                        w.append(pk((acc[0] + acc[1]).astype(bf16)))
                    tie = (w[0] | w[1]) | (w[2] | w[3])
                    w = [jnp.where(never, tie, w_) for w_ in w]
                    if depth:
                        pend.append(tie)
                        if len(pend) >= depth:
                            UH[DUM, zero, 0, :, 0:128] = pltpu.bitcast(pend.pop(0), f32)
                    for j in range(2):
                        col = slice(ci * 256 + j * 128, ci * 256 + (j + 1) * 128)
                        Q_ref[r2 * 4:r2 * 4 + 8, col] = w[2 * j]
                        Q_ref[HB + r2 * 4:HB + r2 * 4 + 8, col] = w[2 * j + 1]

        def idft():
            flip = 7 - lax.broadcasted_iota(jnp.int32, (8, 128), 0)
            ys = []
            for c in range(NT):
                qs = slice(c * 256, (c + 1) * 256)
                cc = jnp.dot(G_ref[0:HB, :], upk(Q_ref[0:HB, qs]), preferred_element_type=f32)
                ss = jnp.dot(G_ref[HB:, :], upk(Q_ref[HB:, qs]), preferred_element_type=f32)
                lo, hi = cc - ss, cc + ss
                pieces = []
                for j in range(2):
                    js = slice(j * 128, (j + 1) * 128)
                    pieces.append(lo[:, js])
                    pieces += [jnp.take_along_axis(hi[r * 8:(r + 1) * 8, js], flip, axis=0)
                               for r in reversed(range(HB // 8))]
                ys.append(jnp.concatenate(pieces, axis=0))
            return ys

        def combine(t, ys, os_, xb):
            for c in range(NT):
                cs = slice(c * 128, (c + 1) * 128)
                out = (upk(xb[:, cs]).astype(f32) * ys[c] + os_[c]) + x_v[rows(t), cs].astype(f32)
                o_v[rows(t), cs] = out.astype(bf16)
                co(t, c).start()

        G = {}

        def mlp1_piece(q0, q1, n0, n1, split):
            for q in range(q0, q1, split):
                g_ = mlp1(x2_ref.at[q * 64:(q + split) * 64], n0 * 128, n1 * 128)
                for qq in range(split):
                    for n in range(n0, n1):
                        G[(q + qq, n)] = g_[qq * 128:(qq + 1) * 128, (n - n0) * 128:(n - n0 + 1) * 128]

        def w1_load(i):
            lo, hi = W1C[i]
            w1p[lo // 2:hi // 2, :] = pk((w1_v[lo:hi, :].astype(f32) * 0.5).astype(bf16))

        n1, n2, n3 = (W1C[i][1] // 128 for i in range(3))
        def mlp1_cols(q0, q1, n0, n1_):
            e = n1_ - (n1_ - n0) % 4
            if e > n0:
                mlp1_piece(q0, q1, n0, e, q1 - q0)
            for n in range(e, n1_):
                if q1 - q0 == 2 and (n1_ - e) % 2 == 1 and n == e:
                    for q in range(q0, q1):
                        G[(q, n)] = jnp.concatenate(
                            [mlp1(x2_ref.at[q * 64 + h * 32:q * 64 + (h + 1) * 32], n * 128, (n + 1) * 128)
                             for h in range(2)], axis=0)
                else:
                    mlp1_piece(q0, q1, n, n + 1, 1)

        wait("w0", g0)
        layernorm(0, x2_ref.at[0:TM // 2])
        wait("w1", g1)
        w1_load(0)
        mlp1_cols(0, 2, 0, n1)

        wait("w2", g2)
        w1_load(1)
        mlp1_cols(0, 2, n1, n2)
        layernorm(1, x2_ref.at[TM // 2:TM])
        mlp1_cols(2, 4, 0, n2)

        wait("w3", g3)
        w1_load(2)
        b1t = jnp.broadcast_to(b1_ref[...].astype(f32)[None, F - 128:], (128, 128)).T
        b1c_ref[...] = b1t[64:] * 0.5
        mlp1_cols(0, 4, n2, n3)

        wait("w4", g4)
        w1_load(3)
        gr = mlp1_rem(x2_ref)
        rounds = itertools.chain(*[h_rounds(c) for c in range(nh1)])
        pieces = [(q, n) for n in range(n3, FM // 128) for q in range(4)]
        done = 0
        for i, (q, n) in enumerate(pieces):
            for _ in range((i + 1) * 4 * nh1 // len(pieces) - done):
                next(rounds)
                done += 1
            mlp1_piece(q, q + 1, n, n + 1, 1)

        wait("w5", g5)
        skf = sk_ref[...].astype(f32)
        for j in range(4):
            skb_ref[8 * j:8 * j + 8, :] = jnp.broadcast_to(skf[j:j + 1, :], (8, D))
        b2 = b2_ref[...].astype(f32)[None, :]
        parts = []

        def gslice(qs, k0, k1):
            rws = []
            for q in qs:
                tiles = [G[(q, n)] for n in range(k0 // 128, min(k1, FM) // 128)]
                if k1 > FM:
                    tiles.append(gr[q * 128:(q + 1) * 128])
                rws.append(jnp.concatenate(tiles, axis=1))
            return jnp.concatenate(rws, axis=0)

        def mmk(qs, n, k0, k1, acc, fresh):
            cs = slice(n * 128, (n + 1) * 128)
            if fresh:
                w2 = w2_v[k0:k1, cs]
                w2p[k0 // 2:k1 // 2, cs] = pk(w2)
            else:
                w2 = upk(w2p[k0 // 2:k1 // 2, cs])
            acc = jnp.dot(gslice(qs, k0, k1), w2, preferred_element_type=f32) + (b2[:, cs] if acc is None else acc)
            parts.extend(row_anchors(acc, 8 * len(qs)))
            return acc

        rounds = itertools.chain(*[h_rounds(c) for c in range(nh1, NT)])
        nr = 4 * (NT - nh1)
        o0 = []
        done = 0
        for i in range(2 * NT):
            o0.append(mmk([i % 2], i // 2, *KG[0], None, i % 2 == 0))
            for _ in range(min(nr, ((i + 1) * nr) // (2 * NT - 1)) - done):
                parts.extend(row_anchors(next(rounds)))
                done += 1
        o0 = [jnp.concatenate(o0[2 * n:2 * n + 2], axis=0) for n in range(NT)]
        o1 = [mmk([2, 3], n, *KG[0], None, False) if n < npull else None for n in range(NT)]
        kv_block(0, spread(parts, *ra[0], NCH))

        wait("w6", g6)
        parts.clear()
        rest = [(n, g) for n in range(NT) for g in KG[1:]]
        ul = u_dft(0)
        for n, g in rest[:fs1]:
            o0[n] = mmk([0, 1], n, *g, o0[n], True)
        mac(0, ul, fsd[0])
        ys = idft()
        for n, g in rest[fs1:]:
            o0[n] = mmk([0, 1], n, *g, o0[n], True)
        kv_block(1, spread(parts, *ra[1], NCH))
        combine(0, ys, o0, x2_ref.at[0:TM // 2])

        wait("w7", blk(2))
        parts.clear()
        rest = [(n, g) for n in range(NT) for g in KG if not (g == KG[0] and n < npull)]
        ul = u_dft(1)
        for n, g in rest[:15 - npull]:
            o1[n] = mmk([2, 3], n, *g, o1[n], False)
        mac(1, ul, fsd[1])
        ys = idft()
        for n, g in rest[15 - npull:]:
            o1[n] = mmk([2, 3], n, *g, o1[n], False)
        layernorm(2, xn_ref, spread(parts, *ra[3], NLN[0]))
        kv_block(2, spread(parts, *ra[2], NCH))
        combine(1, ys, o1, x2_ref.at[TM // 2:TM])

        def body(t, carry):
            @pl.when(t + 1 < NSTEP)
            def _():
                wait("lw", blk(t + 1))

            with jax.named_scope("step"):
                tn = jnp.minimum(t + 1, NSTEP - 1)
                u_dft(t)
                xb_ref[...] = xn_ref[...]
                g = mlp1(xn_ref, 0, FM)
                glast = jnp.concatenate([g[:, KG[-1][0]:], mlp1_rem(xn_ref)], axis=1)
                b2 = b2_ref[...].astype(f32)[None, :]
                parts, os_ = [], []
                for n in range(NT):
                    cs = slice(n * 128, (n + 1) * 128)
                    acc = b2[:, cs]
                    for k0, k1 in KG:
                        acc = jnp.dot(g[:, k0:k1] if k1 < F else glast, upk(w2p[k0 // 2:k1 // 2, cs]),
                                      preferred_element_type=f32) + acc
                        parts.extend(row_anchors(acc))
                    os_.append(acc)
                mac(t)
                ys = idft()
                kv_block(tn, spread(parts, *la[0], NCH))
                layernorm(tn, xn_ref, spread(parts, *la[1], NLN[1]))
                combine(t, ys, os_, xb_ref)
            return carry

        lax.fori_loop(2, NSTEP, body, 0)
        wait("wo", [co(i, c) for i in range(NSTEP) for c in range(NT)])

    consts = dft_mats()

    @jax.jit
    def f(A_q, A_k, A_v, A_shift_k, A_ssm_k, A_ssm_D, B_x, B_w1, B_b1, B_w2, B_b2):
        vm = pltpu.VMEM
        dma = pltpu.SemaphoreType.DMA
        out = pl.pallas_call(
            kern,
            in_specs=[pl.BlockSpec(memory_space=pltpu.SMEM)] + [pl.BlockSpec(memory_space=pl.ANY)] * 11,
            out_specs=pl.BlockSpec(memory_space=pl.ANY),
            out_shape=jax.ShapeDtypeStruct((S, D), bf16),
            scratch_shapes=[
                vm((2 * NB + 2, R8, 3, 8, D), f32), vm((S + 64, D), bf16), vm((S, D), bf16), vm((KVR, D), bf16),
                vm((D, S), bf16), vm((F, D), bf16), vm((F, D), bf16),
                vm((F // 2, D), u32), vm((F // 2, D), u32),
                vm((TM // 2, D), u32), vm((B, 2 * D), u32), vm((TM // 2, D), u32), vm((TM // 2, D), u32),
                vm((TM, D), u32), vm((48, D), f32), vm((64, 128), f32),
                vm((4, D), bf16), vm((D,), bf16), vm((F,), bf16), vm((D,), bf16), vm((3 * B, B), bf16),
                dma((NSTEP - 2,)), dma((5,)), dma((2,)), dma(()), pltpu.SemaphoreType.REGULAR,
            ],
            compiler_params=pltpu.CompilerParams(
                vmem_limit_bytes=110 * 1024 * 1024,
                disable_bounds_checks=not checks, disable_semaphore_checks=not checks),
        )(jnp.zeros((1,), jnp.int32), A_q.reshape(S, D), A_k.reshape(S, D), A_v.reshape(S, D), A_ssm_k,
          B_w1.T, B_w2, A_shift_k.T, A_ssm_D, B_b1, B_b2, jnp.asarray(consts, bf16))
        return out.reshape(1, S, D)

    return f


_impl = make()


@jax.jit
def pallas_parallel_sum__ssm_conv_h3__dense_activation_gelu__prompt_kernel(
    A_q, A_k, A_v, A_shift_k, A_ssm_k, A_ssm_D, B_x, B_w1, B_b1, B_w2, B_b2
):
    return _impl(A_q, A_k, A_v, A_shift_k, A_ssm_k, A_ssm_D, B_x, B_w1, B_b1, B_w2, B_b2)
```
